```python
import os as _os
_os.environ.setdefault('JAX_PLATFORMS', 'cpu')
import jax
import jax.numpy as jnp

def _softmax(x, axis=-1):
    return jax.nn.softmax(x, axis=axis)

def _gelu(x):
    return jax.nn.gelu(x, approximate=True)

def _silu(x):
    return jax.nn.silu(x)

def _sigmoid(x):
    return jax.nn.sigmoid(x)

def _layernorm(x, axis=-1, eps=1e-05):
    m = jnp.mean(x, axis=axis, keepdims=True)
    v = jnp.var(x, axis=axis, keepdims=True)
    return (x - m) / jnp.sqrt(v + eps)

def _scatter_add(tgt, idx, src, axis=0):
    return tgt.at[idx].add(src)

def _segment_sum(src, seg, n):
    return jax.ops.segment_sum(src, seg, n)

class _Rng:

    def __init__(self, key):
        self._k = key

    def _next(self):
        self._k, sub = jax.random.split(self._k)
        return sub

    def normal(self, shape):
        return jax.random.normal(self._next(), shape, dtype=jnp.bfloat16)

    def randint(self, lo, hi, shape):
        return jax.random.randint(self._next(), shape, lo, hi, dtype=jnp.int32)

    def uniform(self, shape, lo=0.0, hi=1.0):
        return jax.random.uniform(self._next(), shape, jnp.bfloat16, lo, hi)

    def permutation(self, n):
        return jax.random.permutation(self._next(), n)
kernel_name = 'interleave_layers__ssm_conv_h3__mixer_gmlp__prompt'

def setup_inputs():
    _rng = _Rng(jax.random.key(int.from_bytes(__import__("os").urandom(4), "little")))
    _w = lambda a: (lambda t: t.astype(jnp.bfloat16) if jnp.issubdtype(t.dtype, jnp.floating) else t)(jnp.asarray(a))

    def _A_setup():
        B, S, D = (1, 2048, 1024)
        ks = 4
        return {'q': _w((lambda *s: _rng.normal(s) * 0.05)(B, S, D)), 'k': _w((lambda *s: _rng.normal(s) * 1.6)(B, S, D)), 'v': _w((lambda *s: _rng.normal(s) * 1.6)(B, S, D)), 'shift_k': _w((lambda *s: _rng.normal(s) * 1.6)(D, ks) * 0.5), 'ssm_k': _w((lambda *s: _rng.normal(s) * 1.6)(D, S) * (1.0 / S ** 0.5)), 'ssm_D': _w((lambda *s: _rng.normal(s) * 1.6)(D))}
    _A_in = _A_setup()

    def _B_setup():
        B, S, D, F = (1, 2048, 1024, 3584)
        Fh = F // 2
        return {'x': _w((lambda *s: _rng.normal(s) * 0.05)(B, S, D)), 'w_in': _w((lambda *s: _rng.normal(s) * 0.8)(D, 2 * Fh)), 'w_sp': _w(0.01 * (lambda *s: _rng.normal(s) * 0.8)(S, S)), 'b_sp': _w(1.0 + 0.01 * (lambda *s: _rng.normal(s) * 0.2)(S)), 'w_out': _w((lambda *s: _rng.normal(s) * 0.2)(Fh, D))}
    _B_in = _B_setup()
    return {'A_q': _A_in['q'], 'A_k': _A_in['k'], 'A_v': _A_in['v'], 'A_shift_k': _A_in['shift_k'], 'A_ssm_k': _A_in['ssm_k'], 'A_ssm_D': _A_in['ssm_D'], 'B_x': _B_in['x'], 'B_w_in': _B_in['w_in'], 'B_w_sp': _B_in['w_sp'], 'B_b_sp': _B_in['b_sp'], 'B_w_out': _B_in['w_out']}

def reference(A_q, A_k, A_v, A_shift_k, A_ssm_k, A_ssm_D, B_x, B_w_in, B_w_sp, B_b_sp, B_w_out):

    def _A_ref(q, k, v, shift_k, ssm_k, ssm_D):
        B, S, D = q.shape
        ks = shift_k.shape[-1]
        k_pad = jnp.pad(k, ((0, 0), (ks - 1, 0), (0, 0)))
        k_shift = jnp.zeros_like(k)
        for t in range(ks):
            k_shift = k_shift + k_pad[:, t:t + S, :] * shift_k[:, ks - 1 - t][None, None, :]
        kv = k_shift * v
        L = 2 * S
        kv_pad = jnp.pad(kv, ((0, 0), (0, S), (0, 0)))
        kf_pad = jnp.pad(ssm_k, ((0, 0), (0, S)))
        kv_f = (lambda x, axes=(-2, -1): jnp.fft.rfft2(x.astype(jnp.float32), axes=axes))(kv_pad[:, None, :, :], axes=(1, 2))
        kf_f = (lambda x, axes=(-2, -1): jnp.fft.rfft2(x.astype(jnp.float32), axes=axes))(kf_pad[:, None, :], axes=(1, 2))
        kf_f = (lambda x, *d: x.transpose(*d))(kf_f, 1, 2, 0)
        y_f = kv_f * kf_f[None, :, :, :]
        y = (lambda x, s, axes=(-2, -1): jnp.fft.irfft2(x, s=s, axes=axes).astype(jnp.bfloat16))(y_f, (1, L), axes=(1, 2))[:, 0, :S, :]
        y = y + kv * ssm_D[None, None, :]
        return q * y

    def _B_ref(x, w_in, w_sp, b_sp, w_out):
        B, S, D = x.shape
        F = w_in.shape[-1]
        Fh = F // 2
        z = _gelu(jnp.einsum('bsd,df->bsf', x, w_in))
        z1 = z[..., :Fh].copy()
        z2 = _layernorm(z[..., Fh:], axis=-1)
        g = jnp.einsum('ts,bsf->btf', w_sp, z2) + b_sp[None, :, None]
        return jnp.einsum('bsf,fd->bsd', z1 * g, w_out)
    x = A_q
    x = x + _A_ref(_layernorm(x, axis=-1), A_k, A_v, A_shift_k, A_ssm_k, A_ssm_D)
    x = x + _B_ref(_layernorm(x, axis=-1), B_w_in, B_w_sp, B_b_sp, B_w_out)
    x = x + _A_ref(_layernorm(x, axis=-1), A_k, A_v, A_shift_k, A_ssm_k, A_ssm_D)
    x = x + _B_ref(_layernorm(x, axis=-1), B_w_in, B_w_sp, B_b_sp, B_w_out)
    return x
```

```python
import math
import jax
import jax.numpy as jnp
from jax import lax
import jax.experimental.pallas as pl
import jax.experimental.pallas.tpu as pltpu

S = 2048
D = 1024
F = 3584
FH = F // 2
KS = 4
B = 128
NB = S // B
EPS = 1e-5
f32 = jnp.float32
bf16 = jnp.bfloat16

CT = 256
TM = 256
TN = 256
RG = 16


def _gelu(x):
    return 0.5 * x * (1.0 + jnp.tanh(0.7978845608028654 * (x + 0.044715 * (x * x * x))))


def _ln(x):
    n = x.shape[-1]
    m = jnp.sum(x, axis=-1, keepdims=True) * (1.0 / n)
    xc = x - m
    v = jnp.sum(xc * xc, axis=-1, keepdims=True) * (1.0 / n)
    return xc * lax.rsqrt(v + EPS)


def _dft_rows(shape, row_dim):
    r = lax.broadcasted_iota(jnp.int32, shape, row_dim)
    n = lax.broadcasted_iota(jnp.int32, shape, 1 - row_dim)
    is_im = r >= B
    rr = jnp.where(is_im, r - B, r)
    odd = rr >= B // 2
    fidx = jnp.where(odd, 2 * (rr - B // 2) + 1, 2 * rr)
    m = (2 * fidx + 1) * n - jnp.where(is_im, B, 0)
    m = jnp.bitwise_and(m, 4 * B - 1)
    m = jnp.where(m > 2 * B, 4 * B - m, m)
    return jnp.cos(m.astype(f32) * (math.pi / (2 * B)))


def _kernel(q_hbm, k_hbm, v_hbm, sk_hbm, h_hbm, sd_hbm, win_hbm, wsp_hbm, bsp_hbm, wout_hbm,
            o_hbm,
            qb, kb, vb, hb, win, wsp, wout, skb, sdb, bspb,
            x_v, y_v, z1_v, z2a, z2b, bb_v, skt, fm_v, im_v, kvb, kvh, h2h, zt, ob,
            sem_c, sem_w, sem_s, sem_o):
    nct = D // CT

    def conv_copies(c):
        cols = pl.ds(c * CT, CT)
        return [
            pltpu.make_async_copy(k_hbm.at[0, :, cols], kb.at[:, cols], sem_c.at[0, c]),
            pltpu.make_async_copy(v_hbm.at[0, :, cols], vb.at[:, cols], sem_c.at[1, c]),
            pltpu.make_async_copy(h_hbm.at[cols, :], hb.at[cols, :], sem_c.at[2, c]),
        ]

    small = [
        pltpu.make_async_copy(sk_hbm, skb, sem_s.at[0]),
        pltpu.make_async_copy(sd_hbm, sdb, sem_s.at[1]),
        pltpu.make_async_copy(bsp_hbm, bspb, sem_s.at[2]),
    ]
    big = [
        pltpu.make_async_copy(q_hbm.at[0], qb, sem_w.at[0]),
        pltpu.make_async_copy(win_hbm, win, sem_w.at[1]),
        pltpu.make_async_copy(wsp_hbm, wsp, sem_w.at[2]),
        pltpu.make_async_copy(wout_hbm, wout, sem_w.at[3]),
    ]
    for cp in small:
        cp.start()
    for c in range(nct):
        for cp in conv_copies(c):
            cp.start()
    for cp in big:
        cp.start()

    fm_v[...] = _dft_rows((2 * B, B), 0).astype(bf16)
    im_v[...] = (_dft_rows((B, 2 * B), 1) * (1.0 / B)).astype(bf16)

    for cp in small:
        cp.wait()
    sel = (lax.broadcasted_iota(jnp.int32, (8, KS), 0) ==
           lax.broadcasted_iota(jnp.int32, (8, KS), 1)).astype(bf16)
    skt[...] = lax.dot_general(sel, skb[...], (((1,), (1,)), ((), ())), preferred_element_type=f32)
    bb_v[...] = jnp.transpose(jnp.broadcast_to(bspb[...].astype(f32), (128, S)))

    def conv_body(c, carry):
        cols = pl.ds(pl.multiple_of(c * CT, CT), CT)
        for j in range(3):
            pltpu.make_async_copy(kb.at[:, pl.ds(0, CT)], kb.at[:, pl.ds(0, CT)], sem_c.at[j, c]).wait()
        sk = skt[:, cols]
        sd = sdb[:, cols].astype(f32)
        fm = fm_v[...]
        row = lax.broadcasted_iota(jnp.int32, (8, CT), 0)
        for a in range(NB):
            kcur = kb[a * B:(a + 1) * B, cols].astype(f32)
            if a == 0:
                kprev = jnp.zeros((8, CT), f32)
            else:
                kprev = kb[a * B - 16:a * B, cols].astype(f32)[8:16]
            ks = kcur * sk[0:1]
            for j in range(1, KS):
                rolled = pltpu.roll(kcur, j, 0)
                head = jnp.where(row < j, pltpu.roll(kprev, j, 0), rolled[0:8])
                shifted = jnp.concatenate([head, rolled[8:]], axis=0)
                ks = ks + shifted * sk[j:j + 1]
            kv = (ks * vb[a * B:(a + 1) * B, cols].astype(f32)).astype(bf16)
            y_v[a * B:(a + 1) * B, cols] = kv.astype(f32) * sd
            kvh[a] = jnp.dot(fm, kv, preferred_element_type=f32)
            hh = lax.dot_general(fm, hb[cols, a * B:(a + 1) * B], (((1,), (1,)), ((), ())),
                                 preferred_element_type=f32)
            if a == 0:
                h2h[0] = hh
            else:
                q4 = B // 2
                h2h[a, 0:q4] = hh[0:q4] + hprev[2 * q4:3 * q4]
                h2h[a, q4:2 * q4] = hh[q4:2 * q4] - hprev[3 * q4:4 * q4]
                h2h[a, 2 * q4:3 * q4] = hh[2 * q4:3 * q4] - hprev[0:q4]
                h2h[a, 3 * q4:4 * q4] = hh[3 * q4:4 * q4] + hprev[q4:2 * q4]
            hprev = hh
        imat = im_v[...]
        for a in range(NB):
            for r in range(0, B, RG):
                zr = zi = None
                for ap in range(a + 1):
                    xr = kvh[ap, r:r + RG]
                    xi = kvh[ap, B + r:B + r + RG]
                    hr = h2h[a - ap, r:r + RG]
                    hi = h2h[a - ap, B + r:B + r + RG]
                    tr = xr * hr - xi * hi
                    ti = xr * hi + xi * hr
                    zr = tr if zr is None else zr + tr
                    zi = ti if zi is None else zi + ti
                kvb[r:r + RG] = zr.astype(bf16)
                kvb[B + r:B + r + RG] = zi.astype(bf16)
            y_v[a * B:(a + 1) * B, cols] += jnp.dot(imat, kvb[...], preferred_element_type=f32)
        return carry

    with jax.named_scope('stageA'):
        lax.fori_loop(0, nct, conv_body, 0)

    def p1(rows, xin, z2_out):
        x1 = xin + _ln(xin) * y_v[rows, :]
        x_v[rows, :] = x1
        xn = _ln(x1).astype(bf16)
        ssum = None
        for n in range(FH // TN):
            z = _gelu(jnp.dot(xn, win[:, FH + n * TN:FH + (n + 1) * TN], preferred_element_type=f32))
            zt[:, n * TN:(n + 1) * TN] = z
            for l in range(TN // 128):
                piece = z[:, l * 128:(l + 1) * 128]
                ssum = piece if ssum is None else ssum + piece
        mean = jnp.sum(ssum, axis=-1, keepdims=True) * (1.0 / FH)
        vsum = None
        for n in range(FH // TN):
            z1_v[rows, n * TN:(n + 1) * TN] = _gelu(
                jnp.dot(xn, win[:, n * TN:(n + 1) * TN], preferred_element_type=f32)).astype(bf16)
        for n in range(FH // 128):
            zc = zt[:, n * 128:(n + 1) * 128] - mean
            zc = zc * zc
            vsum = zc if vsum is None else vsum + zc
        rstd = lax.rsqrt(jnp.sum(vsum, axis=-1, keepdims=True) * (1.0 / FH) + EPS)
        for n in range(FH // TN):
            z2_out[rows, n * TN:(n + 1) * TN] = ((zt[:, n * TN:(n + 1) * TN] - mean) * rstd).astype(bf16)

    def p2(rows, z2_in):
        ws = wsp[rows, :]
        bb = bb_v[rows, :]
        bbt = jnp.concatenate([bb] * (TN // 128), axis=1)
        us = []
        for n in range(FH // TN):
            g = jnp.dot(ws, z2_in[:, n * TN:(n + 1) * TN], preferred_element_type=f32) + bbt
            us.append((z1_v[rows, n * TN:(n + 1) * TN].astype(f32) * g).astype(bf16))
        u = jnp.concatenate(us, axis=1)
        return x_v[rows, :] + jnp.dot(u, wout[...], preferred_element_type=f32)

    nt = S // TM
    big[0].wait()
    big[1].wait()

    def stage_b(t, carry):
        rows = pl.ds(pl.multiple_of(t * TM, TM), TM)
        p1(rows, qb[rows, :].astype(f32), z2a)
        return carry

    with jax.named_scope('stageB'):
        lax.fori_loop(0, nt, stage_b, 0)
    big[2].wait()
    big[3].wait()

    def stage_c(t, carry):
        rows = pl.ds(pl.multiple_of(t * TM, TM), TM)
        x2 = p2(rows, z2a)
        p1(rows, x2, z2b)
        return carry

    with jax.named_scope('stageC'):
        lax.fori_loop(0, nt, stage_c, 0)

    def out_copy(t, slot):
        rows = pl.ds(pl.multiple_of(t * TM, TM), TM)
        return pltpu.make_async_copy(ob.at[slot], o_hbm.at[0, rows, :], sem_o.at[slot])

    def stage_d(t, carry):
        rows = pl.ds(pl.multiple_of(t * TM, TM), TM)
        slot = t % 2
        x4 = p2(rows, z2b)

        @pl.when(t >= 2)
        def _():
            out_copy(t - 2, slot).wait()

        ob[slot] = x4.astype(bf16)
        out_copy(t, slot).start()
        return carry

    with jax.named_scope('stageD'):
        lax.fori_loop(0, nt, stage_d, 0)
    out_copy(nt - 2, 0).wait()
    out_copy(nt - 1, 1).wait()


@jax.jit
def pallas_interleave_layers__ssm_conv_h3__mixer_gmlp__prompt_kernel(A_q, A_k, A_v, A_shift_k, A_ssm_k, A_ssm_D, B_x, B_w_in, B_w_sp, B_b_sp, B_w_out):
    del B_x
    any_spec = pl.BlockSpec(memory_space=pl.ANY)
    scratch = [
        pltpu.VMEM((S, D), bf16),
        pltpu.VMEM((S, D), bf16),
        pltpu.VMEM((S, D), bf16),
        pltpu.VMEM((D, S), bf16),
        pltpu.VMEM((D, F), bf16),
        pltpu.VMEM((S, S), bf16),
        pltpu.VMEM((FH, D), bf16),
        pltpu.VMEM((D, KS), bf16),
        pltpu.VMEM((1, D), bf16),
        pltpu.VMEM((1, S), bf16),
        pltpu.VMEM((S, D), f32),
        pltpu.VMEM((S, D), f32),
        pltpu.VMEM((S, FH), bf16),
        pltpu.VMEM((S, FH), bf16),
        pltpu.VMEM((S, FH), bf16),
        pltpu.VMEM((S, 128), f32),
        pltpu.VMEM((8, D), f32),
        pltpu.VMEM((2 * B, B), bf16),
        pltpu.VMEM((B, 2 * B), bf16),
        pltpu.VMEM((2 * B, CT), bf16),
        pltpu.VMEM((NB, 2 * B, CT), f32),
        pltpu.VMEM((NB, 2 * B, CT), f32),
        pltpu.VMEM((TM, FH), f32),
        pltpu.VMEM((2, TM, D), bf16),
        pltpu.SemaphoreType.DMA((3, D // CT)),
        pltpu.SemaphoreType.DMA((4,)),
        pltpu.SemaphoreType.DMA((3,)),
        pltpu.SemaphoreType.DMA((2,)),
    ]
    return pl.pallas_call(
        _kernel,
        out_shape=jax.ShapeDtypeStruct((1, S, D), bf16),
        in_specs=[any_spec] * 10,
        out_specs=any_spec,
        scratch_shapes=scratch,
        compiler_params=pltpu.CompilerParams(vmem_limit_bytes=120 * 1024 * 1024),
    )(A_q, A_k, A_v, A_shift_k, A_ssm_k, A_ssm_D.reshape(1, D), B_w_in, B_w_sp,
      B_b_sp.reshape(1, S), B_w_out)
```

```python
import functools
import math
import jax
import jax.numpy as jnp
from jax import lax
import jax.experimental.pallas as pl
import jax.experimental.pallas.tpu as pltpu

S = 2048
D = 1024
F = 3584
FH = F // 2
KS = 4
B = 128
NB = S // B
EPS = 1e-5
f32 = jnp.float32
bf16 = jnp.bfloat16
u32 = jnp.uint32

TM = 256
NT = S // TM
TN = 256
NCH = FH // TN
RG = 16
GW = 256
LR = 16
NZ = 8
CAP_A = 9
CAP_B = 14
GWF = 128
ROT = 256


def _plan(cap_a, cap_b):
    done = set((a, ap) for a in (0, 1) for ap in range(a + 1))
    blocks = {}
    for t in range(NT - 1):
        for kind, cap in (('A', cap_a), ('B', cap_b)):
            sel = {}
            n = 0
            lo = 2 * t + 2 if kind == 'A' else 2 * t + 4
            lim = 2 * t + 3
            for a in range(lo, NB):
                g = [ap for ap in range(a + 1) if (a, ap) not in done and ap <= lim and a - ap <= lim]
                if a > lim:
                    g = g[:max(cap - n, 0)]
                if g:
                    sel[a] = g
                    n += len(g)
            groups = []
            for a in sorted(sel):
                first = not any((a, x) in done for x in range(a + 1))
                done.update((a, x) for x in sel[a])
                last = all((a, x) in done for x in range(a + 1))
                assert a < lo + NZ and last == (a <= 2 * t + 3)
                groups.append((a, sel[a], first, last))
            blocks[(kind, t)] = groups
    assert len(done) == NB * (NB + 1) // 2
    return blocks


def _gelu(x):
    u = x * (0.7978845608028654 + 0.035677408136300125 * (x * x))
    h = 0.5 * x
    return h + h * jnp.tanh(u)


def _h(v):
    return pltpu.bitcast(v, bf16)


def _part(v):
    acc = v[:, 0:128]
    for c in range(128, v.shape[1], 128):
        acc = acc + v[:, c:c + 128]
    return acc


def _lsum(acc):
    return jnp.broadcast_to(jnp.sum(acc, axis=1, keepdims=True), acc.shape)


def _wide(v, n):
    return jnp.concatenate([v] * (n // 128), axis=1)


def _ln(x):
    n = x.shape[-1]
    m = jnp.sum(x, axis=-1, keepdims=True) * (1.0 / n)
    xc = x - m
    v = jnp.sum(xc * xc, axis=-1, keepdims=True) * (1.0 / n)
    return xc * lax.rsqrt(v + EPS)


def _dft_rows(shape, row_dim):
    r = lax.broadcasted_iota(jnp.int32, shape, row_dim)
    n = lax.broadcasted_iota(jnp.int32, shape, 1 - row_dim)
    is_im = r >= B
    rr = jnp.where(is_im, r - B, r)
    odd = rr >= B // 2
    fidx = jnp.where(odd, 2 * (rr - B // 2) + 1, 2 * rr)
    m = (2 * fidx + 1) * n - jnp.where(is_im, B, 0)
    m = jnp.bitwise_and(m, 4 * B - 1)
    m = jnp.where(m > 2 * B, 4 * B - m, m)
    return jnp.cos(m.astype(f32) * (math.pi / (2 * B)))


NT_DIMS = (((1,), (1,)), ((), ()))


def _kernel(q_hbm, k_hbm, v_hbm, sk_hbm, h_hbm, sd_hbm, win_hbm, wsp_hbm, bsp_hbm, wout_hbm,
            o_hbm,
            qb, kb, vb, hb, win, wsp, wout, skb, sdb, bspb,
            x_v, y_v, z1_v, z2a, z2b, bb_v, skt, fm_v, im_v, kvb, ks, hs, wold, zp, zb,
            xn_v, zt, ps, st, ua, ub, zs,
            sem_c, sem_w, sem_s, sem_o):
    plan = _plan(CAP_A, CAP_B)

    def pair_copy(j, p):
        if j == 0:
            return pltpu.make_async_copy(k_hbm.at[pl.ds(2 * p, 2)], kb.at[pl.ds(2 * p % 8, 2), pl.ds(0, B)], sem_c.at[p])
        if j == 1:
            return pltpu.make_async_copy(v_hbm.at[pl.ds(2 * p, 2)], vb.at[pl.ds(2 * p % 8, 2)], sem_c.at[NT + p])
        if j == 2:
            cols = pl.ds(p * TM, TM)
            return pltpu.make_async_copy(h_hbm.at[:, cols], hb.at[p % 2], sem_c.at[2 * NT + p])
        return pltpu.make_async_copy(q_hbm.at[p], qb.at[p % 2, pl.ds(0, TM)], sem_c.at[3 * NT + p])

    WG = ((7, 10), (10, 12), (12, 14), (0, 3), (3, 6), (6, 7))

    def w_copy(i):
        cols = pl.ds(WG[i][0] * TN, (WG[i][1] - WG[i][0]) * TN)
        return pltpu.make_async_copy(win_hbm.at[:, cols], win.at[:, cols], sem_w.at[i])

    def issue(*copies):
        for cp in copies:
            cp.start(priority=1)

    small = [
        pltpu.make_async_copy(sk_hbm, skb, sem_s.at[0]),
        pltpu.make_async_copy(sd_hbm, sdb, sem_s.at[1]),
        pltpu.make_async_copy(bsp_hbm, bspb, sem_s.at[2]),
    ]
    big = [
        pltpu.make_async_copy(wsp_hbm, wsp, sem_s.at[3]),
        pltpu.make_async_copy(wout_hbm, wout, sem_s.at[4]),
    ]
    for cp in small:
        cp.start()
    pair_copy(0, 0).start(priority=1)
    pair_copy(1, 0).start(priority=1)

    def zinit(i, c):
        zs[i] = 0
        return c
    lax.fori_loop(0, 16, zinit, 0)
    issue(pair_copy(2, 0))

    fm_v[...] = _dft_rows((2 * B, B), 0).astype(bf16)
    im_v[...] = (_dft_rows((B, 2 * B), 1) * (1.0 / B)).astype(bf16)

    for cp in small:
        cp.wait()
    sk4 = skb[...].astype(f32)
    for j in range(KS):
        skt[j] = jnp.broadcast_to(sk4[j:j + 1, :], (8, D))
    sd8 = sdb[...].astype(f32)
    skt[KS] = jnp.concatenate([jnp.broadcast_to(sd8[i:i + 1, :], (8, 128)) for i in range(8)], axis=1)

    def kvprep(p, z):
        for a in (2 * p, 2 * p + 1):
            for c in range(0, D, GW):
                for r0 in range(0, B, 32):
                    kcur = kb[a % 8 + z, r0:r0 + 32, c:c + GW].astype(f32)
                    if a == 0 and r0 == 0:
                        kprev = jnp.zeros((8, GW), f32)
                    elif r0 == 0:
                        kprev = kb[(a - 1) % 8 + z, B - 16:B, c:c + GW].astype(f32)[8:16]
                    else:
                        kprev = kb[a % 8 + z, r0 - 16:r0, c:c + GW].astype(f32)[8:16]
                    ext = jnp.concatenate([kprev, kcur], axis=0)
                    sk = [jnp.concatenate([skt[j, :, c:c + GW]] * 4, axis=0) for j in range(KS)]
                    acc = kcur * sk[0]
                    for j in range(1, KS):
                        acc = acc + pltpu.roll(ext, j, 0)[8:] * sk[j]
                    kvb[a % 4, r0:r0 + 32, c:c + GW] = (acc * vb[a % 8, r0:r0 + 32, c:c + GW].astype(f32)).astype(bf16)

    CW = 512

    def rot(c, k, w):
        c = (c + ROT * k) % D
        return slice(c, c + w)

    def put(ref, i, c, val, k):
        for j in range(0, CW, 256):
            ref[i, 0:B, rot(c + j, k, 256)] = val[0:B, j:j + 256]
            ref[i, B:2 * B, rot(c + j, k + 2, 256)] = val[B:2 * B, j:j + 256]

    def fw_h(p):
        fm = fm_v[...]
        res = []
        for a in (2 * p, 2 * p + 1):
            for c in range(0, D, CW):
                hh = lax.dot_general(fm, hb[p % 2, c:c + CW, (a % 2) * B:(a % 2 + 1) * B], NT_DIMS,
                                     preferred_element_type=f32)
                res.append(hh)
                if a == 0:
                    sd = jnp.concatenate([skt[KS, :, c:c + CW]] * (B // 8), axis=0)
                    hh = jnp.concatenate([hh[0:B] + sd, hh[B:2 * B]], axis=0)
                put(hs[p], a % 2, c, hh, 1)
        return res

    def fw_k(p, zk):
        fm = fm_v[...]
        res = []
        for a in (2 * p, 2 * p + 1):
            for c in range(0, D, CW):
                hh = jnp.dot(fm, kvb[a % 4 + zk, :, c:c + CW], preferred_element_type=f32)
                res.append(hh)
                put(ks[p], a % 2, c, hh, 0)
        return res

    def term_tasks(groups, newp):
        def acc(a, g, first, r, c, z, GW):
            zr = zi = None
            for ap in g:
                d = a - ap
                xr = ks[ap // 2][ap % 2 + z, r:r + RG, c:c + GW]
                xi = ks[ap // 2][ap % 2 + z, B + r:B + r + RG, rot(c, 2, GW)]
                hr = hs[d // 2][d % 2 + z, r:r + RG, rot(c, 1, GW)]
                hi = hs[d // 2][d % 2 + z, B + r:B + r + RG, rot(c, 3, GW)]
                tr = xr * hr - xi * hi
                ti = xr * hi + xi * hr
                zr = tr if zr is None else zr + tr
                zi = ti if zi is None else zi + ti
            if not first:
                zr = zr + zp[a % NZ, r:r + RG, c:c + GW]
                zi = zi + zp[a % NZ, B + r:B + r + RG, c:c + GW]
            return zr, zi

        def part_task(a, g, first, r, c, z):
            zr, zi = acc(a, g, first, r, c, z, GW)
            zp[a % NZ, r:r + RG, c:c + GW] = zr
            zp[a % NZ, B + r:B + r + RG, c:c + GW] = zi

        def fin_task(fin, r, c, z):
            GW = GWF
            if fin[0][0] > 0:
                pr = wold[0, r:r + RG, c:c + GW]
                pi = wold[0, B + r:B + r + RG, c:c + GW]
            for (a, g, first, last) in fin:
                wr, wi = acc(a, g, first, r, c, z, GW)
                if a == 0:
                    zr, zi = wr, wi
                elif r < B // 2:
                    zr, zi = wr + pi, wi - pr
                else:
                    zr, zi = wr - pi, wi + pr
                zb[a % 2, r:r + RG, c:c + GW] = zr.astype(bf16)
                zb[a % 2, B + r:B + r + RG, c:c + GW] = zi.astype(bf16)
                pr, pi = wr, wi
            if fin[-1][0] < NB - 1:
                wold[0, r:r + RG, c:c + GW] = pr
                wold[0, B + r:B + r + RG, c:c + GW] = pi

        def srcs(gs):
            return (set(('k', ap // 2) for (a, g, _, _) in gs for ap in g)
                    | set(('h', (a - ap) // 2) for (a, g, _, _) in gs for ap in g))

        rc = [(r, c) for r in range(0, B, RG) for c in range(0, D, GW)]
        tasks = []
        for grp in groups:
            a, g, first, last = grp
            if not last:
                sr = srcs([grp])
                new = any(i == newp for (_, i) in sr)
                tasks += [(len(g), new, sr, ('zp', a % NZ),
                           functools.partial(part_task, a, g, first, r, c)) for (r, c) in rc]
        tasks.sort(key=lambda x: x[1])
        fin = [x for x in groups if x[3]]
        if fin:
            tasks += [(sum(len(x[1]) for x in fin) + 1, True, srcs(fin), ('zb', 0),
                       functools.partial(fin_task, fin, r, c)) for r in range(0, B, RG) for c in range(0, D, GWF)]
        return tasks

    def split_tasks(tasks, caps):
        total = sum(x[0] for x in tasks)
        out = [[] for _ in caps]
        cum = 0
        for x in tasks:
            pos = (cum + 0.5 * x[0]) / max(total, 1) * sum(caps)
            k = 0
            while k + 1 < len(caps) and pos > sum(caps[:k + 1]):
                k += 1
            out[k].append(x)
            cum += x[0]
        return out

    def run_tasks(tasks, val, z):
        for (kind, i) in sorted(set().union(*[x[2] for x in tasks])) if tasks else []:
            (ks if kind == 'k' else hs)[i][0, 2 * B:2 * B + 8, 0:128] = val
        for x in tasks:
            x[4](z)
        probes = {}
        for x in tasks:
            probes[x[3][0]] = x[3][1]
        return probes

    def probe(probes, z):
        vals = []
        if 'zp' in probes:
            vals.append(zp[probes['zp'] + z, 0:8, 0:128])
        if 'zb' in probes:
            vals.append(zb[z, 0:16, 0:128].astype(f32)[0:8])
        return vals

    def sync(vals):
        v = vals[0]
        for w in vals[1:]:
            v = v + w
        return _lsum(v)

    def inv(p, z):
        im = im_v[...]
        res = []
        for d in range(2):
            for c in range(0, D, CW):
                y = jnp.dot(im, zb[d + z, :, c:c + CW], preferred_element_type=f32)
                res.append(y)
                y_v[p, d * B:(d + 1) * B, c:c + CW] = y
        return res

    R = range(0, TM, LR)

    def corner(acc):
        return acc[acc.shape[0] - 8:, acc.shape[1] - 128:]

    def b16(v):
        return jnp.concatenate([v, v], axis=0).astype(bf16)

    def stat_part(x, i, r, n):
        w = x.shape[1]
        mu = _part(x) * (128.0 / w)
        dv = x - _wide(mu, w)
        ps[i, r:r + n] = mu
        ps[i + 1, r:r + n] = _part(dv * dv)

    def stat_mean(i, j, w, z):
        mu = ps[i + z]
        m = _lsum(mu) * (1.0 / 128)
        st[j] = m
        e = mu - m
        ps[i] = ps[i + 1 + z] + (w / 128.0) * (e * e)

    def stat_rstd(i, j, w, z):
        st[j + 1] = lax.rsqrt(_lsum(ps[i + z]) * (1.0 / w) + EPS)

    def norm(x, j, r, n):
        w = x.shape[1]
        return (x - _wide(st[j, r:r + n], w)) * _wide(st[j + 1, r:r + n], w)

    PG = 4

    def z_dot(xn, n):
        return jnp.dot(xn, win[:, n * TN:(n + 1) * TN], preferred_element_type=f32)

    def kick():
        return jnp.dot(fm_v[0:16, :], fm_v[0:128, :], preferred_element_type=f32)

    def lead(ref, i):
        return ref[i, 0:16, 0:128].astype(f32)[0:8]

    def tile_rows(t, r, n):
        if isinstance(t, int):
            return slice(t * TM // 2 + r, t * TM // 2 + r + n)
        return pl.ds(pl.multiple_of(t * (TM // 2) + r, 8), n)

    def block(items):
        z = [zs[j] for j in range(8)]
        c = dict(sg=None, acc=None, vals=[], xn={}, ng=0)

        def mxu(res):
            if c['sg'] is None:
                c['sg'] = res[0][0:8, 0:128]
            c['acc'] = res[-1]

        def get_xn(i):
            if i not in c['xn']:
                c['xn'][i] = pltpu.bitcast(xn_v[i], bf16)
            return c['xn'][i]

        for it in items:
            kind = it[0]
            sg = c['sg']
            if kind == 'kick':
                mxu([kick()])
            elif kind == 'z1':
                for n in it[3]:
                    acc = z_dot(get_xn(it[2]), n)
                    z1_v[it[1], :, n * TN:(n + 1) * TN] = _gelu(acc).astype(bf16)
                    mxu([acc])
            elif kind == 'z2':
                for n in it[3]:
                    acc = z_dot(get_xn(it[2]), NCH + n)
                    zt[it[1]][0, 0:TM, n * TN:(n + 1) * TN] = _gelu(acc)
                    mxu([acc])
            elif kind == 'inv':
                mxu(inv(it[1], z[1] if it[2] else 0))
            elif kind == 'fwh':
                mxu(fw_h(it[1]))
            elif kind == 'fwk':
                mxu(fw_k(it[1], z[1] if it[2] else 0))
            elif kind == 'g':
                ws = wsp[it[1]]
                bbt = _wide(bb_v[it[1]], TN)
                for n in it[3]:
                    acc = jnp.dot(ws, _h(it[2][:, n * TN:(n + 1) * TN]), preferred_element_type=f32)
                    u = (z1_v[it[1], :, n * TN:(n + 1) * TN].astype(f32) * (acc + bbt)).astype(bf16)
                    u = pltpu.bitcast(u, u32)
                    if n < NCH - 1:
                        ua[0, :, n * TN:(n + 1) * TN] = u
                    else:
                        ub[0] = u
                    mxu([acc])
            elif kind == 'o':
                zu = z[1] if it[3] else 0
                u = _h(jnp.concatenate([ua[zu], ub[zu]], axis=1))
                for n in range(D // TN):
                    acc = jnp.dot(u, wout[:, n * TN:(n + 1) * TN], preferred_element_type=f32)
                    x2 = x_v[it[1], 0:TM, n * TN:(n + 1) * TN] + acc
                    if it[2]:
                        z1_v[it[1], :, n * TN:(n + 1) * TN] = x2.astype(bf16)
                    else:
                        wold[0, 0:TM, n * TN:(n + 1) * TN] = x2
                    mxu([acc])
            elif kind == 'xn':
                x_v[0, TM:TM + 8, 0:128] = sg
                for r in R:
                    xn_v[it[2], r // 2:(r + LR) // 2] = pltpu.bitcast(
                        norm(x_v[it[1] + z[0], r:r + LR], 2, r, LR).astype(bf16), u32)
                if it[3]:
                    c['xn'][it[2]] = pltpu.bitcast(xn_v[it[2] + z[1]], bf16)
                else:
                    c['vals'].append(lead(xn_v, it[2] + z[6]))
            elif kind == 'z2n':
                zt[it[2]][0, TM:TM + 8, 0:128] = sg
                for r in R:
                    it[3][tile_rows(it[1], r // 2, LR // 2), :] = pltpu.bitcast(
                        norm(zt[it[2]][z[0], r:r + LR], 4, r, LR).astype(bf16), u32)
                c['vals'].append(pltpu.bitcast(it[3][tile_rows(it[1] + z[6], 0, 8), 0:128], f32))
            elif kind == 'qstat':
                qb[0, TM:TM + 16, 0:128] = b16(sg)
                for r in R:
                    stat_part(qb[it[1] % 2 + z[0], r:r + LR].astype(f32), 0, r, LR)
            elif kind == 'zstat':
                zt[it[1]][0, TM:TM + 8, 0:128] = sg
                for r in range(0, TM, 8):
                    stat_part(zt[it[1]][z[0], r:r + 8], 2, r, 8)
            elif kind == 'x1':
                if it[2]:
                    qb[0, TM:TM + 16, 0:128] = b16(sg)
                for r in R:
                    x0 = qb[it[1] % 2 + (z[0] if it[2] else 0), r:r + LR].astype(f32)
                    x1 = x0 + norm(x0, 0, r, LR) * y_v[it[1] + (0 if it[2] else z[1]), r:r + LR]
                    x_v[it[1], r:r + LR] = x1
                    stat_part(x1, 0, r, LR)
            elif kind == 'x2stat':
                wold[0, TM:TM + 8, 0:128] = sg
                for r in R:
                    stat_part(wold[z[0], r:r + LR], 0, r, LR)
            elif kind == 'x3':
                wold[0, TM:TM + 8, 0:128] = sg
                for r in R:
                    x0 = wold[z[0], r:r + LR]
                    x1 = x0 + norm(x0, 0, r, LR) * y_v[it[1], r:r + LR]
                    x_v[it[2], r:r + LR] = x1
                    stat_part(x1, 0, r, LR)
            elif kind == 'kvprep':
                kb[0, B:B + 16, 0:128] = b16(sg)
                kvprep(it[1], z[0])
                if not it[2]:
                    c['vals'].append(lead(kvb, (2 * it[1]) % 4 + z[6]))
            elif kind == 'terms':
                c['vals'] += probe(run_tasks(it[1], sg, z[0]), z[6])
            elif kind == 'mean' or kind == 'rstd':
                ps[PG, 8 * c['ng']:8 * c['ng'] + 8] = corner(c['acc'])
                c['ng'] += 1
                for (i, j, w) in it[1]:
                    (stat_mean if kind == 'mean' else stat_rstd)(i, j, w, z[1 + c['ng']])
            elif kind == 'bb':
                bs16 = bspb[...].astype(f32)
                for i in range(S // 128):
                    bb_v[i // 2, (i % 2) * 128:(i % 2 + 1) * 128, :] = jnp.transpose(
                        jnp.broadcast_to(bs16[i:i + 1, :], (128, 128)))
        if c['vals']:
            ps[PG, 32:40] = sync([c['acc'][0:8, 0:128]] + c['vals'])

    def run(name, items, cond=None):
        with jax.named_scope(name):
            pl.when(zs[15] == 0 if cond is None else cond)(lambda: block(items))

    SQ, SX, SZ = (0, 0, D), (0, 2, D), (2, 4, FH)
    ALL = list(range(NCH))

    def block_p0():
        kvprep(0, 0)

    def block_p1():
        fw_k(0, 0)
        fw_h(0)

    def block_p2():
        z = [zs[j] for j in range(4)]
        sg = fw_h(1)[0][0:8, 0:128]
        run_tasks(term_tasks([(0, [0], True, True), (1, [0, 1], True, True)], 0), sg, z[1])
        qb[0, TM:TM + 16, 0:128] = b16(sg)
        for r in R:
            stat_part(qb[z[1], r:r + LR].astype(f32), 0, r, LR)
        stat_mean(0, 0, D, z[2])
        inv(0, z[0])
        stat_rstd(0, 0, D, z[3])

    def block_p3():
        kvprep(1, 0)
        fw_k(1, zs[0])
        for r in R:
            x0 = qb[0, r:r + LR].astype(f32)
            x1 = x0 + norm(x0, 0, r, LR) * y_v[0, r:r + LR]
            x_v[0, r:r + LR] = x1
            xn_v[0, r // 2:(r + LR) // 2] = pltpu.bitcast(_ln(x1).astype(bf16), u32)

    for name, waits, fn, nxt in (
            ('P0', ((0, 0), (1, 0)), block_p0, [pair_copy(3, 0), pair_copy(2, 1)]),
            ('P1', ((2, 0),), block_p1, [pair_copy(0, 1), pair_copy(1, 1)]),
            ('P2', ((3, 0), (2, 1)), block_p2, [w_copy(0)]),
            ('P3', ((0, 1), (1, 1)), block_p3, [pair_copy(3, 1), w_copy(1)])):
        issue(*nxt)
        for (j, p) in waits:
            pair_copy(j, p).wait()
        with jax.named_scope(name):
            pl.when(zs[15] == 0)(fn)

    for t in range(NT):
        conv = t < NT - 1
        ta = term_tasks(plan[('A', t)], -1) if conv else []
        tb = term_tasks(plan[('B', t)], -1) if conv else []
        if t == 0:
            ch = split_tasks(ta, [3, 1.5, 2])
            issue(w_copy(2))
            w_copy(0).wait()
            run('A0a', [('kick',), ('terms', ch[0]), ('z2', 0, 0, [0, 1, 2])])
            issue(pair_copy(0, 2), pair_copy(1, 2), pair_copy(2, 2))
            pair_copy(3, 1).wait()
            w_copy(1).wait()
            run('A0b', [('kick',), ('qstat', 1), ('terms', ch[1]), ('z2', 0, 0, [3]), ('mean', [SQ]),
                        ('z2', 0, 0, [4])])
            issue(w_copy(3))
            w_copy(2).wait()
            run('A0c', [('kick',), ('rstd', [SQ]), ('terms', ch[2]), ('z2', 0, 0, [5, 6])])
            issue(w_copy(4))
            for j in range(3):
                pair_copy(j, 2).wait()
            run('B0a', [('inv', 1, 0), ('kvprep', 2, 1), ('fwh', 2), ('fwk', 2, 1)])
            issue(w_copy(5), pair_copy(3, 2), pair_copy(0, 3), pair_copy(1, 3))
            w_copy(3).wait()
            run('B0b', [('kick',), ('zstat', 0), ('x1', 1, 1), ('z1', 0, 0, [0, 1]), ('mean', [SX, SZ]),
                        ('z1', 0, 0, [2])])
            w_copy(4).wait()
            run('B0c', [('kick',), ('rstd', [SX, SZ]), ('terms', tb), ('bb',), ('z1', 0, 0, [3, 4, 5])])
            w_copy(5).wait()
            continue
        if t + 2 < NT:
            pair_copy(2, t + 2).start()
            pair_copy(3, t + 2).start()
        if t + 3 < NT:
            pair_copy(0, t + 3).start()
            pair_copy(1, t + 3).start()
        if t == 1:
            issue(big[0])
        if t == 3:
            issue(big[1])
        if conv:
            pair_copy(3, t + 1).wait()
        if t + 2 < NT:
            pair_copy(0, t + 2).wait()
            pair_copy(1, t + 2).wait()
        s0, s1 = t % 2, (t - 1) % 2
        items = [('z1', t - 1, s1, [NCH - 1]), ('xn', t, s0, 1), ('z2n', t - 1, s1, z2a)]
        if conv:
            items += [('qstat', t + 1)]
            if t + 2 < NT:
                items += [('kvprep', t + 2, 0)]
            items += [('terms', ta), ('z2', s0, s0, ALL[:4]), ('mean', [SQ]), ('z2', s0, s0, ALL[4:5]),
                      ('rstd', [SQ]), ('z2', s0, s0, ALL[5:])]
        else:
            items += [('z2', s0, s0, ALL)]
        run('A%d' % t, items)
        if t + 2 < NT:
            pair_copy(2, t + 2).wait()
        if conv:
            items = [('inv', t + 1, 0), ('zstat', s0), ('x1', t + 1, 0), ('terms', tb)]
            if t + 2 < NT:
                items += [('fwh', t + 2), ('fwk', t + 2, 0)]
            items += [('z1', t, s0, ALL[:3]), ('mean', [SX, SZ]), ('z1', t, s0, ALL[3:4]), ('rstd', [SX, SZ]),
                      ('z1', t, s0, ALL[4:6])]
            run('B%d' % t, items)
        else:
            run('B7a', [('kick',), ('zstat', s0), ('z1', t, s0, [0]), ('mean', [SZ]), ('z1', t, s0, [1]),
                        ('rstd', [SZ]), ('z1', t, s0, [2])])
            run('B7b', [('kick',), ('z2n', t, s0, z2a), ('z1', t, s0, [3])])

    big[0].wait()
    big[1].wait()

    def stage_c(i, carry):
        t = i - 1
        tc = jnp.maximum(t, 0)
        run('K1', [('g', i, z2a, ALL[:1]), ('x3', tc, jnp.where(t < 0, NT, t)),
                   ('z2n', jnp.maximum(t - 1, 0), 0, z2b), ('g', i, z2a, ALL[1:3]), ('mean', [SX]),
                   ('g', i, z2a, ALL[3:4]), ('rstd', [SX]), ('g', i, z2a, ALL[4:])])
        run('K2h', [('o', 0, 0, 0)], t < 0)
        run('K3h', [('kick',), ('x2stat',), ('z1', NT - 1, 1, [4]), ('mean', [SQ]), ('z1', NT - 1, 1, [5]),
                    ('rstd', [SQ]), ('z1', NT - 1, 1, [6])], t < 0)
        run('K2', [('kick',), ('xn', tc, 0, 1), ('o', i, 0, 0), ('z2', 0, 0, ALL)], t >= 0)
        run('K3', [('kick',), ('x2stat',), ('zstat', 0), ('z1', tc, 0, ALL[:3]), ('mean', [SQ, SZ]),
                   ('z1', tc, 0, ALL[3:4]), ('rstd', [SQ, SZ]), ('z1', tc, 0, ALL[4:])],
            jnp.logical_and(t >= 0, t < NT - 2))
        return carry

    def stage_d(t, carry):
        run('D', [('g', t, z2b, ALL), ('o', t, 1, 1)])
        out_copy(t).start()
        return carry

    def out_copy(t):
        return pltpu.make_async_copy(z1_v.at[t, :, pl.ds(0, D)], o_hbm.at[t], sem_o.at[t])

    lax.fori_loop(0, NT, stage_c, 0)
    t = NT - 2
    run('T1', [('kick',), ('x2stat',), ('zstat', 0), ('z1', t, 0, [0]), ('mean', [SQ, SZ]), ('z1', t, 0, [1]),
               ('rstd', [SQ, SZ]), ('z1', t, 0, [2])])
    run('T2', [('kick',), ('x3', t + 1, t + 1), ('z2n', t, 0, z2b), ('z1', t, 0, [3]), ('mean', [SX]),
               ('z1', t, 0, [4]), ('rstd', [SX]), ('z1', t, 0, [5])])
    run('T3', [('z1', t, 0, [6]), ('xn', t + 1, 1, 1), ('z2', 0, 1, ALL)])
    t = NT - 1
    run('T4', [('kick',), ('zstat', 0), ('z1', t, 1, ALL[:2]), ('mean', [SZ]), ('z1', t, 1, [2]),
               ('rstd', [SZ]), ('z1', t, 1, [3, 4])])
    run('T5', [('kick',), ('z2n', t, 0, z2b), ('z1', t, 1, [5, 6])])
    lax.fori_loop(0, NT, stage_d, 0)
    for t in range(NT):
        out_copy(t).wait()


@jax.jit
def pallas_interleave_layers__ssm_conv_h3__mixer_gmlp__prompt_kernel(
        A_q, A_k, A_v, A_shift_k, A_ssm_k, A_ssm_D, B_x, B_w_in, B_w_sp, B_b_sp, B_w_out):
    del B_x
    any_spec = pl.BlockSpec(memory_space=pl.ANY)
    scratch = [
        pltpu.VMEM((2, TM + 16, D), bf16),
        pltpu.VMEM((8, B + 16, D), bf16),
        pltpu.VMEM((8, B, D), bf16),
        pltpu.VMEM((2, D, TM), bf16),
        pltpu.VMEM((D, F), bf16),
        pltpu.VMEM((NT, TM, S), bf16),
        pltpu.VMEM((FH, D), bf16),
        pltpu.VMEM((KS, D), bf16),
        pltpu.VMEM((8, 128), bf16),
        pltpu.VMEM((16, 128), bf16),
        pltpu.VMEM((NT + 1, TM + 8, D), f32),
        pltpu.VMEM((NT, TM, D), f32),
        pltpu.VMEM((NT, TM, FH), bf16),
        pltpu.VMEM((S // 2, FH), u32),
        pltpu.VMEM((S // 2, FH), u32),
        pltpu.VMEM((NT, TM, 128), f32),
        pltpu.VMEM((KS + 1, 8, D), f32),
        pltpu.VMEM((2 * B, B), bf16),
        pltpu.VMEM((B, 2 * B), bf16),
        pltpu.VMEM((4, B, D), bf16),
        [pltpu.VMEM((2, 2 * B + 8, D), f32)] * NT,
        [pltpu.VMEM((2, 2 * B + 8, D), f32)] * NT,
        pltpu.VMEM((1, TM + 8, D), f32),
        pltpu.VMEM((NZ, 2 * B, D), f32),
        pltpu.VMEM((2, 2 * B, D), bf16),
        pltpu.VMEM((2, TM // 2, D), u32),
        [pltpu.VMEM((1, TM + 8, FH), f32)] * 2,
        pltpu.VMEM((5, TM, 128), f32),
        pltpu.VMEM((6, TM, 128), f32),
        pltpu.VMEM((1, TM // 2, FH - TN), u32),
        pltpu.VMEM((1, TM // 2, TN), u32),
        pltpu.SMEM((16,), jnp.int32),
        pltpu.SemaphoreType.DMA((4 * NT,)),
        pltpu.SemaphoreType.DMA((6,)),
        pltpu.SemaphoreType.DMA((5,)),
        pltpu.SemaphoreType.DMA((NT,)),
    ]
    out = pl.pallas_call(
        _kernel,
        out_shape=jax.ShapeDtypeStruct((NT, TM, D), bf16),
        in_specs=[any_spec] * 10,
        out_specs=any_spec,
        scratch_shapes=scratch,
        compiler_params=pltpu.CompilerParams(vmem_limit_bytes=127 * 1024 * 1024),
    )(A_q.reshape(NT, TM, D), A_k.reshape(NB, B, D), A_v.reshape(NB, B, D), A_shift_k.T, A_ssm_k,
      A_ssm_D.reshape(8, 128), B_w_in, B_w_sp.reshape(NT, TM, S), B_b_sp.reshape(16, 128), B_w_out)
    return out.reshape(1, S, D)
```

```python
import functools
import math
import jax
import jax.numpy as jnp
from jax import lax
import jax.experimental.pallas as pl
import jax.experimental.pallas.tpu as pltpu

S = 2048
D = 1024
F = 3584
FH = F // 2
KS = 4
B = 128
NB = S // B
EPS = 1e-5
f32 = jnp.float32
bf16 = jnp.bfloat16
u32 = jnp.uint32

TM = 256
NT = S // TM
TN = 256
NCH = FH // TN
RG = 16
GW = 256
LR = 16
NZ = 8
CAP_A = 9
CAP_B = 14
GWF = 128
OS = 3
ROT = 256


def _plan(cap_a, cap_b):
    done = set((a, ap) for a in (0, 1) for ap in range(a + 1))
    blocks = {}
    for t in range(NT - 1):
        for kind, cap in (('A', cap_a), ('B', cap_b)):
            sel = {}
            n = 0
            lo = 2 * t + 2 if kind == 'A' else 2 * t + 4
            lim = 2 * t + 3
            for a in range(lo, NB):
                g = [ap for ap in range(a + 1) if (a, ap) not in done and ap <= lim and a - ap <= lim]
                if a > lim:
                    g = g[:max(cap - n, 0)]
                if g:
                    sel[a] = g
                    n += len(g)
            groups = []
            for a in sorted(sel):
                first = not any((a, x) in done for x in range(a + 1))
                done.update((a, x) for x in sel[a])
                last = all((a, x) in done for x in range(a + 1))
                assert a < lo + NZ and last == (a <= 2 * t + 3)
                groups.append((a, sel[a], first, last))
            blocks[(kind, t)] = groups
    assert len(done) == NB * (NB + 1) // 2
    return blocks


def _gelu(x):
    u = x * (0.7978845608028654 + 0.035677408136300125 * (x * x))
    h = 0.5 * x
    return h + h * jnp.tanh(u)


def _h(v):
    return pltpu.bitcast(v, bf16)


def _part(v):
    acc = v[:, 0:128]
    for c in range(128, v.shape[1], 128):
        acc = acc + v[:, c:c + 128]
    return acc


def _lsum(acc):
    return jnp.broadcast_to(jnp.sum(acc, axis=1, keepdims=True), acc.shape)


def _wide(v, n):
    return jnp.concatenate([v] * (n // 128), axis=1)


def _ln(x):
    n = x.shape[-1]
    m = jnp.sum(x, axis=-1, keepdims=True) * (1.0 / n)
    xc = x - m
    v = jnp.sum(xc * xc, axis=-1, keepdims=True) * (1.0 / n)
    return xc * lax.rsqrt(v + EPS)


def _dft_rows(shape, row_dim):
    r = lax.broadcasted_iota(jnp.int32, shape, row_dim)
    n = lax.broadcasted_iota(jnp.int32, shape, 1 - row_dim)
    is_im = r >= B
    rr = jnp.where(is_im, r - B, r)
    odd = rr >= B // 2
    fidx = jnp.where(odd, 2 * (rr - B // 2) + 1, 2 * rr)
    m = (2 * fidx + 1) * n - jnp.where(is_im, B, 0)
    m = jnp.bitwise_and(m, 4 * B - 1)
    m = jnp.where(m > 2 * B, 4 * B - m, m)
    return jnp.cos(m.astype(f32) * (math.pi / (2 * B)))


NT_DIMS = (((1,), (1,)), ((), ()))


def _kernel(q_hbm, k_hbm, v_hbm, sk_hbm, h_hbm, sd_hbm, win_hbm, wsp_hbm, bsp_hbm, wout_hbm,
            o_hbm,
            qb, kb, vb, hb, win, wsp, wout, skb, sdb, bspb,
            x_v, y_v, z1_v, z2a, z2b, bb_v, skt, fm_v, im_v, kvb, ks, hs, wold, zp, zb,
            xn_v, zt, zc, xa, ps, st, ua, ub, zs,
            sem_c, sem_w, sem_s, sem_o):
    plan = _plan(CAP_A, CAP_B)

    def pair_copy(j, p):
        if j == 0:
            return pltpu.make_async_copy(k_hbm.at[pl.ds(2 * p, 2)], kb.at[pl.ds(2 * p % 8, 2), pl.ds(0, B)], sem_c.at[p % 2])
        if j == 1:
            return pltpu.make_async_copy(v_hbm.at[pl.ds(2 * p, 2)], vb.at[pl.ds(2 * p % 8, 2)], sem_c.at[2 + p % 2])
        if j == 2:
            cols = pl.ds(p * TM, TM)
            return pltpu.make_async_copy(h_hbm.at[:, cols], hb.at[p % 2], sem_c.at[4 + p % 2])
        return pltpu.make_async_copy(q_hbm.at[p], qb.at[p % 2, pl.ds(0, TM)], sem_c.at[6 + p % 2])

    WG = ((7, 10), (10, 12), (12, 14), (0, 3), (3, 6), (6, 7))

    def w_copy(i):
        cols = pl.ds(WG[i][0] * TN, (WG[i][1] - WG[i][0]) * TN)
        return pltpu.make_async_copy(win_hbm.at[:, cols], win.at[:, cols], sem_w.at[i % 3])

    def out_copy(t, j):
        cols = pl.ds(0, OS * TN) if j == 0 else pl.ds(OS * TN, D - OS * TN)
        return pltpu.make_async_copy(z1_v.at[t, :, cols], o_hbm.at[t, :, cols], sem_o.at[2 * (t % 2) + j])

    def issue(*copies):
        for cp in copies:
            cp.start(priority=1)

    def issue_big(j):
        if j >= 2:
            big[j - 2].wait()
        issue(big[j])

    small = [
        pltpu.make_async_copy(sk_hbm, skb, sem_o.at[0]),
        pltpu.make_async_copy(sd_hbm, sdb, sem_o.at[1]),
        pltpu.make_async_copy(bsp_hbm, bspb, sem_o.at[2]),
    ]
    WR = FH // 4
    big = ([pltpu.make_async_copy(wsp_hbm.at[j], wsp.at[j], sem_s.at[j % 2]) for j in range(NT)]
           + [pltpu.make_async_copy(wout_hbm.at[pl.ds(j * WR, WR)], wout.at[pl.ds(j * WR, WR)], sem_s.at[j % 2])
              for j in range(4)])
    for cp in small:
        cp.start()
    pair_copy(0, 0).start(priority=1)
    pair_copy(1, 0).start(priority=1)

    def zinit(i, c):
        zs[i] = 0
        return c
    lax.fori_loop(0, 16, zinit, 0)
    issue(pair_copy(2, 0))

    fm_v[...] = _dft_rows((2 * B, B), 0).astype(bf16)
    im_v[...] = (_dft_rows((B, 2 * B), 1) * (1.0 / B)).astype(bf16)

    for cp in small:
        cp.wait()
    sk4 = skb[...].astype(f32)
    for j in range(KS):
        skt[j] = jnp.broadcast_to(sk4[j:j + 1, :], (8, D))
    sd8 = sdb[...].astype(f32)
    skt[KS] = jnp.concatenate([jnp.broadcast_to(sd8[i:i + 1, :], (8, 128)) for i in range(8)], axis=1)

    def kvprep(p, z):
        for a in (2 * p, 2 * p + 1):
            for c in range(0, D, GW):
                for r0 in range(0, B, 32):
                    kcur = kb[a % 8 + z, r0:r0 + 32, c:c + GW].astype(f32)
                    if a == 0 and r0 == 0:
                        kprev = jnp.zeros((8, GW), f32)
                    elif r0 == 0:
                        kprev = kb[(a - 1) % 8 + z, B - 16:B, c:c + GW].astype(f32)[8:16]
                    else:
                        kprev = kb[a % 8 + z, r0 - 16:r0, c:c + GW].astype(f32)[8:16]
                    ext = jnp.concatenate([kprev, kcur], axis=0)
                    sk = [jnp.concatenate([skt[j, :, c:c + GW]] * 4, axis=0) for j in range(KS)]
                    acc = kcur * sk[0]
                    for j in range(1, KS):
                        acc = acc + pltpu.roll(ext, j, 0)[8:] * sk[j]
                    kvb[a % 4, r0:r0 + 32, c:c + GW] = (acc * vb[a % 8, r0:r0 + 32, c:c + GW].astype(f32)).astype(bf16)

    CW = 512

    def rot(c, k, w):
        c = (c + ROT * k) % D
        return slice(c, c + w)

    def put(ref, i, c, val, k):
        for j in range(0, CW, 256):
            ref[i, 0:B, rot(c + j, k, 256)] = val[0:B, j:j + 256]
            ref[i, B:2 * B, rot(c + j, k + 2, 256)] = val[B:2 * B, j:j + 256]

    def fw_h(p):
        fm = fm_v[...]
        res = []
        for a in (2 * p, 2 * p + 1):
            for c in range(0, D, CW):
                hh = lax.dot_general(fm, hb[p % 2, c:c + CW, (a % 2) * B:(a % 2 + 1) * B], NT_DIMS,
                                     preferred_element_type=f32)
                res.append(hh)
                if a == 0:
                    sd = jnp.concatenate([skt[KS, :, c:c + CW]] * (B // 8), axis=0)
                    hh = jnp.concatenate([hh[0:B] + sd, hh[B:2 * B]], axis=0)
                put(hs[p], a % 2, c, hh, 1)
        return res

    def fw_k(p, zk):
        fm = fm_v[...]
        res = []
        for a in (2 * p, 2 * p + 1):
            for c in range(0, D, CW):
                hh = jnp.dot(fm, kvb[a % 4 + zk, :, c:c + CW], preferred_element_type=f32)
                res.append(hh)
                put(ks[p], a % 2, c, hh, 0)
        return res

    def term_tasks(groups, newp):
        def acc(a, g, first, r, c, z, GW):
            zr = zi = None
            for ap in g:
                d = a - ap
                xr = ks[ap // 2][ap % 2 + z, r:r + RG, c:c + GW]
                xi = ks[ap // 2][ap % 2 + z, B + r:B + r + RG, rot(c, 2, GW)]
                hr = hs[d // 2][d % 2 + z, r:r + RG, rot(c, 1, GW)]
                hi = hs[d // 2][d % 2 + z, B + r:B + r + RG, rot(c, 3, GW)]
                tr = xr * hr - xi * hi
                ti = xr * hi + xi * hr
                zr = tr if zr is None else zr + tr
                zi = ti if zi is None else zi + ti
            if not first:
                zr = zr + zp[a % NZ, r:r + RG, c:c + GW]
                zi = zi + zp[a % NZ, B + r:B + r + RG, c:c + GW]
            return zr, zi

        def part_task(a, g, first, r, c, z):
            zr, zi = acc(a, g, first, r, c, z, GW)
            zp[a % NZ, r:r + RG, c:c + GW] = zr
            zp[a % NZ, B + r:B + r + RG, c:c + GW] = zi

        def fin_task(fin, r, c, z):
            GW = GWF
            if fin[0][0] > 0:
                pr = wold[0, r:r + RG, c:c + GW]
                pi = wold[0, B + r:B + r + RG, c:c + GW]
            for (a, g, first, last) in fin:
                wr, wi = acc(a, g, first, r, c, z, GW)
                if a == 0:
                    zr, zi = wr, wi
                elif r < B // 2:
                    zr, zi = wr + pi, wi - pr
                else:
                    zr, zi = wr - pi, wi + pr
                zb[a % 2, r:r + RG, c:c + GW] = zr.astype(bf16)
                zb[a % 2, B + r:B + r + RG, c:c + GW] = zi.astype(bf16)
                pr, pi = wr, wi
            if fin[-1][0] < NB - 1:
                wold[0, r:r + RG, c:c + GW] = pr
                wold[0, B + r:B + r + RG, c:c + GW] = pi

        def srcs(gs):
            return (set(('k', ap // 2) for (a, g, _, _) in gs for ap in g)
                    | set(('h', (a - ap) // 2) for (a, g, _, _) in gs for ap in g))

        rc = [(r, c) for r in range(0, B, RG) for c in range(0, D, GW)]
        tasks = []
        for grp in groups:
            a, g, first, last = grp
            if not last:
                sr = srcs([grp])
                new = any(i == newp for (_, i) in sr)
                tasks += [(len(g), new, sr, ('zp', a % NZ),
                           functools.partial(part_task, a, g, first, r, c)) for (r, c) in rc]
        tasks.sort(key=lambda x: x[1])
        fin = [x for x in groups if x[3]]
        if fin:
            tasks += [(sum(len(x[1]) for x in fin) + 1, True, srcs(fin), ('zb', 0),
                       functools.partial(fin_task, fin, r, c)) for r in range(0, B, RG) for c in range(0, D, GWF)]
        return tasks

    def split_tasks(tasks, caps):
        total = sum(x[0] for x in tasks)
        out = [[] for _ in caps]
        cum = 0
        for x in tasks:
            pos = (cum + 0.5 * x[0]) / max(total, 1) * sum(caps)
            k = 0
            while k + 1 < len(caps) and pos > sum(caps[:k + 1]):
                k += 1
            out[k].append(x)
            cum += x[0]
        return out

    def run_tasks(tasks, val, z):
        for (kind, i) in sorted(set().union(*[x[2] for x in tasks])) if tasks else []:
            (ks if kind == 'k' else hs)[i][0, 2 * B:2 * B + 8, 0:128] = val
        for x in tasks:
            x[4](z)
        probes = {}
        for x in tasks:
            probes[x[3][0]] = x[3][1]
        return probes

    def probe(probes, z):
        vals = []
        if 'zp' in probes:
            vals.append(zp[probes['zp'] + z, 0:8, 0:128])
        if 'zb' in probes:
            vals.append(zb[z, 0:16, 0:128].astype(f32)[0:8])
        return vals

    def sync(vals):
        v = vals[0]
        for w in vals[1:]:
            v = v + w
        return _lsum(v)

    def inv(p, z):
        im = im_v[...]
        res = []
        for d in range(2):
            for c in range(0, D, CW):
                y = jnp.dot(im, zb[d + z, :, c:c + CW], preferred_element_type=f32)
                res.append(y)
                y_v[p, d * B:(d + 1) * B, c:c + CW] = y
        return res

    R = range(0, TM, LR)

    def corner(acc):
        return acc[acc.shape[0] - 8:, acc.shape[1] - 128:]

    def b16(v):
        return jnp.concatenate([v, v], axis=0).astype(bf16)

    def stat_part(x, i, r, n):
        w = x.shape[1]
        mu = _part(x) * (128.0 / w)
        dv = x - _wide(mu, w)
        ps[i, r:r + n] = mu
        ps[i + 1, r:r + n] = _part(dv * dv)

    def stat_mean(i, j, w, z):
        mu = ps[i + z]
        m = _lsum(mu) * (1.0 / 128)
        st[j] = m
        e = mu - m
        ps[i] = ps[i + 1 + z] + (w / 128.0) * (e * e)

    def stat_rstd(i, j, w, z):
        st[j + 1] = lax.rsqrt(_lsum(ps[i + z]) * (1.0 / w) + EPS)

    def norm(x, j, r, n):
        w = x.shape[1]
        return (x - _wide(st[j, r:r + n], w)) * _wide(st[j + 1, r:r + n], w)

    PG = 6

    def z_dot(xn, n):
        return jnp.dot(xn, win[:, n * TN:(n + 1) * TN], preferred_element_type=f32)

    def kick():
        return jnp.dot(fm_v[0:16, :], fm_v[0:128, :], preferred_element_type=f32)

    def lead(ref, i):
        return ref[i, 0:16, 0:128].astype(f32)[0:8]

    def tile_rows(t, r, n):
        if isinstance(t, int):
            return slice(t * TM // 2 + r, t * TM // 2 + r + n)
        return pl.ds(pl.multiple_of(t * (TM // 2) + r, 8), n)

    def block(items):
        z = [zs[j] for j in range(8)]
        c = dict(sg=None, acc=None, vals=[], xn={}, ng=0, rel=[])

        def release(ref):
            if not any(ref is x for x in c['rel']):
                c['rel'].append(ref)
                ref[0, TM:TM + 8, 0:128] = c['sg']

        def mxu(res):
            if c['sg'] is None:
                c['sg'] = res[0][0:8, 0:128]
            c['acc'] = res[-1]

        def get_xn(i):
            if id(i) not in c['xn']:
                c['xn'][id(i)] = pltpu.bitcast(xn_v[i], bf16)
            return c['xn'][id(i)]

        for it in items:
            kind = it[0]
            sg = c['sg']
            if kind == 'kick':
                mxu([kick()])
            elif kind == 'z1':
                for n in it[3]:
                    acc = z_dot(get_xn(it[2]), n)
                    z1_v[it[1], :, n * TN:(n + 1) * TN] = _gelu(acc).astype(bf16)
                    mxu([acc])
            elif kind == 'z2':
                for n in it[3]:
                    acc = z_dot(get_xn(it[2]), NCH + n)
                    it[1][0][it[1][1], 0:TM, n * TN:(n + 1) * TN] = _gelu(acc)
                    mxu([acc])
            elif kind == 'inv':
                mxu(inv(it[1], z[1] if it[2] else 0))
            elif kind == 'fwh':
                mxu(fw_h(it[1]))
            elif kind == 'fwk':
                mxu(fw_k(it[1], z[1] if it[2] else 0))
            elif kind == 'g':
                ws = wsp[it[1]]
                bbt = _wide(bb_v[it[1]], TN)
                for n in it[3]:
                    acc = jnp.dot(ws, _h(it[2][:, n * TN:(n + 1) * TN]), preferred_element_type=f32)
                    u = (z1_v[it[1], :, n * TN:(n + 1) * TN].astype(f32) * (acc + bbt)).astype(bf16)
                    u = pltpu.bitcast(u, u32)
                    if n < NCH - 1:
                        ua[0, :, n * TN:(n + 1) * TN] = u
                    else:
                        ub[0] = u
                    mxu([acc])
            elif kind == 'o':
                u = _h(jnp.concatenate([ua[z[1]], ub[z[1]]], axis=1))
                for n in range(D // TN):
                    acc = jnp.dot(u, wout[:, n * TN:(n + 1) * TN], preferred_element_type=f32)
                    x2 = (zp if it[2] is None else x_v)[it[1], 0:TM, n * TN:(n + 1) * TN] + acc
                    if it[2] is None:
                        z1_v[it[1], :, n * TN:(n + 1) * TN] = x2.astype(bf16)
                        if n == OS - 1:
                            out_copy(it[1], 0).start()
                    else:
                        xa[it[2], 0:TM, n * TN:(n + 1) * TN] = x2
                    mxu([acc])
            elif kind == 'xn':
                release(it[1])
                for r in R:
                    xn_v[it[3], r // 2:(r + LR) // 2] = pltpu.bitcast(
                        norm(it[1][it[2] + z[0], r:r + LR], 2, r, LR).astype(bf16), u32)
                c['xn'][id(it[3])] = pltpu.bitcast(xn_v[it[3] + z[1]], bf16)
                if it[4]:
                    c['vals'].append(pltpu.bitcast(xn_v[it[3] + z[6], 0:8, 0:128], f32))
            elif kind == 'z2n':
                release(it[2][0])
                for r in R:
                    it[3][tile_rows(it[1], r // 2, LR // 2), :] = pltpu.bitcast(
                        norm(it[2][0][it[2][1] + z[0], r:r + LR], it[4], r, LR).astype(bf16), u32)
                c['vals'].append(pltpu.bitcast(it[3][tile_rows(it[1] + z[6], 0, 8), 0:128], f32))
            elif kind == 'qstat':
                qb[0, TM:TM + 16, 0:128] = b16(sg)
                for r in R:
                    stat_part(qb[it[1] % 2 + z[0], r:r + LR].astype(f32), 0, r, LR)
            elif kind == 'zstat':
                release(it[1][0])
                for r in range(0, TM, 8):
                    stat_part(it[1][0][it[1][1] + z[0], r:r + 8], 2, r, 8)
            elif kind == 'x1':
                if it[2]:
                    qb[0, TM:TM + 16, 0:128] = b16(sg)
                for r in R:
                    x0 = qb[it[1] % 2 + (z[0] if it[2] else 0), r:r + LR].astype(f32)
                    x1 = x0 + norm(x0, 0, r, LR) * y_v[it[1] + (0 if it[2] else z[1]), r:r + LR]
                    x_v[it[1], r:r + LR] = x1
                    stat_part(x1, 0, r, LR)
            elif kind == 'x2stat':
                release(xa)
                for r in R:
                    stat_part(xa[it[1] + z[0], r:r + LR], 4, r, LR)
            elif kind == 'x3':
                release(xa)
                for r in R:
                    x0 = xa[it[2] + z[0], r:r + LR]
                    x1 = x0 + norm(x0, 0, r, LR) * y_v[it[1], r:r + LR]
                    zp[it[1], r:r + LR] = x1
                    stat_part(x1, 0, r, LR)
            elif kind == 'kvprep':
                kb[0, B:B + 16, 0:128] = b16(sg)
                kvprep(it[1], z[0])
                if not it[2]:
                    c['vals'].append(lead(kvb, (2 * it[1]) % 4 + z[6]))
            elif kind == 'terms':
                c['vals'] += probe(run_tasks(it[1], sg, z[0]), z[6])
            elif kind == 'mean' or kind == 'rstd':
                gate = corner(c['acc'])
                if len(it) > 2:
                    for v in c['vals']:
                        gate = gate + v
                    c['vals'] = []
                ps[PG, 8 * c['ng']:8 * c['ng'] + 8] = gate
                c['ng'] += 1
                for (i, j, w) in it[1]:
                    (stat_mean if kind == 'mean' else stat_rstd)(i, j, w, z[1 + c['ng']])
            elif kind == 'bb':
                bs16 = bspb[...].astype(f32)
                for i in range(S // 128):
                    bb_v[i // 2, (i % 2) * 128:(i % 2 + 1) * 128, :] = jnp.transpose(
                        jnp.broadcast_to(bs16[i:i + 1, :], (128, 128)))
        if c['vals']:
            ps[PG, 32:40] = sync([c['acc'][0:8, 0:128]] + c['vals'])

    def run(name, items, cond=None):
        with jax.named_scope(name):
            pl.when(zs[15] == 0 if cond is None else cond)(lambda: block(items))

    SQ, SX, SZ, S2, SL = (0, 0, D), (0, 2, D), (2, 4, FH), (4, 0, D), (2, 6, FH)
    Z0 = (zt[0], 0)
    ALL = list(range(NCH))

    def block_p0():
        kvprep(0, 0)

    def block_p1():
        fw_k(0, 0)
        fw_h(0)

    def block_p2():
        z = [zs[j] for j in range(4)]
        sg = fw_h(1)[0][0:8, 0:128]
        run_tasks(term_tasks([(0, [0], True, True), (1, [0, 1], True, True)], 0), sg, z[1])
        qb[0, TM:TM + 16, 0:128] = b16(sg)
        for r in R:
            stat_part(qb[z[1], r:r + LR].astype(f32), 0, r, LR)
        stat_mean(0, 0, D, z[2])
        inv(0, z[0])
        stat_rstd(0, 0, D, z[3])

    def block_p3():
        kvprep(1, 0)
        fw_k(1, zs[0])
        for r in R:
            x0 = qb[0, r:r + LR].astype(f32)
            x1 = x0 + norm(x0, 0, r, LR) * y_v[0, r:r + LR]
            x_v[0, r:r + LR] = x1
            xn_v[0, r // 2:(r + LR) // 2] = pltpu.bitcast(_ln(x1).astype(bf16), u32)

    for name, waits, fn, nxt in (
            ('P0', ((0, 0), (1, 0)), block_p0, [pair_copy(3, 0), pair_copy(2, 1)]),
            ('P1', ((2, 0),), block_p1, [pair_copy(0, 1), pair_copy(1, 1)]),
            ('P2', ((3, 0), (2, 1)), block_p2, [w_copy(0)]),
            ('P3', ((0, 1), (1, 1)), block_p3, [pair_copy(3, 1), w_copy(1)])):
        issue(*nxt)
        for (j, p) in waits:
            pair_copy(j, p).wait()
        with jax.named_scope(name):
            pl.when(zs[15] == 0)(fn)

    for t in range(NT):
        conv = t < NT - 1
        ta = term_tasks(plan[('A', t)], -1) if conv else []
        tb = term_tasks(plan[('B', t)], -1) if conv else []
        if t == 0:
            ch = split_tasks(ta, [3, 1.5, 2])
            issue(w_copy(2))
            w_copy(0).wait()
            run('A0a', [('kick',), ('terms', ch[0]), ('z2', Z0, 0, [0, 1, 2])])
            issue(pair_copy(0, 2), pair_copy(1, 2), pair_copy(2, 2))
            pair_copy(3, 1).wait()
            w_copy(1).wait()
            run('A0b', [('kick',), ('qstat', 1), ('terms', ch[1]), ('z2', Z0, 0, [3]), ('mean', [SQ]),
                        ('z2', Z0, 0, [4])])
            issue(w_copy(3))
            w_copy(2).wait()
            run('A0c', [('kick',), ('rstd', [SQ]), ('terms', ch[2]), ('z2', Z0, 0, [5, 6])])
            issue(w_copy(4))
            for j in range(3):
                pair_copy(j, 2).wait()
            run('B0a', [('inv', 1, 0), ('kvprep', 2, 1), ('fwh', 2), ('fwk', 2, 1)])
            issue(w_copy(5), pair_copy(3, 2), pair_copy(0, 3), pair_copy(1, 3))
            w_copy(3).wait()
            run('B0b', [('kick',), ('zstat', Z0), ('x1', 1, 1), ('z1', 0, 0, [0, 1]), ('mean', [SX, SZ]),
                        ('z1', 0, 0, [2])])
            w_copy(4).wait()
            run('B0c', [('kick',), ('rstd', [SX, SZ]), ('terms', tb), ('bb',), ('z1', 0, 0, [3, 4, 5])])
            w_copy(5).wait()
            continue
        if t + 2 < NT:
            issue(pair_copy(2, t + 2), pair_copy(3, t + 2))
        if t + 3 < NT:
            issue(pair_copy(0, t + 3), pair_copy(1, t + 3))
        if t > 1:
            issue_big(2 * t - 3)
        if conv:
            pair_copy(3, t + 1).wait()
        if t + 2 < NT and t > 1:
            pair_copy(0, t + 2).wait()
            pair_copy(1, t + 2).wait()
        s0, s1 = t % 2, (t - 1) % 2
        za, zo = (zt[s0], 0), (zt[s1], 0)
        items = [('z1', t - 1, s1, [NCH - 1 if conv else NCH - 2]), ('xn', x_v, t, s0, 0), ('z2n', t - 1, zo, z2a, 4)]
        if conv:
            items += [('qstat', t + 1)]
            if t + 2 < NT and t > 1:
                items += [('kvprep', t + 2, 0)]
            items += [('terms', ta), ('z2', za, s0, ALL[:4]), ('mean', [SQ]), ('z2', za, s0, ALL[4:5]),
                      ('rstd', [SQ]), ('z2', za, s0, ALL[5:])]
        else:
            items += [('z2', za, s0, ALL)]
        run('A%d' % t, items)
        if conv:
            issue_big(2 * t - 2)
        if t == 1:
            pair_copy(0, t + 2).wait()
            pair_copy(1, t + 2).wait()
        if t + 2 < NT:
            pair_copy(2, t + 2).wait()
        if conv:
            items = [('inv', t + 1, 0), ('zstat', za), ('x1', t + 1, 0)]
            if t == 1:
                items += [('kvprep', t + 2, 1)]
            items += [('terms', tb)]
            if t + 2 < NT:
                items += [('fwh', t + 2)]
            if t + 2 < NT and t > 1:
                items += [('fwk', t + 2, 0)]
            items += [('z1', t, s0, ALL[:3]), ('mean', [SX, SZ]), ('z1', t, s0, ALL[3:4]), ('rstd', [SX, SZ])]
            if t == 1:
                items += [('fwk', t + 2, 1)]
            items += [('z1', t, s0, ALL[4:6] if t + 2 < NT else ALL[4:5])]
            run('B%d' % t, items)
        else:
            run('B7a', [('kick',), ('zstat', za), ('z1', t, s0, [0]), ('mean', [SZ]), ('z1', t, s0, [1]),
                        ('rstd', [SZ]), ('z1', t, s0, [2])])
            run('B7b', [('kick',), ('z2n', t, za, z2a, 4), ('z1', t - 1, s1, [NCH - 1])])

    for cp in big[-2:]:
        cp.wait()

    def stage_c(full, i, carry):
        p0 = lax.rem(i, 2)
        p1 = 1 - p0
        fx = [('x3', jnp.maximum(i - 2, 0), p0), ('x2stat', p1)]
        if not full:
            run('V1', [('g', i, z2a, ALL[:1])] + fx + [('g', i, z2a, ALL[1:4]), ('mean', [SX, S2]),
                       ('g', i, z2a, ALL[4:5]), ('rstd', [SX, S2]), ('g', i, z2a, ALL[5:]), ('o', i, p0)])
            return carry
        run('V2', [('g', i, z2a, ALL[:1]), ('xn', zp, i - 3, p1, 1)] + fx
            + [('z2n', jnp.maximum(i - 5, 0), (zc, p1), z2b, 4), ('zstat', (zc, p0)),
               ('g', i, z2a, ALL[1:5]), ('mean', [SX, SZ, S2], 1), ('g', i, z2a, ALL[5:6]), ('rstd', [SX, SZ, S2]),
               ('g', i, z2a, ALL[6:]), ('o', i, p0), ('z1', lax.rem(i + NT - 4, NT), p0, ALL[3:]),
               ('z1', i - 3, p1, ALL[:3]), ('z2', (zc, p1), p1, ALL)])
        return carry

    def stage_d(t, carry):
        @pl.when(t >= 2)
        def _():
            out_copy(t - 2, 0).wait()
            out_copy(t - 2, 1).wait()

        run('D', [('g', t, z2b, ALL), ('o', t, None)])
        out_copy(t, 1).start()
        return carry

    lax.fori_loop(0, 3, functools.partial(stage_c, False), 0)
    lax.fori_loop(3, NT, functools.partial(stage_c, True), 0)
    zbuf = {3: (zc, 1), 4: (zc, 0), 5: (zt[0], 0), 6: (zt[1], 0), 7: (zc, 0)}
    for i in range(NT, NT + 3):
        p0, p1 = i % 2, (i + 1) % 2
        sz_old, sz_new = (SZ, SL) if p0 == 0 else (SL, SZ)
        items = [('z1', i - 4, p0, ALL[3:4]), ('xn', zp, i - 3, p1, 0), ('z2n', i - 5, zbuf[i - 5], z2b, sz_old[1]),
                 ('zstat', zbuf[i - 4])]
        stats = [sz_new]
        if i - 2 < NT:
            items += [('x3', i - 2, p0)]
            stats += [SX]
        if i - 1 < NT:
            items += [('x2stat', p1)]
            stats += [S2]
        items += [('z1', i - 4, p0, ALL[4:]), ('z1', i - 3, p1, ALL[:3]), ('z2', zbuf[i - 3], p1, ALL[:2]),
                  ('mean', stats), ('z2', zbuf[i - 3], p1, ALL[2:3]), ('rstd', stats),
                  ('z2', zbuf[i - 3], p1, ALL[3:])]
        run('V3%d' % i, items)
    t = NT - 1
    run('T1', [('kick',), ('zstat', zbuf[t]), ('z2n', t - 1, zbuf[t - 1], z2b, SL[1]), ('z1', t, 1, [3]),
               ('mean', [SZ]), ('z1', t, 1, [4]), ('rstd', [SZ]), ('z1', t, 1, [5])])
    run('T2', [('kick',), ('z2n', t, zbuf[t], z2b, SZ[1]), ('z1', t, 1, [6])])
    lax.fori_loop(0, NT, stage_d, 0)
    for t in range(NT - 2, NT):
        out_copy(t, 0).wait()
        out_copy(t, 1).wait()


@jax.jit
def pallas_interleave_layers__ssm_conv_h3__mixer_gmlp__prompt_kernel(
        A_q, A_k, A_v, A_shift_k, A_ssm_k, A_ssm_D, B_x, B_w_in, B_w_sp, B_b_sp, B_w_out):
    del B_x
    any_spec = pl.BlockSpec(memory_space=pl.ANY)
    scratch = [
        pltpu.VMEM((2, TM + 16, D), bf16),
        pltpu.VMEM((8, B + 16, D), bf16),
        pltpu.VMEM((8, B, D), bf16),
        pltpu.VMEM((2, D, TM), bf16),
        pltpu.VMEM((D, F), bf16),
        pltpu.VMEM((NT, TM, S), bf16),
        pltpu.VMEM((FH, D), bf16),
        pltpu.VMEM((KS, D), bf16),
        pltpu.VMEM((8, 128), bf16),
        pltpu.VMEM((16, 128), bf16),
        pltpu.VMEM((NT, TM + 8, D), f32),
        pltpu.VMEM((NT, TM, D), f32),
        pltpu.VMEM((NT, TM, FH), bf16),
        pltpu.VMEM((S // 2, FH), u32),
        pltpu.VMEM((S // 2, FH), u32),
        pltpu.VMEM((NT, TM, 128), f32),
        pltpu.VMEM((KS + 1, 8, D), f32),
        pltpu.VMEM((2 * B, B), bf16),
        pltpu.VMEM((B, 2 * B), bf16),
        pltpu.VMEM((4, B, D), bf16),
        [pltpu.VMEM((2, 2 * B + 8, D), f32)] * NT,
        [pltpu.VMEM((2, 2 * B + 8, D), f32)] * NT,
        pltpu.VMEM((1, TM, D), f32),
        pltpu.VMEM((NZ, 2 * B + 8, D), f32),
        pltpu.VMEM((2, 2 * B, D), bf16),
        pltpu.VMEM((2, TM // 2, D), u32),
        [pltpu.VMEM((1, TM + 8, FH), f32)] * 2,
        pltpu.VMEM((2, TM + 8, FH), f32),
        pltpu.VMEM((2, TM + 8, D), f32),
        pltpu.VMEM((7, TM, 128), f32),
        pltpu.VMEM((8, TM, 128), f32),
        pltpu.VMEM((1, TM // 2, FH - TN), u32),
        pltpu.VMEM((1, TM // 2, TN), u32),
        pltpu.SMEM((16,), jnp.int32),
        pltpu.SemaphoreType.DMA((8,)),
        pltpu.SemaphoreType.DMA((3,)),
        pltpu.SemaphoreType.DMA((2,)),
        pltpu.SemaphoreType.DMA((4,)),
    ]
    out = pl.pallas_call(
        _kernel,
        out_shape=jax.ShapeDtypeStruct((NT, TM, D), bf16),
        in_specs=[any_spec] * 10,
        out_specs=any_spec,
        scratch_shapes=scratch,
        compiler_params=pltpu.CompilerParams(vmem_limit_bytes=127 * 1024 * 1024),
    )(A_q.reshape(NT, TM, D), A_k.reshape(NB, B, D), A_v.reshape(NB, B, D), A_shift_k.T, A_ssm_k,
      A_ssm_D.reshape(8, 128), B_w_in, B_w_sp.reshape(NT, TM, S), B_b_sp.reshape(16, 128), B_w_out)
    return out.reshape(1, S, D)
```

```python
import functools
import math
import jax
import jax.numpy as jnp
from jax import lax
import jax.experimental.pallas as pl
import jax.experimental.pallas.tpu as pltpu

S = 2048
D = 1024
F = 3584
FH = F // 2
KS = 4
B = 128
NB = S // B
EPS = 1e-5
f32 = jnp.float32
bf16 = jnp.bfloat16
u32 = jnp.uint32

TM = 256
NT = S // TM
TN = 256
NCH = FH // TN
RG = 16
GW = 256
LR = 16
NZ = 8
CAP_A = 9
CAP_B = 14
GWF = 128
OS = 3
ROT = 256


def _plan(cap_a, cap_b):
    done = set((a, ap) for a in (0, 1) for ap in range(a + 1))
    blocks = {}
    for t in range(NT - 1):
        for kind, cap in (('A', cap_a), ('B', cap_b)):
            sel = {}
            n = 0
            lo = 2 * t + 2 if kind == 'A' else 2 * t + 4
            lim = 2 * t + 3
            for a in range(lo, NB):
                g = [ap for ap in range(a + 1) if (a, ap) not in done and ap <= lim and a - ap <= lim]
                if a > lim:
                    g = g[:max(cap - n, 0)]
                if g:
                    sel[a] = g
                    n += len(g)
            groups = []
            for a in sorted(sel):
                first = not any((a, x) in done for x in range(a + 1))
                done.update((a, x) for x in sel[a])
                last = all((a, x) in done for x in range(a + 1))
                assert a < lo + NZ and last == (a <= 2 * t + 3)
                groups.append((a, sel[a], first, last))
            blocks[(kind, t)] = groups
    assert len(done) == NB * (NB + 1) // 2
    return blocks


def _gelu(x):
    u = x * (0.7978845608028654 + 0.035677408136300125 * (x * x))
    h = 0.5 * x
    return h + h * jnp.tanh(u)


def _h(v):
    return pltpu.bitcast(v, bf16)


def _part(v):
    acc = v[:, 0:128]
    for c in range(128, v.shape[1], 128):
        acc = acc + v[:, c:c + 128]
    return acc


def _lsum(acc):
    return jnp.broadcast_to(jnp.sum(acc, axis=1, keepdims=True), acc.shape)


def _wide(v, n):
    return jnp.concatenate([v] * (n // 128), axis=1)


def _ln(x):
    n = x.shape[-1]
    m = jnp.sum(x, axis=-1, keepdims=True) * (1.0 / n)
    xc = x - m
    v = jnp.sum(xc * xc, axis=-1, keepdims=True) * (1.0 / n)
    return xc * lax.rsqrt(v + EPS)


def _dft_rows(shape, row_dim):
    r = lax.broadcasted_iota(jnp.int32, shape, row_dim)
    n = lax.broadcasted_iota(jnp.int32, shape, 1 - row_dim)
    is_im = r >= B
    rr = jnp.where(is_im, r - B, r)
    odd = rr >= B // 2
    fidx = jnp.where(odd, 2 * (rr - B // 2) + 1, 2 * rr)
    m = (2 * fidx + 1) * n - jnp.where(is_im, B, 0)
    m = jnp.bitwise_and(m, 4 * B - 1)
    m = jnp.where(m > 2 * B, 4 * B - m, m)
    return jnp.cos(m.astype(f32) * (math.pi / (2 * B)))


NT_DIMS = (((1,), (1,)), ((), ()))


def _kernel(q_hbm, k_hbm, v_hbm, sk_hbm, h_hbm, sd_hbm, win_hbm, wsp_hbm, bsp_hbm, wout_hbm,
            o_hbm,
            qb, kb, vb, hb, win, wsp, wout, skb, sdb, bspb,
            x_v, y_v, z1_v, z2a, z2b, bb_v, skt, fm_v, im_v, kvb, ks, hs, wold, zp, zb,
            xn_v, zt, zc, xa, ps, st, ua, ub, zs,
            sem_c, sem_w, sem_s, sem_o):
    plan = _plan(CAP_A, CAP_B)

    def pair_copy(j, p):
        if j == 0:
            return pltpu.make_async_copy(k_hbm.at[pl.ds(2 * p, 2)], kb.at[pl.ds(2 * p % 8, 2), pl.ds(0, B)], sem_c.at[p % 2])
        if j == 1:
            return pltpu.make_async_copy(v_hbm.at[pl.ds(2 * p, 2)], vb.at[pl.ds(2 * p % 8, 2)], sem_c.at[2 + p % 2])
        if j == 2:
            cols = pl.ds(p * TM, TM)
            return pltpu.make_async_copy(h_hbm.at[:, cols], hb.at[p % 2], sem_c.at[4 + p % 2])
        return pltpu.make_async_copy(q_hbm.at[p], qb.at[p % 2, pl.ds(0, TM)], sem_c.at[6 + p % 2])

    WG = ((7, 10), (10, 12), (12, 14), (0, 3), (3, 6), (6, 7))

    def w_copy(i):
        cols = pl.ds(WG[i][0] * TN, (WG[i][1] - WG[i][0]) * TN)
        return pltpu.make_async_copy(win_hbm.at[:, cols], win.at[:, cols], sem_w.at[i % 3])

    def out_copy(t, j):
        cols = pl.ds(0, OS * TN) if j == 0 else pl.ds(OS * TN, D - OS * TN)
        return pltpu.make_async_copy(z1_v.at[t, :, cols], o_hbm.at[t, :, cols], sem_o.at[2 * (t % 2) + j])

    def issue(*copies):
        for cp in copies:
            cp.start(priority=1)

    def issue_big(j):
        if j >= 2:
            big[j - 2].wait()
        issue(big[j])

    small = [
        pltpu.make_async_copy(sk_hbm, skb, sem_o.at[0]),
        pltpu.make_async_copy(sd_hbm, sdb, sem_o.at[1]),
        pltpu.make_async_copy(bsp_hbm, bspb, sem_o.at[2]),
    ]
    WR = FH // 4
    big = ([pltpu.make_async_copy(wsp_hbm.at[j], wsp.at[j], sem_s.at[j % 2]) for j in range(NT)]
           + [pltpu.make_async_copy(wout_hbm.at[pl.ds(j * WR, WR)], wout.at[pl.ds(j * WR, WR)], sem_s.at[j % 2])
              for j in range(4)])
    for cp in small:
        cp.start()
    pair_copy(0, 0).start(priority=1)
    pair_copy(1, 0).start(priority=1)

    def zinit(i, c):
        zs[i] = 0
        return c
    lax.fori_loop(0, 16, zinit, 0)
    issue(pair_copy(2, 0))

    fm_v[...] = _dft_rows((2 * B, B), 0).astype(bf16)
    im_v[...] = (_dft_rows((B, 2 * B), 1) * (1.0 / B)).astype(bf16)

    for cp in small:
        cp.wait()
    sk4 = skb[...].astype(f32)
    for j in range(KS):
        skt[j] = jnp.broadcast_to(sk4[j:j + 1, :], (8, D))
    sd8 = sdb[...].astype(f32)
    skt[KS] = jnp.concatenate([jnp.broadcast_to(sd8[i:i + 1, :], (8, 128)) for i in range(8)], axis=1)

    def kvprep(p, z):
        for a in (2 * p, 2 * p + 1):
            for c in range(0, D, GW):
                for r0 in range(0, B, 32):
                    kcur = kb[a % 8 + z, r0:r0 + 32, c:c + GW].astype(f32)
                    if a == 0 and r0 == 0:
                        kprev = jnp.zeros((8, GW), f32)
                    elif r0 == 0:
                        kprev = kb[(a - 1) % 8 + z, B - 16:B, c:c + GW].astype(f32)[8:16]
                    else:
                        kprev = kb[a % 8 + z, r0 - 16:r0, c:c + GW].astype(f32)[8:16]
                    ext = jnp.concatenate([kprev, kcur], axis=0)
                    sk = [jnp.concatenate([skt[j, :, c:c + GW]] * 4, axis=0) for j in range(KS)]
                    acc = kcur * sk[0]
                    for j in range(1, KS):
                        acc = acc + pltpu.roll(ext, j, 0)[8:] * sk[j]
                    kvb[a % 4, r0:r0 + 32, c:c + GW] = (acc * vb[a % 8, r0:r0 + 32, c:c + GW].astype(f32)).astype(bf16)

    CW = 512

    def rot(c, k, w):
        c = (c + ROT * k) % D
        return slice(c, c + w)

    def put(ref, i, c, val, k):
        for j in range(0, CW, 256):
            ref[i, 0:B, rot(c + j, k, 256)] = val[0:B, j:j + 256]
            ref[i, B:2 * B, rot(c + j, k + 2, 256)] = val[B:2 * B, j:j + 256]

    def fw_h(p):
        fm = fm_v[...]
        res = []
        for a in (2 * p, 2 * p + 1):
            for c in range(0, D, CW):
                hh = lax.dot_general(fm, hb[p % 2, c:c + CW, (a % 2) * B:(a % 2 + 1) * B], NT_DIMS,
                                     preferred_element_type=f32)
                res.append(hh)
                if a == 0:
                    sd = jnp.concatenate([skt[KS, :, c:c + CW]] * (B // 8), axis=0)
                    hh = jnp.concatenate([hh[0:B] + sd, hh[B:2 * B]], axis=0)
                put(hs[p], a % 2, c, hh, 1)
        return res

    def fw_k(p, zk):
        fm = fm_v[...]
        res = []
        for a in (2 * p, 2 * p + 1):
            for c in range(0, D, CW):
                hh = jnp.dot(fm, kvb[a % 4 + zk, :, c:c + CW], preferred_element_type=f32)
                res.append(hh)
                put(ks[p], a % 2, c, hh, 0)
        return res

    def term_tasks(groups, newp):
        def acc(a, g, first, r, c, z, GW):
            zr = zi = None
            for ap in g:
                d = a - ap
                xr = ks[ap // 2][ap % 2 + z, r:r + RG, c:c + GW]
                xi = ks[ap // 2][ap % 2 + z, B + r:B + r + RG, rot(c, 2, GW)]
                hr = hs[d // 2][d % 2 + z, r:r + RG, rot(c, 1, GW)]
                hi = hs[d // 2][d % 2 + z, B + r:B + r + RG, rot(c, 3, GW)]
                tr = xr * hr - xi * hi
                ti = xr * hi + xi * hr
                zr = tr if zr is None else zr + tr
                zi = ti if zi is None else zi + ti
            if not first:
                zr = zr + zp[a % NZ, r:r + RG, c:c + GW]
                zi = zi + zp[a % NZ, B + r:B + r + RG, c:c + GW]
            return zr, zi

        def part_task(a, g, first, r, c, z):
            zr, zi = acc(a, g, first, r, c, z, GW)
            zp[a % NZ, r:r + RG, c:c + GW] = zr
            zp[a % NZ, B + r:B + r + RG, c:c + GW] = zi

        def fin_task(fin, r, c, z):
            GW = GWF
            if fin[0][0] > 0:
                pr = wold[0, r:r + RG, c:c + GW]
                pi = wold[0, B + r:B + r + RG, c:c + GW]
            for (a, g, first, last) in fin:
                wr, wi = acc(a, g, first, r, c, z, GW)
                if a == 0:
                    zr, zi = wr, wi
                elif r < B // 2:
                    zr, zi = wr + pi, wi - pr
                else:
                    zr, zi = wr - pi, wi + pr
                zb[a % 2, r:r + RG, c:c + GW] = zr.astype(bf16)
                zb[a % 2, B + r:B + r + RG, c:c + GW] = zi.astype(bf16)
                pr, pi = wr, wi
            if fin[-1][0] < NB - 1:
                wold[0, r:r + RG, c:c + GW] = pr
                wold[0, B + r:B + r + RG, c:c + GW] = pi

        def srcs(gs):
            return (set(('k', ap // 2) for (a, g, _, _) in gs for ap in g)
                    | set(('h', (a - ap) // 2) for (a, g, _, _) in gs for ap in g))

        rc = [(r, c) for r in range(0, B, RG) for c in range(0, D, GW)]
        tasks = []
        for grp in groups:
            a, g, first, last = grp
            if not last:
                sr = srcs([grp])
                new = any(i == newp for (_, i) in sr)
                tasks += [(len(g), new, sr, ('zp', a % NZ),
                           functools.partial(part_task, a, g, first, r, c)) for (r, c) in rc]
        tasks.sort(key=lambda x: x[1])
        fin = [x for x in groups if x[3]]
        if fin:
            tasks += [(sum(len(x[1]) for x in fin) + 1, True, srcs(fin), ('zb', 0),
                       functools.partial(fin_task, fin, r, c)) for r in range(0, B, RG) for c in range(0, D, GWF)]
        return tasks

    def split_tasks(tasks, caps):
        total = sum(x[0] for x in tasks)
        out = [[] for _ in caps]
        cum = 0
        for x in tasks:
            pos = (cum + 0.5 * x[0]) / max(total, 1) * sum(caps)
            k = 0
            while k + 1 < len(caps) and pos > sum(caps[:k + 1]):
                k += 1
            out[k].append(x)
            cum += x[0]
        return out

    def run_tasks(tasks, val, z):
        for (kind, i) in sorted(set().union(*[x[2] for x in tasks])) if tasks else []:
            (ks if kind == 'k' else hs)[i][0, 2 * B:2 * B + 8, 0:128] = val
        for x in tasks:
            x[4](z)
        probes = {}
        for x in tasks:
            probes[x[3][0]] = x[3][1]
        return probes

    def probe(probes, z):
        vals = []
        if 'zp' in probes:
            vals.append(zp[probes['zp'] + z, 0:8, 0:128])
        if 'zb' in probes:
            vals.append(zb[z, 0:16, 0:128].astype(f32)[0:8])
        return vals

    def sync(vals):
        v = vals[0]
        for w in vals[1:]:
            v = v + w
        return _lsum(v)

    def inv(p, z):
        im = im_v[...]
        res = []
        for d in range(2):
            for c in range(0, D, CW):
                y = jnp.dot(im, zb[d + z, :, c:c + CW], preferred_element_type=f32)
                res.append(y)
                y_v[p, d * B:(d + 1) * B, c:c + CW] = y
        return res

    R = range(0, TM, LR)

    def corner(acc):
        return acc[acc.shape[0] - 8:, acc.shape[1] - 128:]

    def b16(v):
        return jnp.concatenate([v, v], axis=0).astype(bf16)

    def stat_part(x, i, r, n):
        w = x.shape[1]
        mu = _part(x) * (128.0 / w)
        dv = x - _wide(mu, w)
        ps[i, r:r + n] = mu
        ps[i + 1, r:r + n] = _part(dv * dv)

    def stat_mean(i, j, w, z):
        mu = ps[i + z]
        m = _lsum(mu) * (1.0 / 128)
        st[j] = m
        e = mu - m
        ps[i] = ps[i + 1 + z] + (w / 128.0) * (e * e)

    def stat_rstd(i, j, w, z):
        st[j + 1] = lax.rsqrt(_lsum(ps[i + z]) * (1.0 / w) + EPS)

    def norm(x, j, r, n):
        w = x.shape[1]
        return (x - _wide(st[j, r:r + n], w)) * _wide(st[j + 1, r:r + n], w)

    PG = 6

    def z_dot(xn, n):
        return jnp.dot(xn, win[:, n * TN:(n + 1) * TN], preferred_element_type=f32)

    def kick():
        return jnp.dot(fm_v[0:16, :], fm_v[0:128, :], preferred_element_type=f32)

    def lead(ref, i):
        return ref[i, 0:16, 0:128].astype(f32)[0:8]

    def tile_rows(t, r, n):
        if isinstance(t, int):
            return slice(t * TM // 2 + r, t * TM // 2 + r + n)
        return pl.ds(pl.multiple_of(t * (TM // 2) + r, 8), n)

    def block(items):
        z = [zs[j] for j in range(8)]
        c = dict(sg=None, acc=None, vals=[], xn={}, ng=0, rel=[])

        def release(ref):
            if not any(ref is x for x in c['rel']):
                c['rel'].append(ref)
                ref[0, TM:TM + 8, 0:128] = c['sg']

        def mxu(res):
            if c['sg'] is None:
                c['sg'] = res[0][0:8, 0:128]
            c['acc'] = res[-1]

        def get_xn(i):
            if id(i) not in c['xn']:
                c['xn'][id(i)] = pltpu.bitcast(xn_v[i], bf16)
            return c['xn'][id(i)]

        for it in items:
            kind = it[0]
            sg = c['sg']
            if kind == 'kick':
                mxu([kick()])
            elif kind == 'z1':
                for n in it[3]:
                    acc = z_dot(get_xn(it[2]), n)
                    z1_v[it[1], :, n * TN:(n + 1) * TN] = _gelu(acc).astype(bf16)
                    mxu([acc])
            elif kind == 'z2':
                for n in it[3]:
                    acc = z_dot(get_xn(it[2]), NCH + n)
                    it[1][0][it[1][1], 0:TM, n * TN:(n + 1) * TN] = _gelu(acc)
                    mxu([acc])
            elif kind == 'inv':
                mxu(inv(it[1], z[1] if it[2] else 0))
            elif kind == 'fwh':
                mxu(fw_h(it[1]))
            elif kind == 'fwk':
                mxu(fw_k(it[1], z[1] if it[2] else 0))
            elif kind == 'g':
                if 'ws' not in c:
                    c['ws'] = wsp[it[1]]
                ws = c['ws']
                bbt = _wide(bb_v[it[1]], TN)
                for n in it[3]:
                    acc = jnp.dot(ws, _h(it[2][:, n * TN:(n + 1) * TN]), preferred_element_type=f32)
                    u = (z1_v[it[1], :, n * TN:(n + 1) * TN].astype(f32) * (acc + bbt)).astype(bf16)
                    u = pltpu.bitcast(u, u32)
                    if n < NCH - 1:
                        ua[0, :, n * TN:(n + 1) * TN] = u
                    else:
                        ub[0] = u
                    mxu([acc])
            elif kind == 'o':
                u = _h(jnp.concatenate([ua[z[1]], ub[z[1]]], axis=1))
                for n in range(D // TN):
                    acc = jnp.dot(u, wout[:, n * TN:(n + 1) * TN], preferred_element_type=f32)
                    x2 = (zp if it[2] is None else x_v)[it[1], 0:TM, n * TN:(n + 1) * TN] + acc
                    if it[2] is None:
                        z1_v[it[1], :, n * TN:(n + 1) * TN] = x2.astype(bf16)
                        if n == OS - 1:
                            out_copy(it[1], 0).start()
                    else:
                        xa[it[2], 0:TM, n * TN:(n + 1) * TN] = x2
                    mxu([acc])
            elif kind == 'xn':
                release(it[1])
                for r in R:
                    xn_v[it[3], r // 2:(r + LR) // 2] = pltpu.bitcast(
                        norm(it[1][it[2] + z[0], r:r + LR], 2, r, LR).astype(bf16), u32)
                c['xn'][id(it[3])] = pltpu.bitcast(xn_v[it[3] + z[1]], bf16)
                if it[4]:
                    c['vals'].append(pltpu.bitcast(xn_v[it[3] + z[6], 0:8, 0:128], f32))
            elif kind == 'z2n':
                release(it[2][0])
                for r in R:
                    it[3][tile_rows(it[1], r // 2, LR // 2), :] = pltpu.bitcast(
                        norm(it[2][0][it[2][1] + z[0], r:r + LR], it[4], r, LR).astype(bf16), u32)
                c['vals'].append(pltpu.bitcast(it[3][tile_rows(it[1] + z[6], 0, 8), 0:128], f32))
            elif kind == 'qstat':
                qb[0, TM:TM + 16, 0:128] = b16(sg)
                for r in R:
                    stat_part(qb[it[1] % 2 + z[0], r:r + LR].astype(f32), 0, r, LR)
            elif kind == 'zstat':
                release(it[1][0])
                for r in range(0, TM, 8):
                    stat_part(it[1][0][it[1][1] + z[0], r:r + 8], 2, r, 8)
            elif kind == 'x1':
                if it[2]:
                    qb[0, TM:TM + 16, 0:128] = b16(sg)
                for r in R:
                    x0 = qb[it[1] % 2 + (z[0] if it[2] else 0), r:r + LR].astype(f32)
                    x1 = x0 + norm(x0, 0, r, LR) * y_v[it[1] + (0 if it[2] else z[1]), r:r + LR]
                    x_v[it[1], r:r + LR] = x1
                    stat_part(x1, 0, r, LR)
            elif kind == 'x2stat':
                release(xa)
                for r in R:
                    stat_part(xa[it[1] + z[0], r:r + LR], 4, r, LR)
            elif kind == 'x3':
                release(xa)
                for r in R:
                    x0 = xa[it[2] + z[0], r:r + LR]
                    x1 = x0 + norm(x0, 0, r, LR) * y_v[it[1], r:r + LR]
                    zp[it[1], r:r + LR] = x1
                    stat_part(x1, 0, r, LR)
            elif kind == 'kvprep':
                kb[0, B:B + 16, 0:128] = b16(sg)
                kvprep(it[1], z[0])
                if not it[2]:
                    c['vals'].append(lead(kvb, (2 * it[1]) % 4 + z[6]))
            elif kind == 'terms':
                c['vals'] += probe(run_tasks(it[1], sg, z[0]), z[6])
            elif kind == 'mean' or kind == 'rstd':
                gate = corner(c['acc'])
                if len(it) > 2:
                    for v in c['vals']:
                        gate = gate + v
                    c['vals'] = []
                ps[PG, 8 * c['ng']:8 * c['ng'] + 8] = gate
                c['ng'] += 1
                for (i, j, w) in it[1]:
                    (stat_mean if kind == 'mean' else stat_rstd)(i, j, w, z[1 + c['ng']])
            elif kind == 'bb':
                bs16 = bspb[...].astype(f32)
                for i in range(S // 128):
                    bb_v[i // 2, (i % 2) * 128:(i % 2 + 1) * 128, :] = jnp.transpose(
                        jnp.broadcast_to(bs16[i:i + 1, :], (128, 128)))
        if c['vals']:
            ps[PG, 64:72] = sync([c['acc'][0:8, 0:128]] + c['vals'])

    def run(name, items, cond=None):
        with jax.named_scope(name):
            pl.when(zs[15] == 0 if cond is None else cond)(lambda: block(items))

    SQ, SX, SZ, S2, SL = (0, 0, D), (0, 2, D), (2, 4, FH), (4, 0, D), (2, 6, FH)
    Z0 = (zt[0], 0)
    ALL = list(range(NCH))

    def block_p0():
        kvprep(0, 0)

    def block_p1():
        fw_k(0, 0)
        fw_h(0)

    def block_p2():
        z = [zs[j] for j in range(4)]
        sg = fw_h(1)[0][0:8, 0:128]
        run_tasks(term_tasks([(0, [0], True, True), (1, [0, 1], True, True)], 0), sg, z[1])
        qb[0, TM:TM + 16, 0:128] = b16(sg)
        for r in R:
            stat_part(qb[z[1], r:r + LR].astype(f32), 0, r, LR)
        stat_mean(0, 0, D, z[2])
        inv(0, z[0])
        stat_rstd(0, 0, D, z[3])

    def block_p3():
        kvprep(1, 0)
        fw_k(1, zs[0])
        for r in R:
            x0 = qb[0, r:r + LR].astype(f32)
            x1 = x0 + norm(x0, 0, r, LR) * y_v[0, r:r + LR]
            x_v[0, r:r + LR] = x1
            xn_v[0, r // 2:(r + LR) // 2] = pltpu.bitcast(_ln(x1).astype(bf16), u32)

    for name, waits, fn, nxt in (
            ('P0', ((0, 0), (1, 0)), block_p0, [pair_copy(3, 0), pair_copy(2, 1)]),
            ('P1', ((2, 0),), block_p1, [pair_copy(0, 1), pair_copy(1, 1)]),
            ('P2', ((3, 0), (2, 1)), block_p2, [w_copy(0)]),
            ('P3', ((0, 1), (1, 1)), block_p3, [pair_copy(3, 1), w_copy(1)])):
        issue(*nxt)
        for (j, p) in waits:
            pair_copy(j, p).wait()
        with jax.named_scope(name):
            pl.when(zs[15] == 0)(fn)

    for t in range(NT):
        conv = t < NT - 1
        ta = term_tasks(plan[('A', t)], -1) if conv else []
        tb = term_tasks(plan[('B', t)], -1) if conv else []
        if t == 0:
            ch = split_tasks(ta, [3, 1.5, 2])
            issue(w_copy(2))
            w_copy(0).wait()
            run('A0a', [('kick',), ('terms', ch[0]), ('z2', Z0, 0, [0, 1, 2])])
            issue(pair_copy(0, 2), pair_copy(1, 2), pair_copy(2, 2))
            pair_copy(3, 1).wait()
            w_copy(1).wait()
            run('A0b', [('kick',), ('qstat', 1), ('terms', ch[1]), ('z2', Z0, 0, [3]), ('mean', [SQ]),
                        ('z2', Z0, 0, [4])])
            issue(w_copy(3))
            w_copy(2).wait()
            run('A0c', [('kick',), ('rstd', [SQ]), ('terms', ch[2]), ('z2', Z0, 0, [5, 6])])
            issue(w_copy(4))
            for j in range(3):
                pair_copy(j, 2).wait()
            run('B0a', [('inv', 1, 0), ('kvprep', 2, 1), ('fwh', 2), ('fwk', 2, 1)])
            issue(w_copy(5), pair_copy(3, 2), pair_copy(0, 3), pair_copy(1, 3))
            w_copy(3).wait()
            run('B0b', [('kick',), ('zstat', Z0), ('x1', 1, 1), ('z1', 0, 0, [0, 1]), ('mean', [SX, SZ]),
                        ('z1', 0, 0, [2])])
            w_copy(4).wait()
            run('B0c', [('kick',), ('rstd', [SX, SZ]), ('terms', tb), ('bb',), ('z1', 0, 0, [3, 4, 5])])
            w_copy(5).wait()
            continue
        if t + 2 < NT:
            issue(pair_copy(2, t + 2), pair_copy(3, t + 2))
        if t + 3 < NT:
            issue(pair_copy(0, t + 3), pair_copy(1, t + 3))
        if t > 1:
            issue_big(2 * t - 3)
        if conv:
            pair_copy(3, t + 1).wait()
        if t + 2 < NT and t > 1:
            pair_copy(0, t + 2).wait()
            pair_copy(1, t + 2).wait()
        s0, s1 = t % 2, (t - 1) % 2
        za, zo = (zt[s0], 0), (zt[s1], 0)
        items = [('z1', t - 1, s1, [NCH - 1 if conv else NCH - 2]), ('xn', x_v, t, s0, 0), ('z2n', t - 1, zo, z2a, 4)]
        if conv:
            items += [('qstat', t + 1)]
            if t + 2 < NT and t > 1:
                items += [('kvprep', t + 2, 0)]
            items += [('terms', ta), ('z2', za, s0, ALL[:4]), ('mean', [SQ]), ('z2', za, s0, ALL[4:5]),
                      ('rstd', [SQ]), ('z2', za, s0, ALL[5:])]
        else:
            items += [('z2', za, s0, ALL)]
        run('A%d' % t, items)
        if conv:
            issue_big(2 * t - 2)
        if t == 1:
            pair_copy(0, t + 2).wait()
            pair_copy(1, t + 2).wait()
        if t + 2 < NT:
            pair_copy(2, t + 2).wait()
        if conv:
            items = [('inv', t + 1, 0), ('zstat', za), ('x1', t + 1, 0)]
            if t == 1:
                items += [('kvprep', t + 2, 1)]
            items += [('terms', tb)]
            if t + 2 < NT:
                items += [('fwh', t + 2)]
            if t + 2 < NT and t > 1:
                items += [('fwk', t + 2, 0)]
            if t + 2 < NT:
                items += [('z1', t, s0, ALL[:2]), ('mean', [SZ]), ('z1', t, s0, ALL[2:3]), ('mean', [SX]),
                          ('z1', t, s0, ALL[3:4]), ('rstd', [SZ])]
                if t == 1:
                    items += [('fwk', t + 2, 1)]
                items += [('z1', t, s0, ALL[4:5]), ('rstd', [SX]), ('z1', t, s0, ALL[5:6])]
            else:
                items += [('z1', t, s0, ALL[:2]), ('mean', [SZ]), ('z1', t, s0, ALL[2:3]), ('mean', [SX]),
                          ('rstd', [SZ]), ('z1', t, s0, ALL[3:4]), ('rstd', [SX]), ('z1', t, s0, ALL[4:5])]
            run('B%d' % t, items)
        else:
            run('B7a', [('kick',), ('zstat', za), ('z1', t, s0, [0]), ('mean', [SZ]), ('z1', t, s0, [1]),
                        ('rstd', [SZ]), ('z1', t, s0, [2])])
            run('B7b', [('kick',), ('z2n', t, za, z2a, 4), ('z1', t - 1, s1, [NCH - 1])])

    for cp in big[-2:]:
        cp.wait()

    def stage_c(full, i, carry):
        p0 = lax.rem(i, 2)
        p1 = 1 - p0
        fx = [('x3', jnp.maximum(i - 2, 0), p0), ('x2stat', p1)]
        if not full:
            run('V1', [('g', i, z2a, ALL[:1])] + fx + [('g', i, z2a, ALL[1:3]), ('mean', [SX]),
                       ('g', i, z2a, ALL[3:4]), ('mean', [S2]), ('g', i, z2a, ALL[4:5]), ('rstd', [SX]),
                       ('g', i, z2a, ALL[5:6]), ('rstd', [S2]), ('g', i, z2a, ALL[6:]), ('o', i, p0)])
            return carry
        t4 = lax.rem(i + NT - 4, NT)
        run('V2', [('g', i, z2a, ALL[:1]), ('xn', zp, i - 3, p1, 1)] + fx
            + [('z2n', jnp.maximum(i - 5, 0), (zc, p1), z2b, 4), ('zstat', (zc, p0)),
               ('g', i, z2a, ALL[1:5]), ('mean', [SX], 1), ('g', i, z2a, ALL[5:6]), ('mean', [SZ]),
               ('g', i, z2a, ALL[6:]), ('mean', [S2]), ('z1', t4, p0, ALL[3:4]), ('rstd', [SX]),
               ('z1', t4, p0, ALL[4:5]), ('rstd', [SZ]), ('z1', t4, p0, ALL[5:6]), ('rstd', [S2]),
               ('z1', t4, p0, ALL[6:]), ('z1', i - 3, p1, ALL[:3]), ('z2', (zc, p1), p1, ALL), ('o', i, p0)])
        return carry

    def stage_d(t, carry):
        @pl.when(t >= 2)
        def _():
            out_copy(t - 2, 0).wait()
            out_copy(t - 2, 1).wait()

        run('D', [('g', t, z2b, ALL), ('o', t, None)])
        out_copy(t, 1).start()
        return carry

    lax.fori_loop(0, 3, functools.partial(stage_c, False), 0)
    lax.fori_loop(3, NT, functools.partial(stage_c, True), 0)
    zbuf = {3: (zc, 1), 4: (zc, 0), 5: (zt[0], 0), 6: (zt[1], 0), 7: (zc, 0)}
    for i in range(NT, NT + 3):
        p0, p1 = i % 2, (i + 1) % 2
        sz_old, sz_new = (SZ, SL) if p0 == 0 else (SL, SZ)
        items = [('z1', i - 4, p0, ALL[3:4]), ('xn', zp, i - 3, p1, 0), ('z2n', i - 5, zbuf[i - 5], z2b, sz_old[1]),
                 ('zstat', zbuf[i - 4])]
        stats = [sz_new]
        if i - 2 < NT:
            items += [('x3', i - 2, p0)]
            stats += [SX]
        if i - 1 < NT:
            items += [('x2stat', p1)]
            stats += [S2]
        items += [('z1', i - 4, p0, ALL[4:]), ('z1', i - 3, p1, ALL[:3])]
        gates = [('mean', [x]) for x in stats] + [('rstd', [x]) for x in stats]
        for n in ALL:
            items += gates[n:n + 1] + [('z2', zbuf[i - 3], p1, [n])]
        run('V3%d' % i, items)
    t = NT - 1
    run('T1', [('kick',), ('zstat', zbuf[t]), ('z2n', t - 1, zbuf[t - 1], z2b, SL[1]), ('z1', t, 1, [3]),
               ('mean', [SZ]), ('z1', t, 1, [4]), ('rstd', [SZ]), ('z1', t, 1, [5])])
    run('T2', [('kick',), ('z2n', t, zbuf[t], z2b, SZ[1]), ('z1', t, 1, [6])])
    lax.fori_loop(0, NT, stage_d, 0)
    for t in range(NT - 2, NT):
        out_copy(t, 0).wait()
        out_copy(t, 1).wait()


@jax.jit
def pallas_interleave_layers__ssm_conv_h3__mixer_gmlp__prompt_kernel(
        A_q, A_k, A_v, A_shift_k, A_ssm_k, A_ssm_D, B_x, B_w_in, B_w_sp, B_b_sp, B_w_out):
    del B_x
    any_spec = pl.BlockSpec(memory_space=pl.ANY)
    scratch = [
        pltpu.VMEM((2, TM + 16, D), bf16),
        pltpu.VMEM((8, B + 16, D), bf16),
        pltpu.VMEM((8, B, D), bf16),
        pltpu.VMEM((2, D, TM), bf16),
        pltpu.VMEM((D, F), bf16),
        pltpu.VMEM((NT, TM, S), bf16),
        pltpu.VMEM((FH, D), bf16),
        pltpu.VMEM((KS, D), bf16),
        pltpu.VMEM((8, 128), bf16),
        pltpu.VMEM((16, 128), bf16),
        pltpu.VMEM((NT, TM + 8, D), f32),
        pltpu.VMEM((NT, TM, D), f32),
        pltpu.VMEM((NT, TM, FH), bf16),
        pltpu.VMEM((S // 2, FH), u32),
        pltpu.VMEM((S // 2, FH), u32),
        pltpu.VMEM((NT, TM, 128), f32),
        pltpu.VMEM((KS + 1, 8, D), f32),
        pltpu.VMEM((2 * B, B), bf16),
        pltpu.VMEM((B, 2 * B), bf16),
        pltpu.VMEM((4, B, D), bf16),
        [pltpu.VMEM((2, 2 * B + 8, D), f32)] * NT,
        [pltpu.VMEM((2, 2 * B + 8, D), f32)] * NT,
        pltpu.VMEM((1, TM, D), f32),
        pltpu.VMEM((NZ, 2 * B + 8, D), f32),
        pltpu.VMEM((2, 2 * B, D), bf16),
        pltpu.VMEM((2, TM // 2, D), u32),
        [pltpu.VMEM((1, TM + 8, FH), f32)] * 2,
        pltpu.VMEM((2, TM + 8, FH), f32),
        pltpu.VMEM((2, TM + 8, D), f32),
        pltpu.VMEM((7, TM, 128), f32),
        pltpu.VMEM((8, TM, 128), f32),
        pltpu.VMEM((1, TM // 2, FH - TN), u32),
        pltpu.VMEM((1, TM // 2, TN), u32),
        pltpu.SMEM((16,), jnp.int32),
        pltpu.SemaphoreType.DMA((8,)),
        pltpu.SemaphoreType.DMA((3,)),
        pltpu.SemaphoreType.DMA((2,)),
        pltpu.SemaphoreType.DMA((4,)),
    ]
    out = pl.pallas_call(
        _kernel,
        out_shape=jax.ShapeDtypeStruct((NT, TM, D), bf16),
        in_specs=[any_spec] * 10,
        out_specs=any_spec,
        scratch_shapes=scratch,
        compiler_params=pltpu.CompilerParams(vmem_limit_bytes=127 * 1024 * 1024),
    )(A_q.reshape(NT, TM, D), A_k.reshape(NB, B, D), A_v.reshape(NB, B, D), A_shift_k.T, A_ssm_k,
      A_ssm_D.reshape(8, 128), B_w_in, B_w_sp.reshape(NT, TM, S), B_b_sp.reshape(16, 128), B_w_out)
    return out.reshape(1, S, D)
```

```python
import functools
import math
import jax
import jax.numpy as jnp
from jax import lax
import jax.experimental.pallas as pl
import jax.experimental.pallas.tpu as pltpu

S = 2048
D = 1024
F = 3584
FH = F // 2
KS = 4
B = 128
NB = S // B
EPS = 1e-5
f32 = jnp.float32
bf16 = jnp.bfloat16
u32 = jnp.uint32

TM = 256
NT = S // TM
TN = 256
NCH = FH // TN
RG = 16
GW = 256
LR = 16
NZ = 8
CAP_A = 9
CAP_B = 14
GWF = 128
OS = 3
ROT = 256


def _plan(cap_a, cap_b):
    done = set((a, ap) for a in (0, 1) for ap in range(a + 1))
    blocks = {}
    for t in range(NT - 1):
        for kind, cap in (('A', cap_a), ('B', cap_b)):
            sel = {}
            n = 0
            lo = 2 * t + 2 if kind == 'A' else 2 * t + 4
            lim = 2 * t + 3
            for a in range(lo, NB):
                g = [ap for ap in range(a + 1) if (a, ap) not in done and ap <= lim and a - ap <= lim]
                if a > lim:
                    g = g[:max(cap - n, 0)]
                if g:
                    sel[a] = g
                    n += len(g)
            groups = []
            for a in sorted(sel):
                first = not any((a, x) in done for x in range(a + 1))
                done.update((a, x) for x in sel[a])
                last = all((a, x) in done for x in range(a + 1))
                assert a < lo + NZ and last == (a <= 2 * t + 3)
                groups.append((a, sel[a], first, last))
            blocks[(kind, t)] = groups
    assert len(done) == NB * (NB + 1) // 2
    return blocks


def _gelu(x):
    u = x * (0.7978845608028654 + 0.035677408136300125 * (x * x))
    h = 0.5 * x
    return h + h * jnp.tanh(u)


def _h(v):
    return pltpu.bitcast(v, bf16)


def _part(v):
    acc = v[:, 0:128]
    for c in range(128, v.shape[1], 128):
        acc = acc + v[:, c:c + 128]
    return acc


def _lsum(acc):
    return jnp.broadcast_to(jnp.sum(acc, axis=1, keepdims=True), acc.shape)


def _wide(v, n):
    return jnp.concatenate([v] * (n // 128), axis=1)


def _ln(x):
    n = x.shape[-1]
    m = jnp.sum(x, axis=-1, keepdims=True) * (1.0 / n)
    xc = x - m
    v = jnp.sum(xc * xc, axis=-1, keepdims=True) * (1.0 / n)
    return xc * lax.rsqrt(v + EPS)


def _dft_rows(shape, row_dim):
    r = lax.broadcasted_iota(jnp.int32, shape, row_dim)
    n = lax.broadcasted_iota(jnp.int32, shape, 1 - row_dim)
    is_im = r >= B
    rr = jnp.where(is_im, r - B, r)
    odd = rr >= B // 2
    fidx = jnp.where(odd, 2 * (rr - B // 2) + 1, 2 * rr)
    m = (2 * fidx + 1) * n - jnp.where(is_im, B, 0)
    m = jnp.bitwise_and(m, 4 * B - 1)
    m = jnp.where(m > 2 * B, 4 * B - m, m)
    return jnp.cos(m.astype(f32) * (math.pi / (2 * B)))


NT_DIMS = (((1,), (1,)), ((), ()))


def _kernel(q_hbm, k_hbm, v_hbm, sk_hbm, h_hbm, sd_hbm, win_hbm, wsp_hbm, bsp_hbm, wout_hbm,
            o_hbm,
            qb, kb, vb, hb, win, wsp, wout, skb, sdb, bspb,
            x_v, y_v, z1_v, z2a, z2b, bb_v, skt, fm_v, im_v, kvb, ks, hs, wold, zp, zb,
            xn_v, zt, zc, xa, ps, st, ua, ub, zs,
            sem_c, sem_w, sem_s, sem_o):
    plan = _plan(CAP_A, CAP_B)

    def pair_copy(j, p):
        if j == 0:
            return pltpu.make_async_copy(k_hbm.at[pl.ds(2 * p, 2)], kb.at[pl.ds(2 * p % 8, 2), pl.ds(0, B)], sem_c.at[p % 2])
        if j == 1:
            return pltpu.make_async_copy(v_hbm.at[pl.ds(2 * p, 2)], vb.at[pl.ds(2 * p % 8, 2)], sem_c.at[2 + p % 2])
        if j == 2:
            cols = pl.ds(p * TM, TM)
            return pltpu.make_async_copy(h_hbm.at[:, cols], hb.at[p % 2], sem_c.at[4 + p % 2])
        return pltpu.make_async_copy(q_hbm.at[p], qb.at[p % 2, pl.ds(0, TM)], sem_c.at[6 + p % 2])

    WG = ((7, 10), (10, 12), (12, 14), (0, 3), (3, 6), (6, 7))

    def w_copy(i):
        cols = pl.ds(WG[i][0] * TN, (WG[i][1] - WG[i][0]) * TN)
        return pltpu.make_async_copy(win_hbm.at[:, cols], win.at[:, cols], sem_w.at[i % 3])

    def out_copy(t, j):
        cols = (pl.ds(0, D), pl.ds(0, OS * TN), pl.ds(OS * TN, D - OS * TN))[j]
        i = 2 * t + min(j, 1)
        return pltpu.make_async_copy(z1_v.at[i, :, cols], o_hbm.at[i, :, cols], sem_o.at[3 * (t % 2) + j])

    def issue(*copies):
        for cp in copies:
            cp.start(priority=1)

    def issue_big(j):
        if j >= 2:
            big[j - 2].wait()
        issue(big[j])

    small = [
        pltpu.make_async_copy(sk_hbm, skb, sem_o.at[0]),
        pltpu.make_async_copy(sd_hbm, sdb, sem_o.at[1]),
        pltpu.make_async_copy(bsp_hbm, bspb, sem_o.at[2]),
    ]
    WR = FH // 4
    big = ([pltpu.make_async_copy(wsp_hbm.at[j], wsp.at[j], sem_s.at[j % 2]) for j in range(NT)]
           + [pltpu.make_async_copy(wout_hbm.at[pl.ds(j * WR, WR)], wout.at[pl.ds(j * WR, WR)], sem_s.at[j % 2])
              for j in range(4)])
    for cp in small:
        cp.start()
    pair_copy(0, 0).start(priority=1)
    pair_copy(1, 0).start(priority=1)

    def zinit(i, c):
        zs[i] = 0
        return c
    lax.fori_loop(0, 16, zinit, 0)
    issue(pair_copy(2, 0))

    fm_v[...] = _dft_rows((2 * B, B), 0).astype(bf16)
    im_v[...] = (_dft_rows((B, 2 * B), 1) * (1.0 / B)).astype(bf16)

    for cp in small:
        cp.wait()
    sk4 = skb[...].astype(f32)
    for j in range(KS):
        skt[j] = jnp.broadcast_to(sk4[j:j + 1, :], (8, D))
    sd8 = sdb[...].astype(f32)
    skt[KS] = jnp.concatenate([jnp.broadcast_to(sd8[i:i + 1, :], (8, 128)) for i in range(8)], axis=1)

    def kvprep(p, z):
        for a in (2 * p, 2 * p + 1):
            for c in range(0, D, GW):
                for r0 in range(0, B, 32):
                    kcur = kb[a % 8 + z, r0:r0 + 32, c:c + GW].astype(f32)
                    if a == 0 and r0 == 0:
                        kprev = jnp.zeros((8, GW), f32)
                    elif r0 == 0:
                        kprev = kb[(a - 1) % 8 + z, B - 16:B, c:c + GW].astype(f32)[8:16]
                    else:
                        kprev = kb[a % 8 + z, r0 - 16:r0, c:c + GW].astype(f32)[8:16]
                    ext = jnp.concatenate([kprev, kcur], axis=0)
                    sk = [jnp.concatenate([skt[j, :, c:c + GW]] * 4, axis=0) for j in range(KS)]
                    acc = kcur * sk[0]
                    for j in range(1, KS):
                        acc = acc + pltpu.roll(ext, j, 0)[8:] * sk[j]
                    kvb[a % 4, r0:r0 + 32, c:c + GW] = (acc * vb[a % 8, r0:r0 + 32, c:c + GW].astype(f32)).astype(bf16)

    CW = 512

    def rot(c, k, w):
        c = (c + ROT * k) % D
        return slice(c, c + w)

    def put(ref, i, c, val, k):
        for j in range(0, CW, 256):
            ref[i, 0:B, rot(c + j, k, 256)] = val[0:B, j:j + 256]
            ref[i, B:2 * B, rot(c + j, k + 2, 256)] = val[B:2 * B, j:j + 256]

    def fw_h(p):
        fm = fm_v[...]
        res = []
        for a in (2 * p, 2 * p + 1):
            for c in range(0, D, CW):
                hh = lax.dot_general(fm, hb[p % 2, c:c + CW, (a % 2) * B:(a % 2 + 1) * B], NT_DIMS,
                                     preferred_element_type=f32)
                res.append(hh)
                if a == 0:
                    sd = jnp.concatenate([skt[KS, :, c:c + CW]] * (B // 8), axis=0)
                    hh = jnp.concatenate([hh[0:B] + sd, hh[B:2 * B]], axis=0)
                put(hs[p], a % 2, c, hh, 1)
        return res

    def fw_k(p, zk):
        fm = fm_v[...]
        res = []
        for a in (2 * p, 2 * p + 1):
            for c in range(0, D, CW):
                hh = jnp.dot(fm, kvb[a % 4 + zk, :, c:c + CW], preferred_element_type=f32)
                res.append(hh)
                put(ks[p], a % 2, c, hh, 0)
        return res

    def term_tasks(groups, newp):
        def acc(a, g, first, r, c, z, GW):
            zr = zi = None
            for ap in g:
                d = a - ap
                xr = ks[ap // 2][ap % 2 + z, r:r + RG, c:c + GW]
                xi = ks[ap // 2][ap % 2 + z, B + r:B + r + RG, rot(c, 2, GW)]
                hr = hs[d // 2][d % 2 + z, r:r + RG, rot(c, 1, GW)]
                hi = hs[d // 2][d % 2 + z, B + r:B + r + RG, rot(c, 3, GW)]
                tr = xr * hr - xi * hi
                ti = xr * hi + xi * hr
                zr = tr if zr is None else zr + tr
                zi = ti if zi is None else zi + ti
            if not first:
                zr = zr + zp[a % NZ, r:r + RG, c:c + GW]
                zi = zi + zp[a % NZ, B + r:B + r + RG, c:c + GW]
            return zr, zi

        def part_task(a, g, first, r, c, z):
            zr, zi = acc(a, g, first, r, c, z, GW)
            zp[a % NZ, r:r + RG, c:c + GW] = zr
            zp[a % NZ, B + r:B + r + RG, c:c + GW] = zi

        def fin_task(fin, r, c, z):
            GW = GWF
            if fin[0][0] > 0:
                pr = wold[0, r:r + RG, c:c + GW]
                pi = wold[0, B + r:B + r + RG, c:c + GW]
            for (a, g, first, last) in fin:
                wr, wi = acc(a, g, first, r, c, z, GW)
                if a == 0:
                    zr, zi = wr, wi
                elif r < B // 2:
                    zr, zi = wr + pi, wi - pr
                else:
                    zr, zi = wr - pi, wi + pr
                zb[a % 2, r:r + RG, c:c + GW] = zr.astype(bf16)
                zb[a % 2, B + r:B + r + RG, c:c + GW] = zi.astype(bf16)
                pr, pi = wr, wi
            if fin[-1][0] < NB - 1:
                wold[0, r:r + RG, c:c + GW] = pr
                wold[0, B + r:B + r + RG, c:c + GW] = pi

        def srcs(gs):
            return (set(('k', ap // 2) for (a, g, _, _) in gs for ap in g)
                    | set(('h', (a - ap) // 2) for (a, g, _, _) in gs for ap in g))

        rc = [(r, c) for r in range(0, B, RG) for c in range(0, D, GW)]
        tasks = []
        for grp in groups:
            a, g, first, last = grp
            if not last:
                sr = srcs([grp])
                new = any(i == newp for (_, i) in sr)
                tasks += [(len(g), new, sr, ('zp', a % NZ),
                           functools.partial(part_task, a, g, first, r, c)) for (r, c) in rc]
        tasks.sort(key=lambda x: x[1])
        fin = [x for x in groups if x[3]]
        if fin:
            tasks += [(sum(len(x[1]) for x in fin) + 1, True, srcs(fin), ('zb', 0),
                       functools.partial(fin_task, fin, r, c)) for r in range(0, B, RG) for c in range(0, D, GWF)]
        return tasks

    def split_tasks(tasks, caps):
        total = sum(x[0] for x in tasks)
        out = [[] for _ in caps]
        cum = 0
        for x in tasks:
            pos = (cum + 0.5 * x[0]) / max(total, 1) * sum(caps)
            k = 0
            while k + 1 < len(caps) and pos > sum(caps[:k + 1]):
                k += 1
            out[k].append(x)
            cum += x[0]
        return out

    def run_tasks(tasks, val, z):
        for (kind, i) in sorted(set().union(*[x[2] for x in tasks])) if tasks else []:
            (ks if kind == 'k' else hs)[i][0, 2 * B:2 * B + 8, 0:128] = val
        for x in tasks:
            x[4](z)
        probes = {}
        for x in tasks:
            probes[x[3][0]] = x[3][1]
        return probes

    def probe(probes, z):
        vals = []
        if 'zp' in probes:
            vals.append(zp[probes['zp'] + z, 0:8, 0:128])
        if 'zb' in probes:
            vals.append(zb[z, 0:16, 0:128].astype(f32)[0:8])
        return vals

    def sync(vals):
        v = vals[0]
        for w in vals[1:]:
            v = v + w
        return _lsum(v)

    def inv(p, z):
        im = im_v[...]
        res = []
        for d in range(2):
            for c in range(0, D, CW):
                y = jnp.dot(im, zb[d + z, :, c:c + CW], preferred_element_type=f32)
                res.append(y)
                y_v[p, d * B:(d + 1) * B, c:c + CW] = y
        return res

    R = range(0, TM, LR)

    def corner(acc):
        return acc[acc.shape[0] - 8:, acc.shape[1] - 128:]

    def b16(v):
        return jnp.concatenate([v, v], axis=0).astype(bf16)

    def stat_part(x, i, r, n):
        w = x.shape[1]
        mu = _part(x) * (128.0 / w)
        dv = x - _wide(mu, w)
        ps[i, r:r + n] = mu
        ps[i + 1, r:r + n] = _part(dv * dv)

    def stat_mean(i, j, w, z):
        mu = ps[i + z]
        m = _lsum(mu) * (1.0 / 128)
        st[j] = m
        e = mu - m
        ps[i] = ps[i + 1 + z] + (w / 128.0) * (e * e)

    def stat_rstd(i, j, w, z):
        st[j + 1] = lax.rsqrt(_lsum(ps[i + z]) * (1.0 / w) + EPS)

    def norm(x, j, r, n):
        w = x.shape[1]
        return (x - _wide(st[j, r:r + n], w)) * _wide(st[j + 1, r:r + n], w)

    PG = 6

    def z_dot(xn, n):
        return jnp.dot(xn, win[:, n * TN:(n + 1) * TN], preferred_element_type=f32)

    def kick():
        return jnp.dot(fm_v[0:16, :], fm_v[0:128, :], preferred_element_type=f32)

    def lead(ref, i):
        return ref[i, 0:16, 0:128].astype(f32)[0:8]

    def tile_rows(t, r, n):
        if isinstance(t, int):
            return slice(t * TM // 2 + r, t * TM // 2 + r + n)
        return pl.ds(pl.multiple_of(t * (TM // 2) + r, 8), n)

    def block(items):
        z = [zs[j] for j in range(8)]
        c = dict(sg=None, acc=None, vals=[], xn={}, ng=0, rel=[])

        def release(ref):
            if not any(ref is x for x in c['rel']):
                c['rel'].append(ref)
                ref[0, TM:TM + 8, 0:128] = c['sg']

        def mxu(res):
            if c['sg'] is None:
                c['sg'] = res[0][0:8, 0:128]
            c['acc'] = res[-1]

        def get_xn(i):
            if id(i) not in c['xn']:
                c['xn'][id(i)] = pltpu.bitcast(xn_v[i], bf16)
            return c['xn'][id(i)]

        for it in items:
            kind = it[0]
            sg = c['sg']
            if kind == 'kick':
                mxu([kick()])
            elif kind == 'z1':
                for n in it[3]:
                    acc = z_dot(get_xn(it[2]), n)
                    z1_v[it[1], :, n * TN:(n + 1) * TN] = _gelu(acc).astype(bf16)
                    mxu([acc])
            elif kind == 'z2':
                for n in it[3]:
                    acc = z_dot(get_xn(it[2]), NCH + n)
                    it[1][0][it[1][1], 0:TM, n * TN:(n + 1) * TN] = _gelu(acc)
                    mxu([acc])
            elif kind == 'inv':
                mxu(inv(it[1], z[1] if it[2] else 0))
            elif kind == 'fwh':
                mxu(fw_h(it[1]))
            elif kind == 'fwk':
                mxu(fw_k(it[1], z[1] if it[2] else 0))
            elif kind == 'g':
                if c.get('wt') is not it[1]:
                    c['wt'], c['ws'] = it[1], wsp[it[1]]
                ws = c['ws']
                bbt = _wide(bb_v[it[1]], TN)
                for n in it[3]:
                    acc = jnp.dot(ws, _h(it[2][:, n * TN:(n + 1) * TN]), preferred_element_type=f32)
                    u = (z1_v[it[1], :, n * TN:(n + 1) * TN].astype(f32) * (acc + bbt)).astype(bf16)
                    u = pltpu.bitcast(u, u32)
                    if n < NCH - 1:
                        ua[0, :, n * TN:(n + 1) * TN] = u
                    else:
                        ub[0] = u
                    mxu([acc])
            elif kind == 'o':
                u = _h(jnp.concatenate([ua[z[1]], ub[z[1]]], axis=1))
                for n in range(D // TN):
                    acc = jnp.dot(u, wout[:, n * TN:(n + 1) * TN], preferred_element_type=f32)
                    x2 = (zp if it[2] is None else x_v)[it[1], 0:TM, n * TN:(n + 1) * TN] + acc
                    if it[2] is None:
                        z1_v[it[1], :, n * TN:(n + 1) * TN] = x2.astype(bf16)
                        if n == it[3]:
                            it[4].start()
                    else:
                        xa[it[2], 0:TM, n * TN:(n + 1) * TN] = x2
                    mxu([acc])
            elif kind == 'xn':
                release(it[1])
                for r in R:
                    xn_v[it[3], r // 2:(r + LR) // 2] = pltpu.bitcast(
                        norm(it[1][it[2] + z[0], r:r + LR], 2, r, LR).astype(bf16), u32)
                c['xn'][id(it[3])] = pltpu.bitcast(xn_v[it[3] + z[1]], bf16)
                if it[4]:
                    c['vals'].append(pltpu.bitcast(xn_v[it[3] + z[6], 0:8, 0:128], f32))
            elif kind == 'z2n':
                release(it[2][0])
                for r in R:
                    it[3][tile_rows(it[1], r // 2, LR // 2), :] = pltpu.bitcast(
                        norm(it[2][0][it[2][1] + z[0], r:r + LR], it[4], r, LR).astype(bf16), u32)
                c['vals'].append(pltpu.bitcast(it[3][tile_rows(it[1] + z[6], 0, 8), 0:128], f32))
            elif kind == 'qstat':
                qb[0, TM:TM + 16, 0:128] = b16(sg)
                for r in R:
                    stat_part(qb[it[1] % 2 + z[0], r:r + LR].astype(f32), 0, r, LR)
            elif kind == 'zstat':
                release(it[1][0])
                for r in range(0, TM, 8):
                    stat_part(it[1][0][it[1][1] + z[0], r:r + 8], 2, r, 8)
            elif kind == 'x1':
                if it[2]:
                    qb[0, TM:TM + 16, 0:128] = b16(sg)
                for r in R:
                    x0 = qb[it[1] % 2 + (z[0] if it[2] else 0), r:r + LR].astype(f32)
                    x1 = x0 + norm(x0, 0, r, LR) * y_v[it[1] + (0 if it[2] else z[1]), r:r + LR]
                    x_v[it[1], r:r + LR] = x1
                    stat_part(x1, 0, r, LR)
            elif kind == 'x2stat':
                release(xa)
                for r in R:
                    stat_part(xa[it[1] + z[0], r:r + LR], 4, r, LR)
            elif kind == 'x3':
                release(xa)
                for r in R:
                    x0 = xa[it[2] + z[0], r:r + LR]
                    x1 = x0 + norm(x0, 0, r, LR) * y_v[it[1], r:r + LR]
                    zp[it[1], r:r + LR] = x1
                    stat_part(x1, 0, r, LR)
            elif kind == 'kvprep':
                kb[0, B:B + 16, 0:128] = b16(sg)
                kvprep(it[1], z[0])
                if not it[2]:
                    c['vals'].append(lead(kvb, (2 * it[1]) % 4 + z[6]))
            elif kind == 'terms':
                c['vals'] += probe(run_tasks(it[1], sg, z[0]), z[6])
            elif kind == 'mean' or kind == 'rstd':
                gate = corner(c['acc'])
                if len(it) > 2:
                    for v in c['vals']:
                        gate = gate + v
                    c['vals'] = []
                ps[PG, 8 * c['ng']:8 * c['ng'] + 8] = gate
                c['ng'] += 1
                for (i, j, w) in it[1]:
                    (stat_mean if kind == 'mean' else stat_rstd)(i, j, w, z[1 + c['ng']])
            elif kind == 'bb':
                bs16 = bspb[...].astype(f32)
                for i in range(S // 128):
                    bb_v[i // 2, (i % 2) * 128:(i % 2 + 1) * 128, :] = jnp.transpose(
                        jnp.broadcast_to(bs16[i:i + 1, :], (128, 128)))
        if c['vals']:
            ps[PG, 64:72] = sync([c['acc'][0:8, 0:128]] + c['vals'])

    def run(name, items, cond=None):
        with jax.named_scope(name):
            pl.when(zs[15] == 0 if cond is None else cond)(lambda: block(items))

    SQ, SX, SZ, S2, SL = (0, 0, D), (0, 2, D), (2, 4, FH), (4, 0, D), (2, 6, FH)
    Z0 = (zt[0], 0)
    ALL = list(range(NCH))

    def block_p0():
        kvprep(0, 0)

    def block_p1():
        fw_k(0, 0)
        fw_h(0)

    def block_p2():
        z = [zs[j] for j in range(4)]
        sg = fw_h(1)[0][0:8, 0:128]
        run_tasks(term_tasks([(0, [0], True, True), (1, [0, 1], True, True)], 0), sg, z[1])
        qb[0, TM:TM + 16, 0:128] = b16(sg)
        for r in R:
            stat_part(qb[z[1], r:r + LR].astype(f32), 0, r, LR)
        stat_mean(0, 0, D, z[2])
        inv(0, z[0])
        stat_rstd(0, 0, D, z[3])

    def block_p3():
        kvprep(1, 0)
        fw_k(1, zs[0])
        for r in R:
            x0 = qb[0, r:r + LR].astype(f32)
            x1 = x0 + norm(x0, 0, r, LR) * y_v[0, r:r + LR]
            x_v[0, r:r + LR] = x1
            xn_v[0, r // 2:(r + LR) // 2] = pltpu.bitcast(_ln(x1).astype(bf16), u32)

    for name, waits, fn, nxt in (
            ('P0', ((0, 0), (1, 0)), block_p0, [pair_copy(3, 0), pair_copy(2, 1)]),
            ('P1', ((2, 0),), block_p1, [pair_copy(0, 1), pair_copy(1, 1)]),
            ('P2', ((3, 0), (2, 1)), block_p2, [w_copy(0)]),
            ('P3', ((0, 1), (1, 1)), block_p3, [pair_copy(3, 1), w_copy(1)])):
        issue(*nxt)
        for (j, p) in waits:
            pair_copy(j, p).wait()
        with jax.named_scope(name):
            pl.when(zs[15] == 0)(fn)

    for t in range(NT):
        conv = t < NT - 1
        ta = term_tasks(plan[('A', t)], -1) if conv else []
        tb = term_tasks(plan[('B', t)], -1) if conv else []
        if t == 0:
            ch = split_tasks(ta, [3, 1.5, 2])
            issue(w_copy(2))
            w_copy(0).wait()
            run('A0a', [('kick',), ('terms', ch[0]), ('z2', Z0, 0, [0, 1, 2])])
            issue(pair_copy(0, 2), pair_copy(1, 2), pair_copy(2, 2))
            pair_copy(3, 1).wait()
            w_copy(1).wait()
            run('A0b', [('kick',), ('qstat', 1), ('terms', ch[1]), ('z2', Z0, 0, [3]), ('mean', [SQ]),
                        ('z2', Z0, 0, [4])])
            issue(w_copy(3))
            w_copy(2).wait()
            run('A0c', [('kick',), ('rstd', [SQ]), ('terms', ch[2]), ('z2', Z0, 0, [5, 6])])
            issue(w_copy(4))
            for j in range(3):
                pair_copy(j, 2).wait()
            run('B0a', [('inv', 1, 0), ('kvprep', 2, 1), ('fwh', 2), ('fwk', 2, 1)])
            issue(w_copy(5), pair_copy(3, 2), pair_copy(0, 3), pair_copy(1, 3))
            w_copy(3).wait()
            run('B0b', [('kick',), ('zstat', Z0), ('x1', 1, 1), ('z1', 0, 0, [0, 1]), ('mean', [SX, SZ]),
                        ('z1', 0, 0, [2])])
            w_copy(4).wait()
            run('B0c', [('kick',), ('rstd', [SX, SZ]), ('terms', tb), ('bb',), ('z1', 0, 0, [3, 4, 5])])
            w_copy(5).wait()
            continue
        if t + 2 < NT:
            issue(pair_copy(2, t + 2), pair_copy(3, t + 2))
        if t + 3 < NT:
            issue(pair_copy(0, t + 3), pair_copy(1, t + 3))
        if t > 1:
            issue_big(2 * t - 3)
        if conv:
            pair_copy(3, t + 1).wait()
        if t + 2 < NT and t > 1:
            pair_copy(0, t + 2).wait()
            pair_copy(1, t + 2).wait()
        s0, s1 = t % 2, (t - 1) % 2
        za, zo = (zt[s0], 0), (zt[s1], 0)
        items = [('z1', t - 1, s1, [NCH - 1 if conv else NCH - 2]), ('xn', x_v, t, s0, 0), ('z2n', t - 1, zo, z2a, 4)]
        if conv:
            items += [('qstat', t + 1)]
            if t + 2 < NT and t > 1:
                items += [('kvprep', t + 2, 0)]
            items += [('terms', ta), ('z2', za, s0, ALL[:4]), ('mean', [SQ]), ('z2', za, s0, ALL[4:5]),
                      ('rstd', [SQ]), ('z2', za, s0, ALL[5:])]
        else:
            items += [('z2', za, s0, ALL)]
        run('A%d' % t, items)
        if conv:
            issue_big(2 * t - 2)
        if t == 1:
            pair_copy(0, t + 2).wait()
            pair_copy(1, t + 2).wait()
        if t + 2 < NT:
            pair_copy(2, t + 2).wait()
        if conv:
            items = [('inv', t + 1, 0), ('zstat', za), ('x1', t + 1, 0)]
            if t == 1:
                items += [('kvprep', t + 2, 1)]
            items += [('terms', tb)]
            if t + 2 < NT:
                items += [('fwh', t + 2)]
            if t + 2 < NT and t > 1:
                items += [('fwk', t + 2, 0)]
            if t + 2 < NT:
                items += [('z1', t, s0, ALL[:2]), ('mean', [SZ]), ('z1', t, s0, ALL[2:3]), ('mean', [SX]),
                          ('z1', t, s0, ALL[3:4]), ('rstd', [SZ])]
                if t == 1:
                    items += [('fwk', t + 2, 1)]
                items += [('z1', t, s0, ALL[4:5]), ('rstd', [SX]), ('z1', t, s0, ALL[5:6])]
            else:
                items += [('z1', t, s0, ALL[:2]), ('mean', [SZ]), ('z1', t, s0, ALL[2:3]), ('mean', [SX]),
                          ('rstd', [SZ]), ('z1', t, s0, ALL[3:4]), ('rstd', [SX]), ('z1', t, s0, ALL[4:5])]
            run('B%d' % t, items)
        else:
            run('B7a', [('kick',), ('zstat', za), ('z1', t, s0, [0]), ('mean', [SZ]), ('z1', t, s0, [1]),
                        ('rstd', [SZ]), ('z1', t, s0, [2])])
            run('B7b', [('kick',), ('z2n', t, za, z2a, 4), ('z1', t - 1, s1, [NCH - 1])])

    for cp in big[-2:]:
        cp.wait()

    def stage_c(full, i, carry):
        p0 = lax.rem(i, 2)
        p1 = 1 - p0
        fx = [('x3', jnp.maximum(i - 2, 0), p0), ('x2stat', p1)]
        if not full:
            run('V1', [('g', i, z2a, ALL[:1])] + fx + [('g', i, z2a, ALL[1:3]), ('mean', [SX]),
                       ('g', i, z2a, ALL[3:4]), ('mean', [S2]), ('g', i, z2a, ALL[4:5]), ('rstd', [SX]),
                       ('g', i, z2a, ALL[5:6]), ('rstd', [S2]), ('g', i, z2a, ALL[6:]), ('o', i, p0)])
            return carry
        t4 = lax.rem(i + NT - 4, NT)
        run('V2', [('g', i, z2a, ALL[:1]), ('xn', zp, i - 3, p1, 1)] + fx
            + [('z2n', jnp.maximum(i - 5, 0), (zc, p1), z2b, 4), ('zstat', (zc, p0)),
               ('g', i, z2a, ALL[1:5]), ('mean', [SX], 1), ('g', i, z2a, ALL[5:6]), ('mean', [SZ]),
               ('g', i, z2a, ALL[6:]), ('mean', [S2]), ('z1', t4, p0, ALL[3:4]), ('rstd', [SX]),
               ('z1', t4, p0, ALL[4:5]), ('rstd', [SZ]), ('z1', t4, p0, ALL[5:6]), ('rstd', [S2]),
               ('z1', t4, p0, ALL[6:]), ('z1', i - 3, p1, ALL[:3]), ('z2', (zc, p1), p1, ALL), ('o', i, p0)])
        return carry

    def stage_d(t, carry):
        @pl.when(t >= 2)
        def _():
            for j in range(3):
                out_copy(t - 2, j).wait()

        t0, t1 = 2 * t, 2 * t + 1
        run('D', [('g', t0, z2b, ALL), ('o', t0, None, D // TN - 1, out_copy(t, 0)),
                  ('g', t1, z2b, ALL), ('o', t1, None, OS - 1, out_copy(t, 1))])
        out_copy(t, 2).start()
        return carry

    lax.fori_loop(0, 3, functools.partial(stage_c, False), 0)
    lax.fori_loop(3, NT, functools.partial(stage_c, True), 0)
    zbuf = {3: (zc, 1), 4: (zc, 0), 5: (zt[0], 0), 6: (zt[1], 0), 7: (zc, 0)}
    for i in range(NT, NT + 3):
        p0, p1 = i % 2, (i + 1) % 2
        sz_old, sz_new = (SZ, SL) if p0 == 0 else (SL, SZ)
        items = [('z1', i - 4, p0, ALL[3:4]), ('xn', zp, i - 3, p1, 0), ('z2n', i - 5, zbuf[i - 5], z2b, sz_old[1]),
                 ('zstat', zbuf[i - 4])]
        stats = [sz_new]
        if i - 2 < NT:
            items += [('x3', i - 2, p0)]
            stats += [SX]
        if i - 1 < NT:
            items += [('x2stat', p1)]
            stats += [S2]
        items += [('z1', i - 4, p0, ALL[4:]), ('z1', i - 3, p1, ALL[:3])]
        gates = [('mean', [x]) for x in stats] + [('rstd', [x]) for x in stats]
        for n in ALL:
            items += gates[n:n + 1] + [('z2', zbuf[i - 3], p1, [n])]
        run('V3%d' % i, items)
    t = NT - 1
    run('T1', [('kick',), ('zstat', zbuf[t]), ('z2n', t - 1, zbuf[t - 1], z2b, SL[1]), ('z1', t, 1, [3]),
               ('mean', [SZ]), ('z1', t, 1, [4]), ('rstd', [SZ]), ('z1', t, 1, [5])])
    run('T2', [('kick',), ('z2n', t, zbuf[t], z2b, SZ[1]), ('z1', t, 1, [6])])
    lax.fori_loop(0, NT // 2, stage_d, 0)
    for t in range(NT // 2 - 2, NT // 2):
        for j in range(3):
            out_copy(t, j).wait()


@jax.jit
def pallas_interleave_layers__ssm_conv_h3__mixer_gmlp__prompt_kernel(
        A_q, A_k, A_v, A_shift_k, A_ssm_k, A_ssm_D, B_x, B_w_in, B_w_sp, B_b_sp, B_w_out):
    del B_x
    any_spec = pl.BlockSpec(memory_space=pl.ANY)
    scratch = [
        pltpu.VMEM((2, TM + 16, D), bf16),
        pltpu.VMEM((8, B + 16, D), bf16),
        pltpu.VMEM((8, B, D), bf16),
        pltpu.VMEM((2, D, TM), bf16),
        pltpu.VMEM((D, F), bf16),
        pltpu.VMEM((NT, TM, S), bf16),
        pltpu.VMEM((FH, D), bf16),
        pltpu.VMEM((KS, D), bf16),
        pltpu.VMEM((8, 128), bf16),
        pltpu.VMEM((16, 128), bf16),
        pltpu.VMEM((NT, TM + 8, D), f32),
        pltpu.VMEM((NT, TM, D), f32),
        pltpu.VMEM((NT, TM, FH), bf16),
        pltpu.VMEM((S // 2, FH), u32),
        pltpu.VMEM((S // 2, FH), u32),
        pltpu.VMEM((NT, TM, 128), f32),
        pltpu.VMEM((KS + 1, 8, D), f32),
        pltpu.VMEM((2 * B, B), bf16),
        pltpu.VMEM((B, 2 * B), bf16),
        pltpu.VMEM((4, B, D), bf16),
        [pltpu.VMEM((2, 2 * B + 8, D), f32)] * NT,
        [pltpu.VMEM((2, 2 * B + 8, D), f32)] * NT,
        pltpu.VMEM((1, TM, D), f32),
        pltpu.VMEM((NZ, 2 * B + 8, D), f32),
        pltpu.VMEM((2, 2 * B, D), bf16),
        pltpu.VMEM((2, TM // 2, D), u32),
        [pltpu.VMEM((1, TM + 8, FH), f32)] * 2,
        pltpu.VMEM((2, TM + 8, FH), f32),
        pltpu.VMEM((2, TM + 8, D), f32),
        pltpu.VMEM((7, TM, 128), f32),
        pltpu.VMEM((8, TM, 128), f32),
        pltpu.VMEM((1, TM // 2, FH - TN), u32),
        pltpu.VMEM((1, TM // 2, TN), u32),
        pltpu.SMEM((16,), jnp.int32),
        pltpu.SemaphoreType.DMA((8,)),
        pltpu.SemaphoreType.DMA((3,)),
        pltpu.SemaphoreType.DMA((2,)),
        pltpu.SemaphoreType.DMA((6,)),
    ]
    out = pl.pallas_call(
        _kernel,
        out_shape=jax.ShapeDtypeStruct((NT, TM, D), bf16),
        in_specs=[any_spec] * 10,
        out_specs=any_spec,
        scratch_shapes=scratch,
        compiler_params=pltpu.CompilerParams(vmem_limit_bytes=127 * 1024 * 1024),
    )(A_q.reshape(NT, TM, D), A_k.reshape(NB, B, D), A_v.reshape(NB, B, D), A_shift_k.T, A_ssm_k,
      A_ssm_D.reshape(8, 128), B_w_in, B_w_sp.reshape(NT, TM, S), B_b_sp.reshape(16, 128), B_w_out)
    return out.reshape(1, S, D)
```

```python
import functools
import math
import jax
import jax.numpy as jnp
from jax import lax
import jax.experimental.pallas as pl
import jax.experimental.pallas.tpu as pltpu

S = 2048
D = 1024
F = 3584
FH = F // 2
KS = 4
B = 128
NB = S // B
EPS = 1e-5
f32 = jnp.float32
bf16 = jnp.bfloat16
u32 = jnp.uint32

TM = 256
NT = S // TM
TN = 256
NCH = FH // TN
RG = 16
GW = 256
LR = 16
NZ = 8
CAP_A = 9
CAP_B = 14
GWF = 128
OS = 3
ROT = 256


def _plan(cap_a, cap_b):
    done = set((a, ap) for a in (0, 1) for ap in range(a + 1))
    blocks = {}
    for t in range(NT - 1):
        for kind, cap in (('A', cap_a), ('B', cap_b)):
            sel = {}
            n = 0
            lo = 2 * t + 2 if kind == 'A' else 2 * t + 4
            lim = 2 * t + 3
            for a in range(lo, NB):
                g = [ap for ap in range(a + 1) if (a, ap) not in done and ap <= lim and a - ap <= lim]
                if a > lim:
                    g = g[:max(cap - n, 0)]
                if g:
                    sel[a] = g
                    n += len(g)
            groups = []
            for a in sorted(sel):
                first = not any((a, x) in done for x in range(a + 1))
                done.update((a, x) for x in sel[a])
                last = all((a, x) in done for x in range(a + 1))
                assert a < lo + NZ and last == (a <= 2 * t + 3)
                groups.append((a, sel[a], first, last))
            blocks[(kind, t)] = groups
    assert len(done) == NB * (NB + 1) // 2
    return blocks


def _gelu(x):
    u = x * (0.7978845608028654 + 0.035677408136300125 * (x * x))
    h = 0.5 * x
    return h + h * jnp.tanh(u)


def _h(v):
    return pltpu.bitcast(v, bf16)


def _part(v):
    acc = v[:, 0:128]
    for c in range(128, v.shape[1], 128):
        acc = acc + v[:, c:c + 128]
    return acc


def _lsum(acc):
    return jnp.broadcast_to(jnp.sum(acc, axis=1, keepdims=True), acc.shape)


def _wide(v, n):
    return jnp.concatenate([v] * (n // 128), axis=1)


def _ln(x):
    n = x.shape[-1]
    m = jnp.sum(x, axis=-1, keepdims=True) * (1.0 / n)
    xc = x - m
    v = jnp.sum(xc * xc, axis=-1, keepdims=True) * (1.0 / n)
    return xc * lax.rsqrt(v + EPS)


def _dft_rows(shape, row_dim):
    r = lax.broadcasted_iota(jnp.int32, shape, row_dim)
    n = lax.broadcasted_iota(jnp.int32, shape, 1 - row_dim)
    is_im = r >= B
    rr = jnp.where(is_im, r - B, r)
    odd = rr >= B // 2
    fidx = jnp.where(odd, 2 * (rr - B // 2) + 1, 2 * rr)
    m = (2 * fidx + 1) * n - jnp.where(is_im, B, 0)
    m = jnp.bitwise_and(m, 4 * B - 1)
    m = jnp.where(m > 2 * B, 4 * B - m, m)
    return jnp.cos(m.astype(f32) * (math.pi / (2 * B)))


NT_DIMS = (((1,), (1,)), ((), ()))


def _kernel(q_hbm, k_hbm, v_hbm, sk_hbm, h_hbm, sd_hbm, win_hbm, wsp_hbm, bsp_hbm, wout_hbm,
            o_hbm,
            qb, kb, vb, hb, win, wsp, wout, skb, sdb, bspb,
            x_v, y_v, z1_v, z2a, z2b, bb_v, skt, fm_v, im_v, kvb, ks, hs, wold, zp, zb,
            xn_v, zt, zc, xa, ps, st, ua, ub, zs,
            sem_c, sem_w, sem_s, sem_o):
    plan = _plan(CAP_A, CAP_B)

    def pair_copy(j, p):
        if j == 0:
            return pltpu.make_async_copy(k_hbm.at[pl.ds(2 * p, 2)], kb.at[pl.ds(2 * p % 8, 2), pl.ds(0, B)], sem_c.at[p % 2])
        if j == 1:
            return pltpu.make_async_copy(v_hbm.at[pl.ds(2 * p, 2)], vb.at[pl.ds(2 * p % 8, 2)], sem_c.at[2 + p % 2])
        if j == 2:
            cols = pl.ds(p * TM, TM)
            return pltpu.make_async_copy(h_hbm.at[:, cols], hb.at[p % 2], sem_c.at[4 + p % 2])
        return pltpu.make_async_copy(q_hbm.at[p], qb.at[p % 2, pl.ds(0, TM)], sem_c.at[6 + p % 2])

    WG = ((7, 10), (10, 12), (12, 14), (0, 3), (3, 6), (6, 7))

    def w_copy(i):
        cols = pl.ds(WG[i][0] * TN, (WG[i][1] - WG[i][0]) * TN)
        return pltpu.make_async_copy(win_hbm.at[:, cols], win.at[:, cols], sem_w.at[i % 3])

    def out_copy(t, j):
        cols = (pl.ds(0, D), pl.ds(0, OS * TN), pl.ds(OS * TN, D - OS * TN))[j]
        i = 2 * t + min(j, 1)
        return pltpu.make_async_copy(z1_v.at[i, :, cols], o_hbm.at[i, :, cols], sem_o.at[3 * (t % 2) + j])

    def issue(*copies):
        for cp in copies:
            cp.start(priority=1)

    def issue_big(j):
        if j >= 2:
            big[j - 2].wait()
        issue(big[j])

    small = [
        pltpu.make_async_copy(sk_hbm, skb, sem_o.at[0]),
        pltpu.make_async_copy(sd_hbm, sdb, sem_o.at[1]),
        pltpu.make_async_copy(bsp_hbm, bspb, sem_o.at[2]),
    ]
    WR = FH // 4
    big = ([pltpu.make_async_copy(wsp_hbm.at[j], wsp.at[j], sem_s.at[j % 2]) for j in range(NT)]
           + [pltpu.make_async_copy(wout_hbm.at[pl.ds(j * WR, WR)], wout.at[pl.ds(j * WR, WR)], sem_s.at[j % 2])
              for j in range(4)])
    for cp in small:
        cp.start()
    pair_copy(0, 0).start(priority=1)
    pair_copy(1, 0).start(priority=1)

    def zinit(i, c):
        zs[i] = 0
        return c
    lax.fori_loop(0, 16, zinit, 0)
    issue(pair_copy(2, 0))

    fm_v[...] = _dft_rows((2 * B, B), 0).astype(bf16)
    im_v[...] = (_dft_rows((B, 2 * B), 1) * (1.0 / B)).astype(bf16)

    for cp in small:
        cp.wait()
    sk4 = skb[...].astype(f32)
    for j in range(KS):
        skt[j] = jnp.broadcast_to(sk4[j:j + 1, :], (8, D))
    sd8 = sdb[...].astype(f32)
    skt[KS] = jnp.concatenate([jnp.broadcast_to(sd8[i:i + 1, :], (8, 128)) for i in range(8)], axis=1)

    def kvprep(p, z):
        for a in (2 * p, 2 * p + 1):
            for c in range(0, D, GW):
                for r0 in range(0, B, 32):
                    kcur = kb[a % 8 + z, r0:r0 + 32, c:c + GW].astype(f32)
                    if a == 0 and r0 == 0:
                        kprev = jnp.zeros((8, GW), f32)
                    elif r0 == 0:
                        kprev = kb[(a - 1) % 8 + z, B - 16:B, c:c + GW].astype(f32)[8:16]
                    else:
                        kprev = kb[a % 8 + z, r0 - 16:r0, c:c + GW].astype(f32)[8:16]
                    ext = jnp.concatenate([kprev, kcur], axis=0)
                    sk = [jnp.concatenate([skt[j, :, c:c + GW]] * 4, axis=0) for j in range(KS)]
                    acc = kcur * sk[0]
                    for j in range(1, KS):
                        acc = acc + pltpu.roll(ext, j, 0)[8:] * sk[j]
                    kvb[a % 4, r0:r0 + 32, c:c + GW] = (acc * vb[a % 8, r0:r0 + 32, c:c + GW].astype(f32)).astype(bf16)

    CW = 512

    def rot(c, k, w):
        c = (c + ROT * k) % D
        return slice(c, c + w)

    def put(ref, i, c, val, k):
        for j in range(0, CW, 256):
            ref[i, 0:B, rot(c + j, k, 256)] = val[0:B, j:j + 256]
            ref[i, B:2 * B, rot(c + j, k + 2, 256)] = val[B:2 * B, j:j + 256]

    def fw_h(p):
        fm = fm_v[...]
        res = []
        for a in (2 * p, 2 * p + 1):
            for c in range(0, D, CW):
                hh = lax.dot_general(fm, hb[p % 2, c:c + CW, (a % 2) * B:(a % 2 + 1) * B], NT_DIMS,
                                     preferred_element_type=f32)
                res.append(hh)
                if a == 0:
                    sd = jnp.concatenate([skt[KS, :, c:c + CW]] * (B // 8), axis=0)
                    hh = jnp.concatenate([hh[0:B] + sd, hh[B:2 * B]], axis=0)
                put(hs[p], a % 2, c, hh, 1)
        return res

    def fw_k(p, zk):
        fm = fm_v[...]
        res = []
        for a in (2 * p, 2 * p + 1):
            for c in range(0, D, CW):
                hh = jnp.dot(fm, kvb[a % 4 + zk, :, c:c + CW], preferred_element_type=f32)
                res.append(hh)
                put(ks[p], a % 2, c, hh, 0)
        return res

    def term_tasks(groups, newp):
        def acc(a, g, first, r, c, z, GW):
            zr = zi = None
            for ap in g:
                d = a - ap
                xr = ks[ap // 2][ap % 2 + z, r:r + RG, c:c + GW]
                xi = ks[ap // 2][ap % 2 + z, B + r:B + r + RG, rot(c, 2, GW)]
                hr = hs[d // 2][d % 2 + z, r:r + RG, rot(c, 1, GW)]
                hi = hs[d // 2][d % 2 + z, B + r:B + r + RG, rot(c, 3, GW)]
                tr = xr * hr - xi * hi
                ti = xr * hi + xi * hr
                zr = tr if zr is None else zr + tr
                zi = ti if zi is None else zi + ti
            if not first:
                zr = zr + zp[a % NZ, r:r + RG, c:c + GW]
                zi = zi + zp[a % NZ, B + r:B + r + RG, c:c + GW]
            return zr, zi

        def part_task(a, g, first, r, c, z):
            zr, zi = acc(a, g, first, r, c, z, GW)
            zp[a % NZ, r:r + RG, c:c + GW] = zr
            zp[a % NZ, B + r:B + r + RG, c:c + GW] = zi

        def fin_task(fin, r, c, z):
            GW = GWF
            if fin[0][0] > 0:
                pr = wold[0, r:r + RG, c:c + GW]
                pi = wold[0, B + r:B + r + RG, c:c + GW]
            for (a, g, first, last) in fin:
                wr, wi = acc(a, g, first, r, c, z, GW)
                if a == 0:
                    zr, zi = wr, wi
                elif r < B // 2:
                    zr, zi = wr + pi, wi - pr
                else:
                    zr, zi = wr - pi, wi + pr
                zb[a % 2, r:r + RG, c:c + GW] = zr.astype(bf16)
                zb[a % 2, B + r:B + r + RG, c:c + GW] = zi.astype(bf16)
                pr, pi = wr, wi
            if fin[-1][0] < NB - 1:
                wold[0, r:r + RG, c:c + GW] = pr
                wold[0, B + r:B + r + RG, c:c + GW] = pi

        def srcs(gs):
            return (set(('k', ap // 2) for (a, g, _, _) in gs for ap in g)
                    | set(('h', (a - ap) // 2) for (a, g, _, _) in gs for ap in g))

        rc = [(r, c) for r in range(0, B, RG) for c in range(0, D, GW)]
        tasks = []
        for grp in groups:
            a, g, first, last = grp
            if not last:
                sr = srcs([grp])
                new = any(i == newp for (_, i) in sr)
                tasks += [(len(g), new, sr, ('zp', a % NZ),
                           functools.partial(part_task, a, g, first, r, c)) for (r, c) in rc]
        tasks.sort(key=lambda x: x[1])
        fin = [x for x in groups if x[3]]
        if fin:
            tasks += [(sum(len(x[1]) for x in fin) + 1, True, srcs(fin), ('zb', 0),
                       functools.partial(fin_task, fin, r, c)) for r in range(0, B, RG) for c in range(0, D, GWF)]
        return tasks

    def split_tasks(tasks, caps):
        total = sum(x[0] for x in tasks)
        out = [[] for _ in caps]
        cum = 0
        for x in tasks:
            pos = (cum + 0.5 * x[0]) / max(total, 1) * sum(caps)
            k = 0
            while k + 1 < len(caps) and pos > sum(caps[:k + 1]):
                k += 1
            out[k].append(x)
            cum += x[0]
        return out

    def run_tasks(tasks, val, z):
        for (kind, i) in sorted(set().union(*[x[2] for x in tasks])) if tasks else []:
            (ks if kind == 'k' else hs)[i][z, 2 * B:2 * B + 8, 0:128] = val
        for x in tasks:
            x[4](0)
        probes = {}
        for x in tasks:
            probes[x[3][0]] = x[3][1]
        return probes

    def probe(probes, z):
        vals = []
        if 'zp' in probes:
            vals.append(zp[probes['zp'] + z, 0:8, 0:128])
        if 'zb' in probes:
            vals.append(zb[z, 0:16, 0:128].astype(f32)[0:8])
        return vals

    def sync(vals):
        v = vals[0]
        for w in vals[1:]:
            v = v + w
        return _lsum(v)

    def inv(p, z):
        im = im_v[...]
        res = []
        for d in range(2):
            for c in range(0, D, CW):
                y = jnp.dot(im, zb[d + z, :, c:c + CW], preferred_element_type=f32)
                res.append(y)
                y_v[p, d * B:(d + 1) * B, c:c + CW] = y
        return res

    R = range(0, TM, LR)

    def corner(acc):
        return acc[acc.shape[0] - 8:, acc.shape[1] - 128:]

    def b16(v):
        return jnp.concatenate([v, v], axis=0).astype(bf16)

    def stat_part(x, i, r, n):
        w = x.shape[1]
        mu = _part(x) * (128.0 / w)
        dv = x - _wide(mu, w)
        ps[i, r:r + n] = mu
        ps[i + 1, r:r + n] = _part(dv * dv)

    def stat_mean(i, j, w, z):
        mu = ps[i + z]
        m = _lsum(mu) * (1.0 / 128)
        st[j] = m
        e = mu - m
        ps[i] = ps[i + 1 + z] + (w / 128.0) * (e * e)

    def stat_rstd(i, j, w, z):
        st[j + 1] = lax.rsqrt(_lsum(ps[i + z]) * (1.0 / w) + EPS)

    def norm(x, j, r, n):
        w = x.shape[1]
        return (x - _wide(st[j, r:r + n], w)) * _wide(st[j + 1, r:r + n], w)

    PG = 6

    def z_dot(xn, n):
        return jnp.dot(xn, win[:, n * TN:(n + 1) * TN], preferred_element_type=f32)

    def kick():
        return jnp.dot(fm_v[0:16, :], fm_v[0:128, :], preferred_element_type=f32)

    def lead(ref, i):
        return ref[i, 0:16, 0:128].astype(f32)[0:8]

    def tile_rows(t, r, n):
        if isinstance(t, int):
            return slice(t * TM // 2 + r, t * TM // 2 + r + n)
        return pl.ds(pl.multiple_of(t * (TM // 2) + r, 8), n)

    def block(items):
        z = [zs[j] for j in range(8)]
        c = dict(sg=None, acc=None, vals=[], xn={}, ng=0, rel=[])

        def release(ref):
            if not any(ref is x for x in c['rel']):
                c['rel'].append(ref)
                ref[z[0], TM:TM + 8, 0:128] = c['sg']

        def mxu(res):
            if c['sg'] is None:
                c['sg'] = res[0][0:8, 0:128]
            c['acc'] = res[-1]

        def get_xn(i):
            if id(i) not in c['xn']:
                c['xn'][id(i)] = pltpu.bitcast(xn_v[i, 0:TM // 2], bf16)
            return c['xn'][id(i)]

        for it in items:
            kind = it[0]
            sg = c['sg']
            if kind == 'kick':
                mxu([kick()])
            elif kind == 'z1':
                for n in it[3]:
                    acc = z_dot(get_xn(it[2]), n)
                    z1_v[it[1], :, n * TN:(n + 1) * TN] = _gelu(acc).astype(bf16)
                    mxu([acc])
            elif kind == 'z2':
                for n in it[3]:
                    acc = z_dot(get_xn(it[2]), NCH + n)
                    it[1][0][it[1][1], 0:TM, n * TN:(n + 1) * TN] = _gelu(acc)
                    mxu([acc])
            elif kind == 'inv':
                mxu(inv(it[1], z[1] if it[2] else 0))
            elif kind == 'fwh':
                mxu(fw_h(it[1]))
            elif kind == 'fwk':
                mxu(fw_k(it[1], z[1] if it[2] else 0))
            elif kind == 'g':
                if c.get('wt') is not it[1]:
                    c['wt'], c['ws'] = it[1], wsp[it[1]]
                ws = c['ws']
                bbt = _wide(bb_v[it[1]], TN)
                for n in it[3]:
                    acc = jnp.dot(ws, _h(it[2][:, n * TN:(n + 1) * TN]), preferred_element_type=f32)
                    u = (z1_v[it[1], :, n * TN:(n + 1) * TN].astype(f32) * (acc + bbt)).astype(bf16)
                    u = pltpu.bitcast(u, u32)
                    if n < NCH - 1:
                        ua[0, 0:TM // 2, n * TN:(n + 1) * TN] = u
                    else:
                        ub[0, 0:TM // 2] = u
                    mxu([acc])
            elif kind == 'o':
                ua[z[1], TM // 2:TM // 2 + 8, 0:128] = pltpu.bitcast(sg, u32)
                ub[z[1], TM // 2:TM // 2 + 8, 0:128] = pltpu.bitcast(sg, u32)
                u = _h(jnp.concatenate([ua[0, 0:TM // 2], ub[0, 0:TM // 2]], axis=1))
                for n in range(D // TN):
                    acc = jnp.dot(u, wout[:, n * TN:(n + 1) * TN], preferred_element_type=f32)
                    x2 = (zp if it[2] is None else x_v)[it[1], 0:TM, n * TN:(n + 1) * TN] + acc
                    if it[2] is None:
                        z1_v[it[1], :, n * TN:(n + 1) * TN] = x2.astype(bf16)
                        if n == it[3]:
                            it[4].start()
                    else:
                        xa[it[2], 0:TM, n * TN:(n + 1) * TN] = x2
                    mxu([acc])
            elif kind == 'xn':
                release(it[1])
                for r in R:
                    xn_v[it[3], r // 2:(r + LR) // 2] = pltpu.bitcast(
                        norm(it[1][it[2], r:r + LR], 2, r, LR).astype(bf16), u32)
                xn_v[z[1], TM // 2:TM // 2 + 8, 0:128] = pltpu.bitcast(sg, u32)
                c['xn'] = {}
                if it[4]:
                    c['vals'].append(pltpu.bitcast(xn_v[it[3] + z[6], 0:8, 0:128], f32))
            elif kind == 'z2n':
                release(it[2][0])
                for r in R:
                    it[3][tile_rows(it[1], r // 2, LR // 2), :] = pltpu.bitcast(
                        norm(it[2][0][it[2][1], r:r + LR], it[4], r, LR).astype(bf16), u32)
                c['vals'].append(pltpu.bitcast(it[3][tile_rows(it[1] + z[6], 0, 8), 0:128], f32))
            elif kind == 'qstat':
                qb[z[0], TM:TM + 16, 0:128] = b16(sg)
                for r in R:
                    stat_part(qb[it[1] % 2, r:r + LR].astype(f32), 0, r, LR)
            elif kind == 'zstat':
                release(it[1][0])
                for r in range(0, TM, 8):
                    stat_part(it[1][0][it[1][1], r:r + 8], 2, r, 8)
            elif kind == 'x1':
                if it[2]:
                    qb[z[0], TM:TM + 16, 0:128] = b16(sg)
                for r in R:
                    x0 = qb[it[1] % 2, r:r + LR].astype(f32)
                    x1 = x0 + norm(x0, 0, r, LR) * y_v[it[1] + (0 if it[2] else z[1]), r:r + LR]
                    x_v[it[1], r:r + LR] = x1
                    stat_part(x1, 0, r, LR)
            elif kind == 'x2stat':
                release(xa)
                for r in R:
                    stat_part(xa[it[1], r:r + LR], 4, r, LR)
            elif kind == 'x3':
                release(xa)
                for r in R:
                    x0 = xa[it[2], r:r + LR]
                    x1 = x0 + norm(x0, 0, r, LR) * y_v[it[1], r:r + LR]
                    zp[it[1], r:r + LR] = x1
                    stat_part(x1, 0, r, LR)
            elif kind == 'kvprep':
                kb[z[0], B:B + 16, 0:128] = b16(sg)
                kvprep(it[1], 0)
                if not it[2]:
                    c['vals'].append(lead(kvb, (2 * it[1]) % 4 + z[6]))
            elif kind == 'terms':
                c['vals'] += probe(run_tasks(it[1], sg, z[0]), z[6])
            elif kind == 'mean' or kind == 'rstd':
                gate = corner(c['acc'])
                if len(it) > 2:
                    for v in c['vals']:
                        gate = gate + v
                    c['vals'] = []
                ps[PG + z[2], 8 * c['ng']:8 * c['ng'] + 8] = gate
                c['ng'] += 1
                for (i, j, w) in it[1]:
                    (stat_mean if kind == 'mean' else stat_rstd)(i, j, w, 0)
            elif kind == 'bb':
                bs16 = bspb[...].astype(f32)
                for i in range(S // 128):
                    bb_v[i // 2, (i % 2) * 128:(i % 2 + 1) * 128, :] = jnp.transpose(
                        jnp.broadcast_to(bs16[i:i + 1, :], (128, 128)))
        if c['vals']:
            ps[PG, 64:72] = sync([c['acc'][0:8, 0:128]] + c['vals'])

    def run(name, items, cond=None):
        with jax.named_scope(name):
            pl.when(zs[15] == 0 if cond is None else cond)(lambda: block(items))

    SQ, SX, SZ, S2, SL = (0, 0, D), (0, 2, D), (2, 4, FH), (4, 0, D), (2, 6, FH)
    Z0 = (zt[0], 0)
    ALL = list(range(NCH))

    def block_p0():
        kvprep(0, 0)

    def block_p1():
        fw_k(0, 0)
        fw_h(0)

    def block_p2():
        z = [zs[j] for j in range(4)]
        sg = fw_h(1)[0][0:8, 0:128]
        run_tasks(term_tasks([(0, [0], True, True), (1, [0, 1], True, True)], 0), sg, z[1])
        qb[0, TM:TM + 16, 0:128] = b16(sg)
        for r in R:
            stat_part(qb[z[1], r:r + LR].astype(f32), 0, r, LR)
        stat_mean(0, 0, D, z[2])
        inv(0, z[0])
        stat_rstd(0, 0, D, z[3])

    def block_p3():
        kvprep(1, 0)
        fw_k(1, zs[0])
        for r in R:
            x0 = qb[0, r:r + LR].astype(f32)
            x1 = x0 + norm(x0, 0, r, LR) * y_v[0, r:r + LR]
            x_v[0, r:r + LR] = x1
            xn_v[0, r // 2:(r + LR) // 2] = pltpu.bitcast(_ln(x1).astype(bf16), u32)

    for name, waits, fn, nxt in (
            ('P0', ((0, 0), (1, 0)), block_p0, [pair_copy(3, 0), pair_copy(2, 1)]),
            ('P1', ((2, 0),), block_p1, [pair_copy(0, 1), pair_copy(1, 1)]),
            ('P2', ((3, 0), (2, 1)), block_p2, [w_copy(0)]),
            ('P3', ((0, 1), (1, 1)), block_p3, [pair_copy(3, 1), w_copy(1)])):
        issue(*nxt)
        for (j, p) in waits:
            pair_copy(j, p).wait()
        with jax.named_scope(name):
            pl.when(zs[15] == 0)(fn)

    for t in range(NT):
        conv = t < NT - 1
        ta = term_tasks(plan[('A', t)], -1) if conv else []
        tb = term_tasks(plan[('B', t)], -1) if conv else []
        if t == 0:
            ch = split_tasks(ta, [3, 1.5, 2])
            issue(w_copy(2))
            w_copy(0).wait()
            run('A0a', [('kick',), ('terms', ch[0]), ('z2', Z0, 0, [0, 1, 2])])
            issue(pair_copy(0, 2), pair_copy(1, 2), pair_copy(2, 2))
            pair_copy(3, 1).wait()
            w_copy(1).wait()
            run('A0b', [('kick',), ('qstat', 1), ('terms', ch[1]), ('z2', Z0, 0, [3]), ('mean', [SQ]),
                        ('z2', Z0, 0, [4])])
            issue(w_copy(3))
            w_copy(2).wait()
            run('A0c', [('kick',), ('rstd', [SQ]), ('terms', ch[2]), ('z2', Z0, 0, [5, 6])])
            issue(w_copy(4))
            for j in range(3):
                pair_copy(j, 2).wait()
            run('B0a', [('inv', 1, 0), ('kvprep', 2, 1), ('fwh', 2), ('fwk', 2, 1)])
            issue(w_copy(5), pair_copy(3, 2), pair_copy(0, 3), pair_copy(1, 3))
            w_copy(3).wait()
            run('B0b', [('kick',), ('zstat', Z0), ('x1', 1, 1), ('z1', 0, 0, [0, 1]), ('mean', [SX, SZ]),
                        ('z1', 0, 0, [2])])
            w_copy(4).wait()
            run('B0c', [('kick',), ('rstd', [SX, SZ]), ('terms', tb), ('bb',), ('z1', 0, 0, [3, 4, 5])])
            w_copy(5).wait()
            continue
        if t + 2 < NT:
            issue(pair_copy(2, t + 2), pair_copy(3, t + 2))
        if t + 3 < NT:
            issue(pair_copy(0, t + 3), pair_copy(1, t + 3))
        if t > 1:
            issue_big(2 * t - 3)
        if conv:
            pair_copy(3, t + 1).wait()
        if t + 2 < NT and t > 1:
            pair_copy(0, t + 2).wait()
            pair_copy(1, t + 2).wait()
        s0, s1 = t % 2, (t - 1) % 2
        za, zo = (zt[s0], 0), (zt[s1], 0)
        items = [('z1', t - 1, s1, [NCH - 1 if conv else NCH - 2]), ('xn', x_v, t, s0, 0), ('z2n', t - 1, zo, z2a, 4)]
        if conv:
            items += [('qstat', t + 1)]
            if t + 2 < NT and t > 1:
                items += [('kvprep', t + 2, 0)]
            items += [('terms', ta), ('z2', za, s0, ALL[:4]), ('mean', [SQ]), ('z2', za, s0, ALL[4:5]),
                      ('rstd', [SQ]), ('z2', za, s0, ALL[5:])]
        else:
            items += [('z2', za, s0, ALL)]
        run('A%d' % t, items)
        if conv:
            issue_big(2 * t - 2)
        if t == 1:
            pair_copy(0, t + 2).wait()
            pair_copy(1, t + 2).wait()
        if t + 2 < NT:
            pair_copy(2, t + 2).wait()
        if conv:
            items = [('inv', t + 1, 0), ('zstat', za), ('x1', t + 1, 0)]
            if t == 1:
                items += [('kvprep', t + 2, 1)]
            items += [('terms', tb)]
            if t + 2 < NT:
                items += [('fwh', t + 2)]
            if t + 2 < NT and t > 1:
                items += [('fwk', t + 2, 0)]
            if t + 2 < NT:
                items += [('z1', t, s0, ALL[:2]), ('mean', [SZ]), ('z1', t, s0, ALL[2:3]), ('mean', [SX]),
                          ('z1', t, s0, ALL[3:4]), ('rstd', [SZ])]
                if t == 1:
                    items += [('fwk', t + 2, 1)]
                items += [('z1', t, s0, ALL[4:5]), ('rstd', [SX]), ('z1', t, s0, ALL[5:6])]
            else:
                items += [('z1', t, s0, ALL[:2]), ('mean', [SZ]), ('z1', t, s0, ALL[2:3]), ('mean', [SX]),
                          ('rstd', [SZ]), ('z1', t, s0, ALL[3:4]), ('rstd', [SX]), ('z1', t, s0, ALL[4:5])]
            run('B%d' % t, items)
        else:
            run('B7a', [('kick',), ('zstat', za), ('z1', t, s0, [0]), ('mean', [SZ]), ('z1', t, s0, [1]),
                        ('rstd', [SZ]), ('z1', t, s0, [2])])
            run('B7b', [('kick',), ('z2n', t, za, z2a, 4), ('z1', t - 1, s1, [NCH - 1])])

    for cp in big[-2:]:
        cp.wait()

    def stage_c(full, i, carry):
        p0 = lax.rem(i, 2)
        p1 = 1 - p0
        fx = [('x3', jnp.maximum(i - 2, 0), p0), ('x2stat', p1)]
        if not full:
            run('V1', [('g', i, z2a, ALL[:1])] + fx + [('g', i, z2a, ALL[1:3]), ('mean', [SX]),
                       ('g', i, z2a, ALL[3:4]), ('mean', [S2]), ('g', i, z2a, ALL[4:5]), ('rstd', [SX]),
                       ('g', i, z2a, ALL[5:6]), ('rstd', [S2]), ('g', i, z2a, ALL[6:]), ('o', i, p0)])
            return carry
        t4 = lax.rem(i + NT - 4, NT)
        run('V2', [('g', i, z2a, ALL[:1]), ('xn', zp, i - 3, p1, 1)] + fx
            + [('z2n', jnp.maximum(i - 5, 0), (zc, p1), z2b, 4), ('zstat', (zc, p0)),
               ('g', i, z2a, ALL[1:5]), ('mean', [SX], 1), ('g', i, z2a, ALL[5:6]), ('mean', [SZ]),
               ('g', i, z2a, ALL[6:]), ('mean', [S2]), ('z1', t4, p0, ALL[3:4]), ('rstd', [SX]),
               ('z1', t4, p0, ALL[4:5]), ('rstd', [SZ]), ('z1', t4, p0, ALL[5:6]), ('rstd', [S2]),
               ('z1', t4, p0, ALL[6:]), ('z1', i - 3, p1, ALL[:3]), ('z2', (zc, p1), p1, ALL), ('o', i, p0)])
        return carry

    def stage_d(t, carry):
        @pl.when(t >= 2)
        def _():
            for j in range(3):
                out_copy(jnp.maximum(t - 2, 0), j).wait()

        t0, t1 = 2 * t, 2 * t + 1
        run('D', [('g', t0, z2b, ALL), ('o', t0, None, D // TN - 1, out_copy(t, 0)),
                  ('g', t1, z2b, ALL), ('o', t1, None, OS - 1, out_copy(t, 1))])
        out_copy(t, 2).start()
        return carry

    lax.fori_loop(0, 3, functools.partial(stage_c, False), 0)
    lax.fori_loop(3, NT, functools.partial(stage_c, True), 0)
    zbuf = {3: (zc, 1), 4: (zc, 0), 5: (zt[0], 0), 6: (zt[1], 0), 7: (zc, 0)}
    for i in range(NT, NT + 3):
        p0, p1 = i % 2, (i + 1) % 2
        sz_old, sz_new = (SZ, SL) if p0 == 0 else (SL, SZ)
        items = [('z1', i - 4, p0, ALL[3:4]), ('xn', zp, i - 3, p1, 0), ('z2n', i - 5, zbuf[i - 5], z2b, sz_old[1]),
                 ('zstat', zbuf[i - 4])]
        stats = [sz_new]
        if i - 2 < NT:
            items += [('x3', i - 2, p0)]
            stats += [SX]
        if i - 1 < NT:
            items += [('x2stat', p1)]
            stats += [S2]
        items += [('z1', i - 4, p0, ALL[4:]), ('z1', i - 3, p1, ALL[:3])]
        gates = [('mean', [x]) for x in stats] + [('rstd', [x]) for x in stats]
        for n in ALL:
            items += gates[n:n + 1] + [('z2', zbuf[i - 3], p1, [n])]
        run('V3%d' % i, items)
    t = NT - 1
    run('T1', [('kick',), ('zstat', zbuf[t]), ('z2n', t - 1, zbuf[t - 1], z2b, SL[1]), ('z1', t, 1, [3]),
               ('mean', [SZ]), ('z1', t, 1, [4]), ('rstd', [SZ]), ('z1', t, 1, [5])])
    run('T2', [('kick',), ('z2n', t, zbuf[t], z2b, SZ[1]), ('z1', t, 1, [6])])
    lax.fori_loop(0, NT // 2, stage_d, 0)
    for t in range(NT // 2 - 2, NT // 2):
        for j in range(3):
            out_copy(t, j).wait()


@jax.jit
def pallas_interleave_layers__ssm_conv_h3__mixer_gmlp__prompt_kernel(
        A_q, A_k, A_v, A_shift_k, A_ssm_k, A_ssm_D, B_x, B_w_in, B_w_sp, B_b_sp, B_w_out):
    del B_x
    any_spec = pl.BlockSpec(memory_space=pl.ANY)
    scratch = [
        pltpu.VMEM((2, TM + 16, D), bf16),
        pltpu.VMEM((8, B + 16, D), bf16),
        pltpu.VMEM((8, B, D), bf16),
        pltpu.VMEM((2, D, TM), bf16),
        pltpu.VMEM((D, F), bf16),
        pltpu.VMEM((NT, TM, S), bf16),
        pltpu.VMEM((FH, D), bf16),
        pltpu.VMEM((KS, D), bf16),
        pltpu.VMEM((8, 128), bf16),
        pltpu.VMEM((16, 128), bf16),
        pltpu.VMEM((NT, TM + 8, D), f32),
        pltpu.VMEM((NT, TM, D), f32),
        pltpu.VMEM((NT, TM, FH), bf16),
        pltpu.VMEM((S // 2, FH), u32),
        pltpu.VMEM((S // 2, FH), u32),
        pltpu.VMEM((NT, TM, 128), f32),
        pltpu.VMEM((KS + 1, 8, D), f32),
        pltpu.VMEM((2 * B, B), bf16),
        pltpu.VMEM((B, 2 * B), bf16),
        pltpu.VMEM((4, B, D), bf16),
        [pltpu.VMEM((2, 2 * B + 8, D), f32)] * NT,
        [pltpu.VMEM((2, 2 * B + 8, D), f32)] * NT,
        pltpu.VMEM((1, TM, D), f32),
        pltpu.VMEM((NZ, 2 * B + 8, D), f32),
        pltpu.VMEM((2, 2 * B, D), bf16),
        pltpu.VMEM((2, TM // 2 + 8, D), u32),
        [pltpu.VMEM((1, TM + 8, FH), f32)] * 2,
        pltpu.VMEM((2, TM + 8, FH), f32),
        pltpu.VMEM((2, TM + 8, D), f32),
        pltpu.VMEM((7, TM, 128), f32),
        pltpu.VMEM((8, TM, 128), f32),
        pltpu.VMEM((1, TM // 2 + 8, FH - TN), u32),
        pltpu.VMEM((1, TM // 2 + 8, TN), u32),
        pltpu.SMEM((16,), jnp.int32),
        pltpu.SemaphoreType.DMA((8,)),
        pltpu.SemaphoreType.DMA((3,)),
        pltpu.SemaphoreType.DMA((2,)),
        pltpu.SemaphoreType.DMA((6,)),
    ]
    out = pl.pallas_call(
        _kernel,
        out_shape=jax.ShapeDtypeStruct((NT, TM, D), bf16),
        in_specs=[any_spec] * 10,
        out_specs=any_spec,
        scratch_shapes=scratch,
        compiler_params=pltpu.CompilerParams(vmem_limit_bytes=127 * 1024 * 1024),
    )(A_q.reshape(NT, TM, D), A_k.reshape(NB, B, D), A_v.reshape(NB, B, D), A_shift_k.T, A_ssm_k,
      A_ssm_D.reshape(8, 128), B_w_in, B_w_sp.reshape(NT, TM, S), B_b_sp.reshape(16, 128), B_w_out)
    return out.reshape(1, S, D)
```

```python
import functools
import math
import jax
import jax.numpy as jnp
from jax import lax
import jax.experimental.pallas as pl
import jax.experimental.pallas.tpu as pltpu

S = 2048
D = 1024
F = 3584
FH = F // 2
KS = 4
B = 128
NB = S // B
EPS = 1e-5
f32 = jnp.float32
bf16 = jnp.bfloat16
u32 = jnp.uint32

TM = 256
NT = S // TM
TN = 256
NCH = FH // TN
RG = 16
GW = 256
LR = 16
NZ = 8
CAP_A = 9
CAP_B = 14
GWF = 128
OS = 3
ROT = 256


def _plan(cap_a, cap_b):
    done = set((a, ap) for a in (0, 1) for ap in range(a + 1))
    blocks = {}
    for t in range(NT - 1):
        for kind, cap in (('A', cap_a), ('B', cap_b)):
            sel = {}
            n = 0
            lo = 2 * t + 2 if kind == 'A' else 2 * t + 4
            lim = 2 * t + 3
            for a in range(lo, NB):
                g = [ap for ap in range(a + 1) if (a, ap) not in done and ap <= lim and a - ap <= lim]
                if a > lim:
                    g = g[:max(cap - n, 0)]
                if g:
                    sel[a] = g
                    n += len(g)
            groups = []
            for a in sorted(sel):
                first = not any((a, x) in done for x in range(a + 1))
                done.update((a, x) for x in sel[a])
                last = all((a, x) in done for x in range(a + 1))
                assert a < lo + NZ and last == (a <= 2 * t + 3)
                groups.append((a, sel[a], first, last))
            blocks[(kind, t)] = groups
    assert len(done) == NB * (NB + 1) // 2
    return blocks


def _gelu(x):
    u = x * (0.7978845608028654 + 0.035677408136300125 * (x * x))
    h = 0.5 * x
    return h + h * jnp.tanh(u)


def _h(v):
    return pltpu.bitcast(v, bf16)


def _part(v):
    acc = v[:, 0:128]
    for c in range(128, v.shape[1], 128):
        acc = acc + v[:, c:c + 128]
    return acc


def _lsum(acc):
    return jnp.broadcast_to(jnp.sum(acc, axis=1, keepdims=True), acc.shape)


def _wide(v, n):
    return jnp.concatenate([v] * (n // 128), axis=1)


def _ln(x):
    n = x.shape[-1]
    m = jnp.sum(x, axis=-1, keepdims=True) * (1.0 / n)
    xc = x - m
    v = jnp.sum(xc * xc, axis=-1, keepdims=True) * (1.0 / n)
    return xc * lax.rsqrt(v + EPS)


def _dft_rows(shape, row_dim):
    r = lax.broadcasted_iota(jnp.int32, shape, row_dim)
    n = lax.broadcasted_iota(jnp.int32, shape, 1 - row_dim)
    is_im = r >= B
    rr = jnp.where(is_im, r - B, r)
    odd = rr >= B // 2
    fidx = jnp.where(odd, 2 * (rr - B // 2) + 1, 2 * rr)
    m = (2 * fidx + 1) * n - jnp.where(is_im, B, 0)
    m = jnp.bitwise_and(m, 4 * B - 1)
    m = jnp.where(m > 2 * B, 4 * B - m, m)
    return jnp.cos(m.astype(f32) * (math.pi / (2 * B)))


NT_DIMS = (((1,), (1,)), ((), ()))


def _kernel(q_hbm, k_hbm, v_hbm, sk_hbm, h_hbm, sd_hbm, win_hbm, wsp_hbm, bsp_hbm, wout_hbm,
            o_hbm,
            qb, kb, vb, hb, win, wsp, wout, skb, sdb, bspb,
            x_v, y_v, z1_v, z2a, z2b, bb_v, skt, fm_v, im_v, kvb, ks, hs, wold, zp, zb,
            xn_v, zt, zc, xa, ps, st, ua, ub, zs,
            sem_c, sem_w, sem_s, sem_o):
    plan = _plan(CAP_A, CAP_B)

    def pair_copy(j, p):
        if j == 0:
            return pltpu.make_async_copy(k_hbm.at[pl.ds(2 * p, 2)], kb.at[pl.ds(2 * p % 8, 2), pl.ds(0, B)], sem_c.at[p % 2])
        if j == 1:
            return pltpu.make_async_copy(v_hbm.at[pl.ds(2 * p, 2)], vb.at[pl.ds(2 * p % 8, 2)], sem_c.at[2 + p % 2])
        if j == 2:
            cols = pl.ds(p * TM, TM)
            return pltpu.make_async_copy(h_hbm.at[:, cols], hb.at[p % 2], sem_c.at[4 + p % 2])
        return pltpu.make_async_copy(q_hbm.at[p], qb.at[p % 2, pl.ds(0, TM)], sem_c.at[6 + p % 2])

    WG = ((7, 10), (10, 12), (12, 14), (0, 3), (3, 6), (6, 7))

    def w_copy(i):
        cols = pl.ds(WG[i][0] * TN, (WG[i][1] - WG[i][0]) * TN)
        return pltpu.make_async_copy(win_hbm.at[:, cols], win.at[:, cols], sem_w.at[i % 3])

    def out_copy(t, j):
        cols = (pl.ds(0, D), pl.ds(0, OS * TN), pl.ds(OS * TN, D - OS * TN))[j]
        i = 2 * t + min(j, 1)
        return pltpu.make_async_copy(z1_v.at[i, :, cols], o_hbm.at[i, :, cols], sem_o.at[3 * (t % 2) + j])

    def issue(*copies):
        for cp in copies:
            cp.start(priority=1)

    def issue_big(j):
        if j >= 2:
            big[j - 2].wait()
        issue(big[j])

    small = [
        pltpu.make_async_copy(sk_hbm, skb, sem_o.at[0]),
        pltpu.make_async_copy(sd_hbm, sdb, sem_o.at[1]),
        pltpu.make_async_copy(bsp_hbm, bspb, sem_o.at[2]),
    ]
    WR = FH // 4
    big = ([pltpu.make_async_copy(wsp_hbm.at[j], wsp.at[j], sem_s.at[j % 2]) for j in range(NT)]
           + [pltpu.make_async_copy(wout_hbm.at[pl.ds(j * WR, WR)], wout.at[pl.ds(j * WR, WR)], sem_s.at[j % 2])
              for j in range(4)])
    for cp in small:
        cp.start()
    pair_copy(0, 0).start(priority=1)
    pair_copy(1, 0).start(priority=1)

    def zinit(i, c):
        zs[i] = 0
        return c
    lax.fori_loop(0, 16, zinit, 0)
    issue(pair_copy(2, 0))

    fm_v[...] = _dft_rows((2 * B, B), 0).astype(bf16)
    im_v[...] = (_dft_rows((B, 2 * B), 1) * (1.0 / B)).astype(bf16)

    for cp in small:
        cp.wait()
    sk4 = skb[...].astype(f32)
    for j in range(KS):
        skt[j] = jnp.broadcast_to(sk4[j:j + 1, :], (8, D))
    sd8 = sdb[...].astype(f32)
    skt[KS] = jnp.concatenate([jnp.broadcast_to(sd8[i:i + 1, :], (8, 128)) for i in range(8)], axis=1)

    def kvprep(p, z):
        for a in (2 * p, 2 * p + 1):
            for c in range(0, D, GW):
                for r0 in range(0, B, 32):
                    kcur = kb[a % 8 + z, r0:r0 + 32, c:c + GW].astype(f32)
                    if a == 0 and r0 == 0:
                        kprev = jnp.zeros((8, GW), f32)
                    elif r0 == 0:
                        kprev = kb[(a - 1) % 8 + z, B - 16:B, c:c + GW].astype(f32)[8:16]
                    else:
                        kprev = kb[a % 8 + z, r0 - 16:r0, c:c + GW].astype(f32)[8:16]
                    ext = jnp.concatenate([kprev, kcur], axis=0)
                    sk = [jnp.concatenate([skt[j, :, c:c + GW]] * 4, axis=0) for j in range(KS)]
                    acc = kcur * sk[0]
                    for j in range(1, KS):
                        acc = acc + pltpu.roll(ext, j, 0)[8:] * sk[j]
                    kvb[a % 4, r0:r0 + 32, c:c + GW] = (acc * vb[a % 8, r0:r0 + 32, c:c + GW].astype(f32)).astype(bf16)

    CW = 512

    def rot(c, k, w):
        c = (c + ROT * k) % D
        return slice(c, c + w)

    def put(ref, i, c, val, k):
        for j in range(0, CW, 256):
            ref[i, 0:B, rot(c + j, k, 256)] = val[0:B, j:j + 256]
            ref[i, B:2 * B, rot(c + j, k + 2, 256)] = val[B:2 * B, j:j + 256]

    def fw_h(p):
        fm = fm_v[...]
        res = []
        for a in (2 * p, 2 * p + 1):
            for c in range(0, D, CW):
                hh = lax.dot_general(fm, hb[p % 2, c:c + CW, (a % 2) * B:(a % 2 + 1) * B], NT_DIMS,
                                     preferred_element_type=f32)
                res.append(hh)
                if a == 0:
                    sd = jnp.concatenate([skt[KS, :, c:c + CW]] * (B // 8), axis=0)
                    hh = jnp.concatenate([hh[0:B] + sd, hh[B:2 * B]], axis=0)
                put(hs[p], a % 2, c, hh, 1)
        return res

    def fw_k(p, zk):
        fm = fm_v[...]
        res = []
        for a in (2 * p, 2 * p + 1):
            for c in range(0, D, CW):
                hh = jnp.dot(fm, kvb[a % 4 + zk, :, c:c + CW], preferred_element_type=f32)
                res.append(hh)
                put(ks[p], a % 2, c, hh, 0)
        return res

    def term_tasks(groups, newp):
        def acc(a, g, first, r, c, z, GW):
            zr = zi = None
            for ap in g:
                d = a - ap
                xr = ks[ap // 2][ap % 2 + z, r:r + RG, c:c + GW]
                xi = ks[ap // 2][ap % 2 + z, B + r:B + r + RG, rot(c, 2, GW)]
                hr = hs[d // 2][d % 2 + z, r:r + RG, rot(c, 1, GW)]
                hi = hs[d // 2][d % 2 + z, B + r:B + r + RG, rot(c, 3, GW)]
                tr = xr * hr - xi * hi
                ti = xr * hi + xi * hr
                zr = tr if zr is None else zr + tr
                zi = ti if zi is None else zi + ti
            if not first:
                zr = zr + zp[a % NZ, r:r + RG, c:c + GW]
                zi = zi + zp[a % NZ, B + r:B + r + RG, c:c + GW]
            return zr, zi

        def part_task(a, g, first, r, c, z):
            zr, zi = acc(a, g, first, r, c, z, GW)
            zp[a % NZ, r:r + RG, c:c + GW] = zr
            zp[a % NZ, B + r:B + r + RG, c:c + GW] = zi

        def fin_task(fin, r, c, z):
            GW = GWF
            if fin[0][0] > 0:
                pr = wold[0, r:r + RG, c:c + GW]
                pi = wold[0, B + r:B + r + RG, c:c + GW]
            for (a, g, first, last) in fin:
                wr, wi = acc(a, g, first, r, c, z, GW)
                if a == 0:
                    zr, zi = wr, wi
                elif r < B // 2:
                    zr, zi = wr + pi, wi - pr
                else:
                    zr, zi = wr - pi, wi + pr
                zb[a % 2, r:r + RG, c:c + GW] = zr.astype(bf16)
                zb[a % 2, B + r:B + r + RG, c:c + GW] = zi.astype(bf16)
                pr, pi = wr, wi
            if fin[-1][0] < NB - 1:
                wold[0, r:r + RG, c:c + GW] = pr
                wold[0, B + r:B + r + RG, c:c + GW] = pi

        def srcs(gs):
            return (set(('k', ap // 2) for (a, g, _, _) in gs for ap in g)
                    | set(('h', (a - ap) // 2) for (a, g, _, _) in gs for ap in g))

        rc = [(r, c) for r in range(0, B, RG) for c in range(0, D, GW)]
        tasks = []
        for grp in groups:
            a, g, first, last = grp
            if not last:
                sr = srcs([grp])
                new = any(i == newp for (_, i) in sr)
                tasks += [(len(g), new, sr, ('zp', a % NZ),
                           functools.partial(part_task, a, g, first, r, c)) for (r, c) in rc]
        tasks.sort(key=lambda x: x[1])
        fin = [x for x in groups if x[3]]
        if fin:
            tasks += [(sum(len(x[1]) for x in fin) + 1, True, srcs(fin), ('zb', 0),
                       functools.partial(fin_task, fin, r, c)) for r in range(0, B, RG) for c in range(0, D, GWF)]
        return tasks

    def split_tasks(tasks, caps):
        total = sum(x[0] for x in tasks)
        out = [[] for _ in caps]
        cum = 0
        for x in tasks:
            pos = (cum + 0.5 * x[0]) / max(total, 1) * sum(caps)
            k = 0
            while k + 1 < len(caps) and pos > sum(caps[:k + 1]):
                k += 1
            out[k].append(x)
            cum += x[0]
        return out

    def run_tasks(tasks, val, z):
        for (kind, i) in sorted(set().union(*[x[2] for x in tasks])) if tasks else []:
            (ks if kind == 'k' else hs)[i][z, 2 * B:2 * B + 8, 0:128] = val
        for x in tasks:
            x[4](0)
        probes = {}
        for x in tasks:
            probes[x[3][0]] = x[3][1]
        return probes

    def probe(probes, z):
        vals = []
        if 'zp' in probes:
            vals.append(zp[probes['zp'] + z, 0:8, 0:128])
        if 'zb' in probes:
            vals.append(zb[z, 0:16, 0:128].astype(f32)[0:8])
        return vals

    def sync(vals):
        v = vals[0]
        for w in vals[1:]:
            v = v + w
        return _lsum(v)

    def inv(p, z):
        im = im_v[...]
        res = []
        for d in range(2):
            for c in range(0, D, CW):
                y = jnp.dot(im, zb[d + z, :, c:c + CW], preferred_element_type=f32)
                res.append(y)
                y_v[p, d * B:(d + 1) * B, c:c + CW] = y
        return res

    R = range(0, TM, LR)

    def corner(acc):
        return acc[acc.shape[0] - 8:, acc.shape[1] - 128:]

    def b16(v):
        return jnp.concatenate([v, v], axis=0).astype(bf16)

    def stat_part(x, i, r, n):
        w = x.shape[1]
        mu = _part(x) * (128.0 / w)
        dv = x - _wide(mu, w)
        ps[i, r:r + n] = mu
        ps[i + 1, r:r + n] = _part(dv * dv)

    def stat_mean(i, j, w, z):
        mu = ps[i + z]
        m = _lsum(mu) * (1.0 / 128)
        st[j] = m
        e = mu - m
        ps[i] = ps[i + 1 + z] + (w / 128.0) * (e * e)

    def stat_rstd(i, j, w, z):
        st[j + 1] = lax.rsqrt(_lsum(ps[i + z]) * (1.0 / w) + EPS)

    def norm(x, j, r, n):
        w = x.shape[1]
        return (x - _wide(st[j, r:r + n], w)) * _wide(st[j + 1, r:r + n], w)

    PG = 6

    def z_dot(xn, n):
        return jnp.dot(xn, win[:, n * TN:(n + 1) * TN], preferred_element_type=f32)

    def kick():
        return jnp.dot(fm_v[0:16, :], fm_v[0:128, :], preferred_element_type=f32)

    def lead(ref, i):
        return ref[i, 0:16, 0:128].astype(f32)[0:8]

    def tile_rows(t, r, n):
        if isinstance(t, int):
            return slice(t * TM // 2 + r, t * TM // 2 + r + n)
        return pl.ds(pl.multiple_of(t * (TM // 2) + r, 8), n)

    def block(items):
        z = [zs[j] for j in range(8)]
        c = dict(sg=None, acc=None, vals=[], xn={}, ng=0, rel=[])

        def release(ref):
            if not any(ref is x for x in c['rel']):
                c['rel'].append(ref)
                ref[z[0], TM:TM + 8, 0:128] = c['sg']

        def mxu(res):
            if c['sg'] is None:
                c['sg'] = res[0][0:8, 0:128]
            c['acc'] = res[-1]

        def get_xn(i):
            if id(i) not in c['xn']:
                c['xn'][id(i)] = pltpu.bitcast(xn_v[i, 0:TM // 2], bf16)
            return c['xn'][id(i)]

        for it in items:
            kind = it[0]
            sg = c['sg']
            if kind == 'kick':
                mxu([kick()])
            elif kind == 'z1':
                for n in it[3]:
                    acc = z_dot(get_xn(it[2]), n)
                    z1_v[it[1], :, n * TN:(n + 1) * TN] = _gelu(acc).astype(bf16)
                    mxu([acc])
            elif kind == 'z2':
                for n in it[3]:
                    acc = z_dot(get_xn(it[2]), NCH + n)
                    it[1][0][it[1][1], 0:TM, n * TN:(n + 1) * TN] = _gelu(acc)
                    mxu([acc])
            elif kind == 'inv':
                mxu(inv(it[1], z[1] if it[2] else 0))
            elif kind == 'fwh':
                mxu(fw_h(it[1]))
            elif kind == 'fwk':
                mxu(fw_k(it[1], z[1] if it[2] else 0))
            elif kind == 'g':
                if c.get('wt') is not it[1]:
                    c['wt'], c['ws'] = it[1], wsp[it[1]]
                ws = c['ws']
                bbt = _wide(bb_v[it[1]], TN)
                for n in it[3]:
                    acc = jnp.dot(ws, _h(it[2][:, n * TN:(n + 1) * TN]), preferred_element_type=f32)
                    u = (z1_v[it[1], :, n * TN:(n + 1) * TN].astype(f32) * (acc + bbt)).astype(bf16)
                    u = pltpu.bitcast(u, u32)
                    if n < NCH - 1:
                        ua[0, 0:TM // 2, n * TN:(n + 1) * TN] = u
                    else:
                        ub[0, 0:TM // 2] = u
                    mxu([acc])
            elif kind == 'o':
                ua[z[1], TM // 2:TM // 2 + 8, 0:128] = pltpu.bitcast(sg, u32)
                ub[z[1], TM // 2:TM // 2 + 8, 0:128] = pltpu.bitcast(sg, u32)
                u = _h(jnp.concatenate([ua[0, 0:TM // 2], ub[0, 0:TM // 2]], axis=1))
                for n in range(D // TN):
                    acc = jnp.dot(u, wout[:, n * TN:(n + 1) * TN], preferred_element_type=f32)
                    x2 = (zp if it[2] is None else x_v)[it[1], 0:TM, n * TN:(n + 1) * TN] + acc
                    if it[2] is None:
                        z1_v[it[1], :, n * TN:(n + 1) * TN] = x2.astype(bf16)
                        if n == it[3]:
                            it[4].start()
                    else:
                        xa[it[2], 0:TM, n * TN:(n + 1) * TN] = x2
                    mxu([acc])
            elif kind == 'xn':
                release(it[1])
                for r in R:
                    if it[4]:
                        xn_v[1 - it[3], r // 2:(r + LR) // 2] = xn_v[it[3], r // 2:(r + LR) // 2]
                    xn_v[it[3], r // 2:(r + LR) // 2] = pltpu.bitcast(
                        norm(it[1][it[2], r:r + LR], 2, r, LR).astype(bf16), u32)
                xn_v[z[1], TM // 2:TM // 2 + 8, 0:128] = pltpu.bitcast(sg, u32)
                c['xn'] = {}
                if it[4]:
                    c['vals'].append(pltpu.bitcast(xn_v[it[3] + z[6], 0:8, 0:128], f32))
            elif kind == 'xmove':
                xn_v[0, 0:TM // 2] = xn_v[1, 0:TM // 2]
            elif kind == 'z2n':
                release(it[2][0])
                for r in R:
                    it[3][tile_rows(it[1], r // 2, LR // 2), :] = pltpu.bitcast(
                        norm(it[2][0][it[2][1], r:r + LR], it[4], r, LR).astype(bf16), u32)
                c['vals'].append(pltpu.bitcast(it[3][tile_rows(it[1] + z[6], 0, 8), 0:128], f32))
            elif kind == 'qstat':
                qb[z[0], TM:TM + 16, 0:128] = b16(sg)
                for r in R:
                    stat_part(qb[it[1] % 2, r:r + LR].astype(f32), 0, r, LR)
            elif kind == 'zstat':
                release(it[1][0])
                for r in range(0, TM, 8):
                    stat_part(it[1][0][it[1][1], r:r + 8], 2, r, 8)
            elif kind == 'x1':
                if it[2]:
                    qb[z[0], TM:TM + 16, 0:128] = b16(sg)
                for r in R:
                    x0 = qb[it[1] % 2, r:r + LR].astype(f32)
                    x1 = x0 + norm(x0, 0, r, LR) * y_v[it[1] + (0 if it[2] else z[1]), r:r + LR]
                    x_v[it[1], r:r + LR] = x1
                    stat_part(x1, 0, r, LR)
            elif kind == 'x2stat':
                release(xa)
                for r in R:
                    stat_part(xa[it[1], r:r + LR], 4, r, LR)
            elif kind == 'x3':
                release(xa)
                for r in R:
                    x0 = xa[it[2], r:r + LR]
                    x1 = x0 + norm(x0, 0, r, LR) * y_v[it[1], r:r + LR]
                    zp[it[1], r:r + LR] = x1
                    stat_part(x1, 0, r, LR)
            elif kind == 'kvprep':
                kb[z[0], B:B + 16, 0:128] = b16(sg)
                kvprep(it[1], 0)
                if not it[2]:
                    c['vals'].append(lead(kvb, (2 * it[1]) % 4 + z[6]))
            elif kind == 'terms':
                c['vals'] += probe(run_tasks(it[1], sg, z[0]), z[6])
            elif kind == 'mean' or kind == 'rstd':
                gate = corner(c['acc'])
                if len(it) > 2:
                    for v in c['vals']:
                        gate = gate + v
                    c['vals'] = []
                ps[PG + z[2], 8 * c['ng']:8 * c['ng'] + 8] = gate
                c['ng'] += 1
                for (i, j, w) in it[1]:
                    (stat_mean if kind == 'mean' else stat_rstd)(i, j, w, 0)
            elif kind == 'bb':
                bs16 = bspb[...].astype(f32)
                for i in range(S // 128):
                    bb_v[i // 2, (i % 2) * 128:(i % 2 + 1) * 128, :] = jnp.transpose(
                        jnp.broadcast_to(bs16[i:i + 1, :], (128, 128)))
        if c['vals']:
            ps[PG, 64:72] = sync([c['acc'][0:8, 0:128]] + c['vals'])

    def run(name, items, cond=None):
        with jax.named_scope(name):
            pl.when(zs[15] == 0 if cond is None else cond)(lambda: block(items))

    SQ, SX, SZ, S2, SL = (0, 0, D), (0, 2, D), (2, 4, FH), (4, 0, D), (2, 6, FH)
    Z0 = (zt[0], 0)
    ALL = list(range(NCH))

    def block_p0():
        kvprep(0, 0)

    def block_p1():
        fw_k(0, 0)
        fw_h(0)

    def block_p2():
        z = [zs[j] for j in range(4)]
        sg = fw_h(1)[0][0:8, 0:128]
        run_tasks(term_tasks([(0, [0], True, True), (1, [0, 1], True, True)], 0), sg, z[1])
        qb[0, TM:TM + 16, 0:128] = b16(sg)
        for r in R:
            stat_part(qb[z[1], r:r + LR].astype(f32), 0, r, LR)
        stat_mean(0, 0, D, z[2])
        inv(0, z[0])
        stat_rstd(0, 0, D, z[3])

    def block_p3():
        kvprep(1, 0)
        fw_k(1, zs[0])
        for r in R:
            x0 = qb[0, r:r + LR].astype(f32)
            x1 = x0 + norm(x0, 0, r, LR) * y_v[0, r:r + LR]
            x_v[0, r:r + LR] = x1
            xn_v[0, r // 2:(r + LR) // 2] = pltpu.bitcast(_ln(x1).astype(bf16), u32)

    for name, waits, fn, nxt in (
            ('P0', ((0, 0), (1, 0)), block_p0, [pair_copy(3, 0), pair_copy(2, 1)]),
            ('P1', ((2, 0),), block_p1, [pair_copy(0, 1), pair_copy(1, 1)]),
            ('P2', ((3, 0), (2, 1)), block_p2, [w_copy(0)]),
            ('P3', ((0, 1), (1, 1)), block_p3, [pair_copy(3, 1), w_copy(1)])):
        issue(*nxt)
        for (j, p) in waits:
            pair_copy(j, p).wait()
        with jax.named_scope(name):
            pl.when(zs[15] == 0)(fn)

    for t in range(NT):
        conv = t < NT - 1
        ta = term_tasks(plan[('A', t)], -1) if conv else []
        tb = term_tasks(plan[('B', t)], -1) if conv else []
        if t == 0:
            ch = split_tasks(ta, [3, 1.5, 2])
            issue(w_copy(2))
            w_copy(0).wait()
            run('A0a', [('kick',), ('terms', ch[0]), ('z2', Z0, 0, [0, 1, 2])])
            issue(pair_copy(0, 2), pair_copy(1, 2), pair_copy(2, 2))
            pair_copy(3, 1).wait()
            w_copy(1).wait()
            run('A0b', [('kick',), ('qstat', 1), ('terms', ch[1]), ('z2', Z0, 0, [3]), ('mean', [SQ]),
                        ('z2', Z0, 0, [4])])
            issue(w_copy(3))
            w_copy(2).wait()
            run('A0c', [('kick',), ('rstd', [SQ]), ('terms', ch[2]), ('z2', Z0, 0, [5, 6])])
            issue(w_copy(4))
            for j in range(3):
                pair_copy(j, 2).wait()
            run('B0a', [('inv', 1, 0), ('kvprep', 2, 1), ('fwh', 2), ('fwk', 2, 1)])
            issue(w_copy(5), pair_copy(3, 2), pair_copy(0, 3), pair_copy(1, 3))
            w_copy(3).wait()
            run('B0b', [('kick',), ('zstat', Z0), ('x1', 1, 1), ('z1', 0, 0, [0, 1]), ('mean', [SX, SZ]),
                        ('z1', 0, 0, [2])])
            w_copy(4).wait()
            run('B0c', [('kick',), ('rstd', [SX, SZ]), ('terms', tb), ('bb',), ('z1', 0, 0, [3, 4, 5])])
            w_copy(5).wait()
            continue
        if t + 2 < NT:
            issue(pair_copy(2, t + 2), pair_copy(3, t + 2))
        if t + 3 < NT:
            issue(pair_copy(0, t + 3), pair_copy(1, t + 3))
        if t > 1:
            issue_big(2 * t - 3)
        if conv:
            pair_copy(3, t + 1).wait()
        if t + 2 < NT and t > 1:
            pair_copy(0, t + 2).wait()
            pair_copy(1, t + 2).wait()
        s0, s1 = t % 2, (t - 1) % 2
        za, zo = (zt[s0], 0), (zt[s1], 0)
        items = [('z1', t - 1, s1, [NCH - 1 if conv else NCH - 2]), ('xn', x_v, t, s0, 0), ('z2n', t - 1, zo, z2a, 4)]
        if conv:
            items += [('qstat', t + 1)]
            if t + 2 < NT and t > 1:
                items += [('kvprep', t + 2, 0)]
            items += [('terms', ta), ('z2', za, s0, ALL[:4]), ('mean', [SQ]), ('z2', za, s0, ALL[4:5]),
                      ('rstd', [SQ]), ('z2', za, s0, ALL[5:])]
        else:
            items += [('z2', za, s0, ALL)]
        run('A%d' % t, items)
        if conv:
            issue_big(2 * t - 2)
        if t == 1:
            pair_copy(0, t + 2).wait()
            pair_copy(1, t + 2).wait()
        if t + 2 < NT:
            pair_copy(2, t + 2).wait()
        if conv:
            items = [('inv', t + 1, 0), ('zstat', za), ('x1', t + 1, 0)]
            if t == 1:
                items += [('kvprep', t + 2, 1)]
            items += [('terms', tb)]
            if t + 2 < NT:
                items += [('fwh', t + 2)]
            if t + 2 < NT and t > 1:
                items += [('fwk', t + 2, 0)]
            if t + 2 < NT:
                items += [('z1', t, s0, ALL[:2]), ('mean', [SZ]), ('z1', t, s0, ALL[2:3]), ('mean', [SX]),
                          ('z1', t, s0, ALL[3:4]), ('rstd', [SZ])]
                if t == 1:
                    items += [('fwk', t + 2, 1)]
                items += [('z1', t, s0, ALL[4:5]), ('rstd', [SX]), ('z1', t, s0, ALL[5:6])]
            else:
                items += [('z1', t, s0, ALL[:2]), ('mean', [SZ]), ('z1', t, s0, ALL[2:3]), ('mean', [SX]),
                          ('rstd', [SZ]), ('z1', t, s0, ALL[3:4]), ('rstd', [SX]), ('z1', t, s0, ALL[4:5])]
            run('B%d' % t, items)
        else:
            run('B7a', [('kick',), ('zstat', za), ('z1', t, s0, [0]), ('mean', [SZ]), ('z1', t, s0, [1]),
                        ('rstd', [SZ]), ('z1', t, s0, [2])])
            run('B7b', [('kick',), ('z2n', t, za, z2a, 4), ('z1', t - 1, s1, [NCH - 1])])

    for cp in big[-2:]:
        cp.wait()

    def stage_c(full, i, carry):
        p0 = lax.rem(i, 2)
        p1 = 1 - p0
        fx = [('x3', jnp.maximum(i - 2, 0), p0), ('x2stat', p1)]
        if not full:
            run('V1', [('g', i, z2a, ALL[:1]), ('xmove',)] + fx + [('g', i, z2a, ALL[1:3]), ('mean', [SX]),
                       ('g', i, z2a, ALL[3:4]), ('mean', [S2]), ('g', i, z2a, ALL[4:5]), ('rstd', [SX]),
                       ('g', i, z2a, ALL[5:6]), ('rstd', [S2]), ('g', i, z2a, ALL[6:]), ('o', i, p0)])
            return carry
        t4 = lax.rem(i + NT - 4, NT)
        run('V2', [('g', i, z2a, ALL[:1]), ('xn', zp, i - 3, 0, 1)] + fx
            + [('z2n', jnp.maximum(i - 5, 0), (zc, p1), z2b, 4), ('zstat', (zc, p0)),
               ('g', i, z2a, ALL[1:5]), ('mean', [SX], 1), ('g', i, z2a, ALL[5:6]), ('mean', [SZ]),
               ('g', i, z2a, ALL[6:]), ('mean', [S2]), ('z1', t4, 1, ALL[3:4]), ('rstd', [SX]),
               ('z1', t4, 1, ALL[4:5]), ('rstd', [SZ]), ('z1', t4, 1, ALL[5:6]), ('rstd', [S2]),
               ('z1', t4, 1, ALL[6:]), ('z1', i - 3, 0, ALL[:3]), ('z2', (zc, p1), 0, ALL), ('o', i, p0)])
        return carry

    def stage_d(t, carry):
        @pl.when(t >= 2)
        def _():
            for j in range(3):
                out_copy(jnp.maximum(t - 2, 0), j).wait()

        t0, t1 = 2 * t, 2 * t + 1
        run('D', [('g', t0, z2b, ALL), ('o', t0, None, D // TN - 1, out_copy(t, 0)),
                  ('g', t1, z2b, ALL), ('o', t1, None, OS - 1, out_copy(t, 1))])
        out_copy(t, 2).start()
        return carry

    lax.fori_loop(0, 3, functools.partial(stage_c, False), 0)
    lax.fori_loop(3, NT, functools.partial(stage_c, True), 0)
    zbuf = {3: (zc, 1), 4: (zc, 0), 5: (zt[0], 0), 6: (zt[1], 0), 7: (zc, 0)}
    for i in range(NT, NT + 3):
        p0, p1 = i % 2, (i + 1) % 2
        sz_old, sz_new = (SZ, SL) if p0 == 0 else (SL, SZ)
        items = [('z1', i - 4, p0, ALL[3:4]), ('xn', zp, i - 3, p1, 0), ('z2n', i - 5, zbuf[i - 5], z2b, sz_old[1]),
                 ('zstat', zbuf[i - 4])]
        stats = [sz_new]
        if i - 2 < NT:
            items += [('x3', i - 2, p0)]
            stats += [SX]
        if i - 1 < NT:
            items += [('x2stat', p1)]
            stats += [S2]
        items += [('z1', i - 4, p0, ALL[4:]), ('z1', i - 3, p1, ALL[:3])]
        gates = [('mean', [x]) for x in stats] + [('rstd', [x]) for x in stats]
        for n in ALL:
            items += gates[n:n + 1] + [('z2', zbuf[i - 3], p1, [n])]
        run('V3%d' % i, items)
    t = NT - 1
    run('T1', [('kick',), ('zstat', zbuf[t]), ('z2n', t - 1, zbuf[t - 1], z2b, SL[1]), ('z1', t, 1, [3]),
               ('mean', [SZ]), ('z1', t, 1, [4]), ('rstd', [SZ]), ('z1', t, 1, [5])])
    run('T2', [('kick',), ('z2n', t, zbuf[t], z2b, SZ[1]), ('z1', t, 1, [6])])
    lax.fori_loop(0, NT // 2, stage_d, 0)
    for t in range(NT // 2 - 2, NT // 2):
        for j in range(3):
            out_copy(t, j).wait()


@jax.jit
def pallas_interleave_layers__ssm_conv_h3__mixer_gmlp__prompt_kernel(
        A_q, A_k, A_v, A_shift_k, A_ssm_k, A_ssm_D, B_x, B_w_in, B_w_sp, B_b_sp, B_w_out):
    del B_x
    any_spec = pl.BlockSpec(memory_space=pl.ANY)
    scratch = [
        pltpu.VMEM((2, TM + 16, D), bf16),
        pltpu.VMEM((8, B + 16, D), bf16),
        pltpu.VMEM((8, B, D), bf16),
        pltpu.VMEM((2, D, TM), bf16),
        pltpu.VMEM((D, F), bf16),
        pltpu.VMEM((NT, TM, S), bf16),
        pltpu.VMEM((FH, D), bf16),
        pltpu.VMEM((KS, D), bf16),
        pltpu.VMEM((8, 128), bf16),
        pltpu.VMEM((16, 128), bf16),
        pltpu.VMEM((NT, TM + 8, D), f32),
        pltpu.VMEM((NT, TM, D), f32),
        pltpu.VMEM((NT, TM, FH), bf16),
        pltpu.VMEM((S // 2, FH), u32),
        pltpu.VMEM((S // 2, FH), u32),
        pltpu.VMEM((NT, TM, 128), f32),
        pltpu.VMEM((KS + 1, 8, D), f32),
        pltpu.VMEM((2 * B, B), bf16),
        pltpu.VMEM((B, 2 * B), bf16),
        pltpu.VMEM((4, B, D), bf16),
        [pltpu.VMEM((2, 2 * B + 8, D), f32)] * NT,
        [pltpu.VMEM((2, 2 * B + 8, D), f32)] * NT,
        pltpu.VMEM((1, TM, D), f32),
        pltpu.VMEM((NZ, 2 * B + 8, D), f32),
        pltpu.VMEM((2, 2 * B, D), bf16),
        pltpu.VMEM((2, TM // 2 + 8, D), u32),
        [pltpu.VMEM((1, TM + 8, FH), f32)] * 2,
        pltpu.VMEM((2, TM + 8, FH), f32),
        pltpu.VMEM((2, TM + 8, D), f32),
        pltpu.VMEM((7, TM, 128), f32),
        pltpu.VMEM((8, TM, 128), f32),
        pltpu.VMEM((1, TM // 2 + 8, FH - TN), u32),
        pltpu.VMEM((1, TM // 2 + 8, TN), u32),
        pltpu.SMEM((16,), jnp.int32),
        pltpu.SemaphoreType.DMA((8,)),
        pltpu.SemaphoreType.DMA((3,)),
        pltpu.SemaphoreType.DMA((2,)),
        pltpu.SemaphoreType.DMA((6,)),
    ]
    out = pl.pallas_call(
        _kernel,
        out_shape=jax.ShapeDtypeStruct((NT, TM, D), bf16),
        in_specs=[any_spec] * 10,
        out_specs=any_spec,
        scratch_shapes=scratch,
        compiler_params=pltpu.CompilerParams(vmem_limit_bytes=127 * 1024 * 1024),
    )(A_q.reshape(NT, TM, D), A_k.reshape(NB, B, D), A_v.reshape(NB, B, D), A_shift_k.T, A_ssm_k,
      A_ssm_D.reshape(8, 128), B_w_in, B_w_sp.reshape(NT, TM, S), B_b_sp.reshape(16, 128), B_w_out)
    return out.reshape(1, S, D)
```

```python
import functools
import math
import jax
import jax.numpy as jnp
from jax import lax
import jax.experimental.pallas as pl
import jax.experimental.pallas.tpu as pltpu

S = 2048
D = 1024
F = 3584
FH = F // 2
KS = 4
B = 128
NB = S // B
EPS = 1e-5
f32 = jnp.float32
bf16 = jnp.bfloat16
u32 = jnp.uint32

TM = 256
NT = S // TM
TN = 256
NCH = FH // TN
RG = 16
GW = 256
LR = 16
NZ = 8
CAP_A = 9
CAP_B = 14
GWF = 128
OS = 3
ROT = 256


def _plan(cap_a, cap_b):
    done = set((a, ap) for a in (0, 1) for ap in range(a + 1))
    blocks = {}
    for t in range(NT - 1):
        for kind, cap in (('A', cap_a), ('B', cap_b)):
            sel = {}
            n = 0
            lo = 2 * t + 2 if kind == 'A' else 2 * t + 4
            lim = 2 * t + 3
            for a in range(lo, NB):
                g = [ap for ap in range(a + 1) if (a, ap) not in done and ap <= lim and a - ap <= lim]
                if a > lim:
                    g = g[:max(cap - n, 0)]
                if g:
                    sel[a] = g
                    n += len(g)
            groups = []
            for a in sorted(sel):
                first = not any((a, x) in done for x in range(a + 1))
                done.update((a, x) for x in sel[a])
                last = all((a, x) in done for x in range(a + 1))
                assert a < lo + NZ and last == (a <= 2 * t + 3)
                groups.append((a, sel[a], first, last))
            blocks[(kind, t)] = groups
    assert len(done) == NB * (NB + 1) // 2
    return blocks


def _gelu(x):
    u = x * (0.7978845608028654 + 0.035677408136300125 * (x * x))
    h = 0.5 * x
    return h + h * jnp.tanh(u)


def _h(v):
    return pltpu.bitcast(v, bf16)


def _part(v):
    acc = v[:, 0:128]
    for c in range(128, v.shape[1], 128):
        acc = acc + v[:, c:c + 128]
    return acc


def _lsum(acc):
    return jnp.broadcast_to(jnp.sum(acc, axis=1, keepdims=True), acc.shape)


def _wide(v, n):
    return jnp.concatenate([v] * (n // 128), axis=1)


def _ln(x):
    n = x.shape[-1]
    m = jnp.sum(x, axis=-1, keepdims=True) * (1.0 / n)
    xc = x - m
    v = jnp.sum(xc * xc, axis=-1, keepdims=True) * (1.0 / n)
    return xc * lax.rsqrt(v + EPS)


def _dft_rows(shape, row_dim):
    r = lax.broadcasted_iota(jnp.int32, shape, row_dim)
    n = lax.broadcasted_iota(jnp.int32, shape, 1 - row_dim)
    is_im = r >= B
    rr = jnp.where(is_im, r - B, r)
    odd = rr >= B // 2
    fidx = jnp.where(odd, 2 * (rr - B // 2) + 1, 2 * rr)
    m = (2 * fidx + 1) * n - jnp.where(is_im, B, 0)
    m = jnp.bitwise_and(m, 4 * B - 1)
    m = jnp.where(m > 2 * B, 4 * B - m, m)
    return jnp.cos(m.astype(f32) * (math.pi / (2 * B)))


NT_DIMS = (((1,), (1,)), ((), ()))


def _kernel(q_hbm, k_hbm, v_hbm, sk_hbm, h_hbm, sd_hbm, win_hbm, wsp_hbm, bsp_hbm, wout_hbm,
            o_hbm,
            qb, kb, vb, hb, win, wsp, wout, skb, sdb, bspb,
            x_v, y_v, z1_v, z2a, z2b, bb_v, skt, fm_v, im_v, kvb, ks, hs, wold, zp, zb,
            xn_v, zt, zc, xa, ps, st, ua, ub, zs,
            sem_c, sem_w, sem_s, sem_o):
    plan = _plan(CAP_A, CAP_B)

    def pair_copy(j, p):
        if j == 0:
            return pltpu.make_async_copy(k_hbm.at[pl.ds(2 * p, 2)], kb.at[pl.ds(2 * p % 8, 2), pl.ds(0, B)], sem_c.at[p % 2])
        if j == 1:
            return pltpu.make_async_copy(v_hbm.at[pl.ds(2 * p, 2)], vb.at[pl.ds(2 * p % 8, 2)], sem_c.at[2 + p % 2])
        if j == 2:
            cols = pl.ds(p * TM, TM)
            return pltpu.make_async_copy(h_hbm.at[:, cols], hb.at[p % 2], sem_c.at[4 + p % 2])
        return pltpu.make_async_copy(q_hbm.at[p], qb.at[p % 2, pl.ds(0, TM)], sem_c.at[6 + p % 2])

    WG = ((7, 10), (10, 12), (12, 14), (0, 3), (3, 6), (6, 7))

    def w_copy(i):
        cols = pl.ds(WG[i][0] * TN, (WG[i][1] - WG[i][0]) * TN)
        return pltpu.make_async_copy(win_hbm.at[:, cols], win.at[:, cols], sem_w.at[i % 3])

    def out_copy(t, j):
        cols = (pl.ds(0, D), pl.ds(0, OS * TN), pl.ds(OS * TN, D - OS * TN))[j]
        i = 2 * t + min(j, 1)
        return pltpu.make_async_copy(z1_v.at[i, :, cols], o_hbm.at[i, :, cols], sem_o.at[3 * (t % 2) + j])

    def issue(*copies):
        for cp in copies:
            cp.start(priority=1)

    def issue_big(j):
        if j >= 2:
            big[j - 2].wait()
        issue(big[j])

    small = [
        pltpu.make_async_copy(sk_hbm, skb, sem_o.at[0]),
        pltpu.make_async_copy(sd_hbm, sdb, sem_o.at[1]),
        pltpu.make_async_copy(bsp_hbm, bspb, sem_o.at[2]),
    ]
    WR = FH // 4
    big = ([pltpu.make_async_copy(wsp_hbm.at[j], wsp.at[j], sem_s.at[j % 2]) for j in range(NT)]
           + [pltpu.make_async_copy(wout_hbm.at[pl.ds(j * WR, WR)], wout.at[pl.ds(j * WR, WR)], sem_s.at[j % 2])
              for j in range(4)])
    for cp in small:
        cp.start()
    pair_copy(0, 0).start(priority=1)
    pair_copy(1, 0).start(priority=1)

    def zinit(i, c):
        zs[i] = 0
        return c
    lax.fori_loop(0, 16, zinit, 0)
    issue(pair_copy(2, 0))

    fm_v[...] = _dft_rows((2 * B, B), 0).astype(bf16)
    im_v[...] = (_dft_rows((B, 2 * B), 1) * (1.0 / B)).astype(bf16)

    for cp in small:
        cp.wait()
    sk4 = skb[...].astype(f32)
    for j in range(KS):
        skt[j] = jnp.broadcast_to(sk4[j:j + 1, :], (8, D))
    sd8 = sdb[...].astype(f32)
    skt[KS] = jnp.concatenate([jnp.broadcast_to(sd8[i:i + 1, :], (8, 128)) for i in range(8)], axis=1)

    def kvprep(p, z):
        for a in (2 * p, 2 * p + 1):
            for c in range(0, D, GW):
                for r0 in range(0, B, 32):
                    kcur = kb[a % 8 + z, r0:r0 + 32, c:c + GW].astype(f32)
                    if a == 0 and r0 == 0:
                        kprev = jnp.zeros((8, GW), f32)
                    elif r0 == 0:
                        kprev = kb[(a - 1) % 8 + z, B - 16:B, c:c + GW].astype(f32)[8:16]
                    else:
                        kprev = kb[a % 8 + z, r0 - 16:r0, c:c + GW].astype(f32)[8:16]
                    ext = jnp.concatenate([kprev, kcur], axis=0)
                    sk = [jnp.concatenate([skt[j, :, c:c + GW]] * 4, axis=0) for j in range(KS)]
                    acc = kcur * sk[0]
                    for j in range(1, KS):
                        acc = acc + pltpu.roll(ext, j, 0)[8:] * sk[j]
                    kvb[a % 4, r0:r0 + 32, c:c + GW] = (acc * vb[a % 8, r0:r0 + 32, c:c + GW].astype(f32)).astype(bf16)

    CW = 512

    def rot(c, k, w):
        c = (c + ROT * k) % D
        return slice(c, c + w)

    def put(ref, i, c, val, k):
        for j in range(0, CW, 256):
            ref[i, 0:B, rot(c + j, k, 256)] = val[0:B, j:j + 256]
            ref[i, B:2 * B, rot(c + j, k + 2, 256)] = val[B:2 * B, j:j + 256]

    def fw_h(p):
        fm = fm_v[...]
        res = []
        for a in (2 * p, 2 * p + 1):
            for c in range(0, D, CW):
                hh = lax.dot_general(fm, hb[p % 2, c:c + CW, (a % 2) * B:(a % 2 + 1) * B], NT_DIMS,
                                     preferred_element_type=f32)
                res.append(hh)
                if a == 0:
                    sd = jnp.concatenate([skt[KS, :, c:c + CW]] * (B // 8), axis=0)
                    hh = jnp.concatenate([hh[0:B] + sd, hh[B:2 * B]], axis=0)
                put(hs[p], a % 2, c, hh, 1)
        return res

    def fw_k(p, zk):
        fm = fm_v[...]
        res = []
        for a in (2 * p, 2 * p + 1):
            for c in range(0, D, CW):
                hh = jnp.dot(fm, kvb[a % 4 + zk, :, c:c + CW], preferred_element_type=f32)
                res.append(hh)
                put(ks[p], a % 2, c, hh, 0)
        return res

    def term_tasks(groups, newp):
        def acc(a, g, first, r, c, z, GW):
            zr = zi = None
            for ap in g:
                d = a - ap
                xr = ks[ap // 2][ap % 2 + z, r:r + RG, c:c + GW]
                xi = ks[ap // 2][ap % 2 + z, B + r:B + r + RG, rot(c, 2, GW)]
                hr = hs[d // 2][d % 2 + z, r:r + RG, rot(c, 1, GW)]
                hi = hs[d // 2][d % 2 + z, B + r:B + r + RG, rot(c, 3, GW)]
                tr = xr * hr - xi * hi
                ti = xr * hi + xi * hr
                zr = tr if zr is None else zr + tr
                zi = ti if zi is None else zi + ti
            if not first:
                zr = zr + zp[a % NZ, r:r + RG, c:c + GW]
                zi = zi + zp[a % NZ, B + r:B + r + RG, c:c + GW]
            return zr, zi

        def part_task(a, g, first, r, c, z):
            zr, zi = acc(a, g, first, r, c, z, GW)
            zp[a % NZ, r:r + RG, c:c + GW] = zr
            zp[a % NZ, B + r:B + r + RG, c:c + GW] = zi

        def fin_task(fin, r, c, z):
            GW = GWF
            if fin[0][0] > 0:
                pr = wold[0, r:r + RG, c:c + GW]
                pi = wold[0, B + r:B + r + RG, c:c + GW]
            for (a, g, first, last) in fin:
                wr, wi = acc(a, g, first, r, c, z, GW)
                if a == 0:
                    zr, zi = wr, wi
                elif r < B // 2:
                    zr, zi = wr + pi, wi - pr
                else:
                    zr, zi = wr - pi, wi + pr
                zb[a % 2, r:r + RG, c:c + GW] = zr.astype(bf16)
                zb[a % 2, B + r:B + r + RG, c:c + GW] = zi.astype(bf16)
                pr, pi = wr, wi
            if fin[-1][0] < NB - 1:
                wold[0, r:r + RG, c:c + GW] = pr
                wold[0, B + r:B + r + RG, c:c + GW] = pi

        def srcs(gs):
            return (set(('k', ap // 2) for (a, g, _, _) in gs for ap in g)
                    | set(('h', (a - ap) // 2) for (a, g, _, _) in gs for ap in g))

        rc = [(r, c) for r in range(0, B, RG) for c in range(0, D, GW)]
        tasks = []
        for grp in groups:
            a, g, first, last = grp
            if not last:
                sr = srcs([grp])
                new = any(i == newp for (_, i) in sr)
                tasks += [(len(g), new, sr, ('zp', a % NZ),
                           functools.partial(part_task, a, g, first, r, c)) for (r, c) in rc]
        tasks.sort(key=lambda x: x[1])
        fin = [x for x in groups if x[3]]
        if fin:
            tasks += [(sum(len(x[1]) for x in fin) + 1, True, srcs(fin), ('zb', 0),
                       functools.partial(fin_task, fin, r, c)) for r in range(0, B, RG) for c in range(0, D, GWF)]
        return tasks

    def split_tasks(tasks, caps):
        total = sum(x[0] for x in tasks)
        out = [[] for _ in caps]
        cum = 0
        for x in tasks:
            pos = (cum + 0.5 * x[0]) / max(total, 1) * sum(caps)
            k = 0
            while k + 1 < len(caps) and pos > sum(caps[:k + 1]):
                k += 1
            out[k].append(x)
            cum += x[0]
        return out

    def run_tasks(tasks, val, z):
        for (kind, i) in sorted(set().union(*[x[2] for x in tasks])) if tasks else []:
            (ks if kind == 'k' else hs)[i][z, 2 * B:2 * B + 8, 0:128] = val
        for x in tasks:
            x[4](0)
        probes = {}
        for x in tasks:
            probes[x[3][0]] = x[3][1]
        return probes

    def probe(probes, z):
        vals = []
        if 'zp' in probes:
            vals.append(zp[probes['zp'] + z, 0:8, 0:128])
        if 'zb' in probes:
            vals.append(zb[z, 0:16, 0:128].astype(f32)[0:8])
        return vals

    def sync(vals):
        v = vals[0]
        for w in vals[1:]:
            v = v + w
        return _lsum(v)

    def inv(p, z):
        im = im_v[...]
        res = []
        for d in range(2):
            for c in range(0, D, CW):
                y = jnp.dot(im, zb[d + z, :, c:c + CW], preferred_element_type=f32)
                res.append(y)
                y_v[p, d * B:(d + 1) * B, c:c + CW] = y
        return res

    R = range(0, TM, LR)

    def corner(acc):
        return acc[acc.shape[0] - 8:, acc.shape[1] - 128:]

    def b16(v):
        return jnp.concatenate([v, v], axis=0).astype(bf16)

    def stat_part(x, i, r, n):
        w = x.shape[1]
        mu = _part(x) * (128.0 / w)
        dv = x - _wide(mu, w)
        ps[i, r:r + n] = mu
        ps[i + 1, r:r + n] = _part(dv * dv)

    def stat_mean(i, j, w, z):
        mu = ps[i + z]
        m = _lsum(mu) * (1.0 / 128)
        st[j] = m
        e = mu - m
        ps[i] = ps[i + 1 + z] + (w / 128.0) * (e * e)

    def stat_rstd(i, j, w, z):
        st[j + 1] = lax.rsqrt(_lsum(ps[i + z]) * (1.0 / w) + EPS)

    def norm(x, j, r, n):
        w = x.shape[1]
        return (x - _wide(st[j, r:r + n], w)) * _wide(st[j + 1, r:r + n], w)

    PG = 6

    def z_dot(xn, n):
        return jnp.dot(xn, win[:, n * TN:(n + 1) * TN], preferred_element_type=f32)

    def kick():
        return jnp.dot(fm_v[0:16, :], fm_v[0:128, :], preferred_element_type=f32)

    def lead(ref, i):
        return ref[i, 0:16, 0:128].astype(f32)[0:8]

    def tile_rows(t, r, n):
        if isinstance(t, int):
            return slice(t * TM // 2 + r, t * TM // 2 + r + n)
        return pl.ds(pl.multiple_of(t * (TM // 2) + r, 8), n)

    def block(items):
        z = [zs[j] for j in range(8)]
        c = dict(sg=None, acc=None, vals=[], xn={}, ng=0, rel=[])

        def release(ref):
            if not any(ref is x for x in c['rel']):
                c['rel'].append(ref)
                ref[z[0], TM:TM + 8, 0:128] = c['sg']

        def mxu(res):
            if c['sg'] is None:
                c['sg'] = res[0][0:8, 0:128]
            c['acc'] = res[-1]

        def get_xn(i):
            if i not in c['xn']:
                c['xn'][i] = pltpu.bitcast(xn_v[i, 0:TM // 2], bf16)
            return c['xn'][i]

        for it in items:
            kind = it[0]
            sg = c['sg']
            if kind == 'kick':
                mxu([kick()])
            elif kind == 'z1':
                for n in it[3]:
                    acc = z_dot(get_xn(it[2]), n)
                    z1_v[it[1], :, n * TN:(n + 1) * TN] = _gelu(acc).astype(bf16)
                    mxu([acc])
            elif kind == 'z2':
                for n in it[3]:
                    acc = z_dot(get_xn(it[2]), NCH + n)
                    it[1][0][it[1][1], 0:TM, n * TN:(n + 1) * TN] = _gelu(acc)
                    mxu([acc])
            elif kind == 'inv':
                mxu(inv(it[1], z[1] if it[2] else 0))
            elif kind == 'fwh':
                mxu(fw_h(it[1]))
            elif kind == 'fwk':
                mxu(fw_k(it[1], z[1] if it[2] else 0))
            elif kind == 'g':
                if c.get('wt') is not it[1]:
                    c['wt'], c['ws'] = it[1], wsp[it[1]]
                ws = c['ws']
                bbt = _wide(bb_v[it[1]], TN)
                for n in it[3]:
                    acc = jnp.dot(ws, _h(it[2][:, n * TN:(n + 1) * TN]), preferred_element_type=f32)
                    u = (z1_v[it[1], :, n * TN:(n + 1) * TN].astype(f32) * (acc + bbt)).astype(bf16)
                    u = pltpu.bitcast(u, u32)
                    if n < NCH - 1:
                        ua[0, 0:TM // 2, n * TN:(n + 1) * TN] = u
                    else:
                        ub[0, 0:TM // 2] = u
                    mxu([acc])
            elif kind == 'o':
                ua[z[1], TM // 2:TM // 2 + 8, 0:128] = pltpu.bitcast(sg, u32)
                ub[z[1], TM // 2:TM // 2 + 8, 0:128] = pltpu.bitcast(sg, u32)
                u = _h(jnp.concatenate([ua[0, 0:TM // 2], ub[0, 0:TM // 2]], axis=1))
                for n in range(D // TN):
                    acc = jnp.dot(u, wout[:, n * TN:(n + 1) * TN], preferred_element_type=f32)
                    x2 = (zp if it[2] is None else x_v)[it[1], 0:TM, n * TN:(n + 1) * TN] + acc
                    if it[2] is None:
                        z1_v[it[1], :, n * TN:(n + 1) * TN] = x2.astype(bf16)
                        if n == it[3]:
                            it[4].start()
                    else:
                        xa[it[2], 0:TM, n * TN:(n + 1) * TN] = x2
                    mxu([acc])
            elif kind == 'xn':
                release(it[1])
                for r in R:
                    if it[4]:
                        xn_v[1 - it[3], r // 2:(r + LR) // 2] = xn_v[it[3], r // 2:(r + LR) // 2]
                    xn_v[it[3], r // 2:(r + LR) // 2] = pltpu.bitcast(
                        norm(it[1][it[2], r:r + LR], 2, r, LR).astype(bf16), u32)
                xn_v[z[1], TM // 2:TM // 2 + 8, 0:128] = pltpu.bitcast(sg, u32)
                c['xn'] = {}
                if it[4]:
                    c['vals'].append(pltpu.bitcast(xn_v[it[3] + z[6], 0:8, 0:128], f32))
            elif kind == 'xmove':
                xn_v[0, 0:TM // 2] = xn_v[1, 0:TM // 2]
            elif kind == 'z2n':
                release(it[2][0])
                for r in R:
                    it[3][tile_rows(it[1], r // 2, LR // 2), :] = pltpu.bitcast(
                        norm(it[2][0][it[2][1], r:r + LR], it[4], r, LR).astype(bf16), u32)
                c['vals'].append(pltpu.bitcast(it[3][tile_rows(it[1] + z[6], 0, 8), 0:128], f32))
            elif kind == 'qstat':
                qb[z[0], TM:TM + 16, 0:128] = b16(sg)
                for r in R:
                    stat_part(qb[it[1] % 2, r:r + LR].astype(f32), 0, r, LR)
            elif kind == 'zstat':
                release(it[1][0])
                for r in range(0, TM, 8):
                    stat_part(it[1][0][it[1][1], r:r + 8], 2, r, 8)
            elif kind == 'x1':
                if it[2]:
                    qb[z[0], TM:TM + 16, 0:128] = b16(sg)
                for r in R:
                    x0 = qb[it[1] % 2, r:r + LR].astype(f32)
                    x1 = x0 + norm(x0, 0, r, LR) * y_v[it[1] + (0 if it[2] else z[1]), r:r + LR]
                    x_v[it[1], r:r + LR] = x1
                    stat_part(x1, 0, r, LR)
            elif kind == 'x2stat':
                release(xa)
                for r in R:
                    stat_part(xa[it[1], r:r + LR], 4, r, LR)
            elif kind == 'x3':
                release(xa)
                for r in R:
                    x0 = xa[it[2], r:r + LR]
                    x1 = x0 + norm(x0, 0, r, LR) * y_v[it[1], r:r + LR]
                    zp[it[1], r:r + LR] = x1
                    stat_part(x1, 0, r, LR)
            elif kind == 'kvprep':
                kb[z[0], B:B + 16, 0:128] = b16(sg)
                kvprep(it[1], 0)
                if not it[2]:
                    c['vals'].append(lead(kvb, (2 * it[1]) % 4 + z[6]))
            elif kind == 'terms':
                c['vals'] += probe(run_tasks(it[1], sg, z[0]), z[6])
            elif kind == 'mean' or kind == 'rstd':
                gate = corner(c['acc'])
                if len(it) > 2:
                    for v in c['vals']:
                        gate = gate + v
                    c['vals'] = []
                ps[PG + z[2], 8 * c['ng']:8 * c['ng'] + 8] = gate
                c['ng'] += 1
                for (i, j, w) in it[1]:
                    (stat_mean if kind == 'mean' else stat_rstd)(i, j, w, 0)
            elif kind == 'bb':
                bs16 = bspb[...].astype(f32)
                for i in range(S // 128):
                    bb_v[i // 2, (i % 2) * 128:(i % 2 + 1) * 128, :] = jnp.transpose(
                        jnp.broadcast_to(bs16[i:i + 1, :], (128, 128)))
        if c['vals']:
            ps[PG, 64:72] = sync([c['acc'][0:8, 0:128]] + c['vals'])

    def run(name, items):
        with jax.named_scope(name):
            pl.when(zs[15] == 0)(lambda: block(items))

    SQ, SX, SZ, S2, SL = (0, 0, D), (0, 2, D), (2, 4, FH), (4, 0, D), (2, 6, FH)
    Z0 = (zt[0], 0)
    ALL = list(range(NCH))

    def block_p0():
        kvprep(0, 0)

    def block_p1():
        fw_k(0, 0)
        fw_h(0)

    def block_p2():
        z = [zs[j] for j in range(4)]
        sg = fw_h(1)[0][0:8, 0:128]
        run_tasks(term_tasks([(0, [0], True, True), (1, [0, 1], True, True)], 0), sg, z[1])
        qb[0, TM:TM + 16, 0:128] = b16(sg)
        for r in R:
            stat_part(qb[z[1], r:r + LR].astype(f32), 0, r, LR)
        stat_mean(0, 0, D, z[2])
        inv(0, z[0])
        stat_rstd(0, 0, D, z[3])

    def block_p3():
        kvprep(1, 0)
        fw_k(1, zs[0])
        for r in R:
            x0 = qb[0, r:r + LR].astype(f32)
            x1 = x0 + norm(x0, 0, r, LR) * y_v[0, r:r + LR]
            x_v[0, r:r + LR] = x1
            xn_v[0, r // 2:(r + LR) // 2] = pltpu.bitcast(_ln(x1).astype(bf16), u32)

    for name, waits, fn, nxt in (
            ('P0', ((0, 0), (1, 0)), block_p0, [pair_copy(3, 0), pair_copy(2, 1)]),
            ('P1', ((2, 0),), block_p1, [pair_copy(0, 1), pair_copy(1, 1)]),
            ('P2', ((3, 0), (2, 1)), block_p2, [w_copy(0)]),
            ('P3', ((0, 1), (1, 1)), block_p3, [pair_copy(3, 1), w_copy(1)])):
        issue(*nxt)
        for (j, p) in waits:
            pair_copy(j, p).wait()
        with jax.named_scope(name):
            pl.when(zs[15] == 0)(fn)

    for t in range(NT):
        conv = t < NT - 1
        ta = term_tasks(plan[('A', t)], -1) if conv else []
        tb = term_tasks(plan[('B', t)], -1) if conv else []
        if t == 0:
            ch = split_tasks(ta, [3, 1.5, 2])
            issue(w_copy(2))
            w_copy(0).wait()
            run('A0a', [('kick',), ('terms', ch[0]), ('z2', Z0, 0, [0, 1, 2])])
            issue(pair_copy(0, 2), pair_copy(1, 2), pair_copy(2, 2))
            pair_copy(3, 1).wait()
            w_copy(1).wait()
            run('A0b', [('kick',), ('qstat', 1), ('terms', ch[1]), ('z2', Z0, 0, [3]), ('mean', [SQ]),
                        ('z2', Z0, 0, [4])])
            issue(w_copy(3))
            w_copy(2).wait()
            run('A0c', [('kick',), ('rstd', [SQ]), ('terms', ch[2]), ('z2', Z0, 0, [5, 6])])
            issue(w_copy(4))
            for j in range(3):
                pair_copy(j, 2).wait()
            run('B0a', [('inv', 1, 0), ('kvprep', 2, 1), ('fwh', 2), ('fwk', 2, 1)])
            issue(w_copy(5), pair_copy(3, 2))
            w_copy(3).wait()
            run('B0b', [('kick',), ('zstat', Z0), ('x1', 1, 1), ('z1', 0, 0, [0, 1]), ('mean', [SX, SZ]),
                        ('z1', 0, 0, [2])])
            issue(pair_copy(0, 3), pair_copy(1, 3))
            w_copy(4).wait()
            run('B0c', [('kick',), ('rstd', [SX, SZ]), ('terms', tb), ('bb',), ('z1', 0, 0, [3, 4, 5])])
            w_copy(5).wait()
            continue
        if t + 2 < NT:
            issue(pair_copy(2, t + 2), pair_copy(3, t + 2))
        if t + 3 < NT:
            issue(pair_copy(0, t + 3), pair_copy(1, t + 3))
        if t > 1:
            issue_big(2 * t - 3)
        if conv:
            pair_copy(3, t + 1).wait()
        if t + 2 < NT and t > 1:
            pair_copy(0, t + 2).wait()
            pair_copy(1, t + 2).wait()
        s0, s1 = t % 2, (t - 1) % 2
        za, zo = (zt[s0], 0), (zt[s1], 0)
        items = [('z1', t - 1, s1, [NCH - 1 if conv else NCH - 2]), ('xn', x_v, t, s0, 0), ('z2n', t - 1, zo, z2a, 4)]
        if conv:
            items += [('qstat', t + 1)]
            if t + 2 < NT and t > 1:
                items += [('kvprep', t + 2, 0)]
            items += [('terms', ta), ('z2', za, s0, ALL[:4]), ('mean', [SQ]), ('z2', za, s0, ALL[4:5]),
                      ('rstd', [SQ]), ('z2', za, s0, ALL[5:])]
        else:
            items += [('z2', za, s0, ALL)]
        run('A%d' % t, items)
        if conv:
            issue_big(2 * t - 2)
        if t == 1:
            pair_copy(0, t + 2).wait()
            pair_copy(1, t + 2).wait()
        if t + 2 < NT:
            pair_copy(2, t + 2).wait()
        if conv:
            items = [('inv', t + 1, 0), ('zstat', za), ('x1', t + 1, 0)]
            if t == 1:
                items += [('kvprep', t + 2, 1)]
            items += [('terms', tb)]
            if t + 2 < NT:
                items += [('fwh', t + 2)]
            if t + 2 < NT and t > 1:
                items += [('fwk', t + 2, 0)]
            if t + 2 < NT:
                items += [('z1', t, s0, ALL[:2]), ('mean', [SZ]), ('z1', t, s0, ALL[2:3]), ('mean', [SX]),
                          ('z1', t, s0, ALL[3:4]), ('rstd', [SZ])]
                if t == 1:
                    items += [('fwk', t + 2, 1)]
                items += [('z1', t, s0, ALL[4:5]), ('rstd', [SX]), ('z1', t, s0, ALL[5:6])]
            else:
                items += [('z1', t, s0, ALL[:2]), ('mean', [SZ]), ('z1', t, s0, ALL[2:3]), ('mean', [SX]),
                          ('rstd', [SZ]), ('z1', t, s0, ALL[3:4]), ('rstd', [SX]), ('z1', t, s0, ALL[4:5])]
            run('B%d' % t, items)
        else:
            run('B7a', [('kick',), ('zstat', za), ('z1', t, s0, [0]), ('mean', [SZ]), ('z1', t, s0, [1]),
                        ('rstd', [SZ]), ('z1', t, s0, [2])])
            run('B7b', [('kick',), ('z2n', t, za, z2a, 4), ('z1', t - 1, s1, [NCH - 1])])

    for cp in big[-2:]:
        cp.wait()

    def stage_c(full, i, carry):
        p0 = lax.rem(i, 2)
        p1 = 1 - p0
        fx = [('x3', jnp.maximum(i - 2, 0), p0), ('x2stat', p1)]
        if not full:
            run('V1', [('g', i, z2a, ALL[:1]), ('xmove',)] + fx + [('g', i, z2a, ALL[1:3]), ('mean', [SX]),
                       ('g', i, z2a, ALL[3:4]), ('mean', [S2]), ('g', i, z2a, ALL[4:5]), ('rstd', [SX]),
                       ('g', i, z2a, ALL[5:6]), ('rstd', [S2]), ('g', i, z2a, ALL[6:]), ('o', i, p0)])
            return carry
        t4 = lax.rem(i + NT - 4, NT)
        run('V2', [('g', i, z2a, ALL[:1]), ('xn', zp, i - 3, 0, 1)] + fx
            + [('z2n', jnp.maximum(i - 5, 0), (zc, p1), z2b, 4), ('zstat', (zc, p0)),
               ('g', i, z2a, ALL[1:5]), ('mean', [SX], 1), ('g', i, z2a, ALL[5:6]), ('mean', [SZ]),
               ('g', i, z2a, ALL[6:]), ('mean', [S2]), ('z1', t4, 1, ALL[3:4]), ('rstd', [SX]),
               ('z1', t4, 1, ALL[4:5]), ('rstd', [SZ]), ('z1', t4, 1, ALL[5:6]), ('rstd', [S2]),
               ('z1', t4, 1, ALL[6:]), ('z1', i - 3, 0, ALL[:3]), ('z2', (zc, p1), 0, ALL), ('o', i, p0)])
        return carry

    def stage_d(t, carry):
        @pl.when(t >= 2)
        def _():
            for j in range(3):
                out_copy(jnp.maximum(t - 2, 0), j).wait()

        t0, t1 = 2 * t, 2 * t + 1
        run('D', [('g', t0, z2b, ALL), ('o', t0, None, D // TN - 1, out_copy(t, 0)),
                  ('g', t1, z2b, ALL), ('o', t1, None, OS - 1, out_copy(t, 1))])
        out_copy(t, 2).start()
        return carry

    lax.fori_loop(0, 3, functools.partial(stage_c, False), 0)
    lax.fori_loop(3, NT, functools.partial(stage_c, True), 0)
    zbuf = {3: (zc, 1), 4: (zc, 0), 5: (zt[0], 0), 6: (zt[1], 0), 7: (zc, 0)}
    for i in range(NT, NT + 3):
        p0, p1 = i % 2, (i + 1) % 2
        sz_old, sz_new = (SZ, SL) if p0 == 0 else (SL, SZ)
        items = [('z1', i - 4, p0, ALL[3:4]), ('xn', zp, i - 3, p1, 0), ('z2n', i - 5, zbuf[i - 5], z2b, sz_old[1]),
                 ('zstat', zbuf[i - 4])]
        stats = [sz_new]
        if i - 2 < NT:
            items += [('x3', i - 2, p0)]
            stats += [SX]
        if i - 1 < NT:
            items += [('x2stat', p1)]
            stats += [S2]
        items += [('z1', i - 4, p0, ALL[4:]), ('z1', i - 3, p1, ALL[:3])]
        gates = [('mean', [x]) for x in stats] + [('rstd', [x]) for x in stats]
        for n in ALL:
            items += gates[n:n + 1] + [('z2', zbuf[i - 3], p1, [n])]
        run('V3%d' % i, items)
    t = NT - 1
    run('T1', [('kick',), ('zstat', zbuf[t]), ('z2n', t - 1, zbuf[t - 1], z2b, SL[1]), ('z1', t, 1, [3]),
               ('mean', [SZ]), ('z1', t, 1, [4]), ('rstd', [SZ]), ('z1', t, 1, [5])])
    run('T2', [('kick',), ('z2n', t, zbuf[t], z2b, SZ[1]), ('z1', t, 1, [6])])
    lax.fori_loop(0, NT // 2, stage_d, 0)
    for t in range(NT // 2 - 2, NT // 2):
        for j in range(3):
            out_copy(t, j).wait()


@jax.jit
def pallas_interleave_layers__ssm_conv_h3__mixer_gmlp__prompt_kernel(
        A_q, A_k, A_v, A_shift_k, A_ssm_k, A_ssm_D, B_x, B_w_in, B_w_sp, B_b_sp, B_w_out):
    del B_x
    any_spec = pl.BlockSpec(memory_space=pl.ANY)
    scratch = [
        pltpu.VMEM((2, TM + 16, D), bf16),
        pltpu.VMEM((8, B + 16, D), bf16),
        pltpu.VMEM((8, B, D), bf16),
        pltpu.VMEM((2, D, TM), bf16),
        pltpu.VMEM((D, F), bf16),
        pltpu.VMEM((NT, TM, S), bf16),
        pltpu.VMEM((FH, D), bf16),
        pltpu.VMEM((KS, D), bf16),
        pltpu.VMEM((8, 128), bf16),
        pltpu.VMEM((16, 128), bf16),
        pltpu.VMEM((NT, TM + 8, D), f32),
        pltpu.VMEM((NT, TM, D), f32),
        pltpu.VMEM((NT, TM, FH), bf16),
        pltpu.VMEM((S // 2, FH), u32),
        pltpu.VMEM((S // 2, FH), u32),
        pltpu.VMEM((NT, TM, 128), f32),
        pltpu.VMEM((KS + 1, 8, D), f32),
        pltpu.VMEM((2 * B, B), bf16),
        pltpu.VMEM((B, 2 * B), bf16),
        pltpu.VMEM((4, B, D), bf16),
        [pltpu.VMEM((2, 2 * B + 8, D), f32)] * NT,
        [pltpu.VMEM((2, 2 * B + 8, D), f32)] * NT,
        pltpu.VMEM((1, TM, D), f32),
        pltpu.VMEM((NZ, 2 * B + 8, D), f32),
        pltpu.VMEM((2, 2 * B, D), bf16),
        pltpu.VMEM((2, TM // 2 + 8, D), u32),
        [pltpu.VMEM((1, TM + 8, FH), f32)] * 2,
        pltpu.VMEM((2, TM + 8, FH), f32),
        pltpu.VMEM((2, TM + 8, D), f32),
        pltpu.VMEM((7, TM, 128), f32),
        pltpu.VMEM((8, TM, 128), f32),
        pltpu.VMEM((1, TM // 2 + 8, FH - TN), u32),
        pltpu.VMEM((1, TM // 2 + 8, TN), u32),
        pltpu.SMEM((16,), jnp.int32),
        pltpu.SemaphoreType.DMA((8,)),
        pltpu.SemaphoreType.DMA((3,)),
        pltpu.SemaphoreType.DMA((2,)),
        pltpu.SemaphoreType.DMA((6,)),
    ]
    out = pl.pallas_call(
        _kernel,
        out_shape=jax.ShapeDtypeStruct((NT, TM, D), bf16),
        in_specs=[any_spec] * 10,
        out_specs=any_spec,
        scratch_shapes=scratch,
        compiler_params=pltpu.CompilerParams(vmem_limit_bytes=127 * 1024 * 1024),
    )(A_q.reshape(NT, TM, D), A_k.reshape(NB, B, D), A_v.reshape(NB, B, D), A_shift_k.T, A_ssm_k,
      A_ssm_D.reshape(8, 128), B_w_in, B_w_sp.reshape(NT, TM, S), B_b_sp.reshape(16, 128), B_w_out)
    return out.reshape(1, S, D)
```

```python
import functools
import math
import jax
import jax.numpy as jnp
from jax import lax
import jax.experimental.pallas as pl
import jax.experimental.pallas.tpu as pltpu

S = 2048
D = 1024
F = 3584
FH = F // 2
KS = 4
B = 128
NB = S // B
EPS = 1e-5
f32 = jnp.float32
bf16 = jnp.bfloat16
u32 = jnp.uint32

TM = 256
NT = S // TM
TN = 256
NCH = FH // TN
RG = 16
GW = 256
LR = 16
NZ = 8
CAP_A = 9
CAP_B = 14
GWF = 128
OS = 3
ROT = 256


def _plan(cap_a, cap_b):
    done = set((a, ap) for a in (0, 1) for ap in range(a + 1))
    blocks = {}
    for t in range(NT - 1):
        for kind, cap in (('A', cap_a), ('B', cap_b)):
            if (kind, t) == ('A', 1):
                cap += 4
            if (kind, t) == ('B', NT - 3):
                cap -= 3
            sel = {}
            n = 0
            lo = 2 * t + 2 if kind == 'A' else 2 * t + 4
            lim = 2 * t + 3
            for a in range(lo, NB):
                g = [ap for ap in range(a + 1) if (a, ap) not in done and ap <= lim and a - ap <= lim]
                if a > lim:
                    g = g[:max(cap - n, 0)]
                if g:
                    sel[a] = g
                    n += len(g)
            groups = []
            for a in sorted(sel):
                first = not any((a, x) in done for x in range(a + 1))
                done.update((a, x) for x in sel[a])
                last = all((a, x) in done for x in range(a + 1))
                assert a < lo + NZ and last == (a <= 2 * t + 3)
                groups.append((a, sel[a], first, last))
            blocks[(kind, t)] = groups
    assert len(done) == NB * (NB + 1) // 2
    return blocks


def _gelu(x):
    u = x * (0.7978845608028654 + 0.035677408136300125 * (x * x))
    h = 0.5 * x
    return h + h * jnp.tanh(u)


def _h(v):
    return pltpu.bitcast(v, bf16)


def _part(v):
    acc = v[:, 0:128]
    for c in range(128, v.shape[1], 128):
        acc = acc + v[:, c:c + 128]
    return acc


def _lsum(acc):
    return jnp.broadcast_to(jnp.sum(acc, axis=1, keepdims=True), acc.shape)


def _wide(v, n):
    return jnp.concatenate([v] * (n // 128), axis=1)


def _ln(x):
    n = x.shape[-1]
    m = jnp.sum(x, axis=-1, keepdims=True) * (1.0 / n)
    xc = x - m
    v = jnp.sum(xc * xc, axis=-1, keepdims=True) * (1.0 / n)
    return xc * lax.rsqrt(v + EPS)


def _dft_rows(shape, row_dim):
    r = lax.broadcasted_iota(jnp.int32, shape, row_dim)
    n = lax.broadcasted_iota(jnp.int32, shape, 1 - row_dim)
    is_im = r >= B
    rr = jnp.where(is_im, r - B, r)
    odd = rr >= B // 2
    fidx = jnp.where(odd, 2 * (rr - B // 2) + 1, 2 * rr)
    m = (2 * fidx + 1) * n - jnp.where(is_im, B, 0)
    m = jnp.bitwise_and(m, 4 * B - 1)
    m = jnp.where(m > 2 * B, 4 * B - m, m)
    return jnp.cos(m.astype(f32) * (math.pi / (2 * B)))


NT_DIMS = (((1,), (1,)), ((), ()))


def _kernel(q_hbm, k_hbm, v_hbm, sk_hbm, h_hbm, sd_hbm, win_hbm, wsp_hbm, bsp_hbm, wout_hbm,
            o_hbm,
            qb, kb, vb, hb, win, wsp, wout, skb, sdb, bspb,
            x_v, y_v, z1_v, z2a, z2b, bb_v, skt, fm_v, im_v, kvb, ks, hs, wold, zp, zb,
            xn_v, zt, zc, ps, st, ua, ub, zs,
            sem_c, sem_w, sem_s, sem_o):
    plan = _plan(CAP_A, CAP_B)
    xa = ks[0]

    def pair_copy(j, p):
        if j == 0:
            return pltpu.make_async_copy(k_hbm.at[pl.ds(2 * p, 2)], kb.at[pl.ds(2 * p % 8, 2), pl.ds(0, B)], sem_c.at[p % 2])
        if j == 1:
            return pltpu.make_async_copy(v_hbm.at[pl.ds(2 * p, 2)], vb.at[pl.ds(2 * p % 8, 2)], sem_c.at[2 + p % 2])
        if j == 2:
            cols = pl.ds(p * TM, TM)
            return pltpu.make_async_copy(h_hbm.at[:, cols], hb.at[p % 2], sem_c.at[4 + p % 2])
        return pltpu.make_async_copy(q_hbm.at[p], qb.at[p % 2, pl.ds(0, TM)], sem_c.at[6 + p % 2])

    WG = ((7, 10), (10, 12), (12, 14), (0, 3), (3, 6), (6, 7))

    def w_copy(i):
        cols = pl.ds(WG[i][0] * TN, (WG[i][1] - WG[i][0]) * TN)
        return pltpu.make_async_copy(win_hbm.at[:, cols], win.at[:, cols], sem_w.at[i % 3])

    def out_copy(t, j):
        cols = (pl.ds(0, D), pl.ds(0, OS * TN), pl.ds(OS * TN, D - OS * TN))[j]
        i = 2 * t + min(j, 1)
        return pltpu.make_async_copy(z1_v.at[i, :, cols], o_hbm.at[i, :, cols], sem_o.at[3 * (t % 2) + j])

    def issue(*copies):
        for cp in copies:
            cp.start(priority=1)

    def issue_big(j):
        if j >= 2:
            big[j - 2].wait()
        issue(big[j])

    small = [
        pltpu.make_async_copy(sk_hbm, skb, sem_o.at[0]),
        pltpu.make_async_copy(sd_hbm, sdb, sem_o.at[1]),
        pltpu.make_async_copy(bsp_hbm, bspb, sem_o.at[2]),
    ]
    WR = FH // 4
    big = ([pltpu.make_async_copy(wsp_hbm.at[j], wsp.at[j], sem_s.at[j % 2]) for j in range(NT)]
           + [pltpu.make_async_copy(wout_hbm.at[pl.ds(j * WR, WR)], wout.at[pl.ds(j * WR, WR)], sem_s.at[j % 2])
              for j in range(4)])
    for cp in small:
        cp.start()
    pair_copy(0, 0).start(priority=1)
    pair_copy(1, 0).start(priority=1)

    def zinit(i, c):
        zs[i] = 0
        return c
    lax.fori_loop(0, 16, zinit, 0)
    issue(pair_copy(2, 0))

    fm_v[...] = _dft_rows((2 * B, B), 0).astype(bf16)
    im_v[...] = (_dft_rows((B, 2 * B), 1) * (1.0 / B)).astype(bf16)

    for cp in small:
        cp.wait()
    sk4 = skb[...].astype(f32)
    for j in range(KS):
        skt[j] = jnp.broadcast_to(sk4[j:j + 1, :], (8, D))
    sd8 = sdb[...].astype(f32)
    skt[KS] = jnp.concatenate([jnp.broadcast_to(sd8[i:i + 1, :], (8, 128)) for i in range(8)], axis=1)

    def kvprep(p, z):
        for a in (2 * p, 2 * p + 1):
            for c in range(0, D, GW):
                for r0 in range(0, B, 32):
                    kcur = kb[a % 8 + z, r0:r0 + 32, c:c + GW].astype(f32)
                    if a == 0 and r0 == 0:
                        kprev = jnp.zeros((8, GW), f32)
                    elif r0 == 0:
                        kprev = kb[(a - 1) % 8 + z, B - 16:B, c:c + GW].astype(f32)[8:16]
                    else:
                        kprev = kb[a % 8 + z, r0 - 16:r0, c:c + GW].astype(f32)[8:16]
                    ext = jnp.concatenate([kprev, kcur], axis=0)
                    sk = [jnp.concatenate([skt[j, :, c:c + GW]] * 4, axis=0) for j in range(KS)]
                    acc = kcur * sk[0]
                    for j in range(1, KS):
                        acc = acc + pltpu.roll(ext, j, 0)[8:] * sk[j]
                    kvb[a % 4, r0:r0 + 32, c:c + GW] = (acc * vb[a % 8, r0:r0 + 32, c:c + GW].astype(f32)).astype(bf16)

    CW = 512

    def rot(c, k, w):
        c = (c + ROT * k) % D
        return slice(c, c + w)

    def put(ref, i, c, val, k):
        for j in range(0, CW, 256):
            ref[i, 0:B, rot(c + j, k, 256)] = val[0:B, j:j + 256]
            ref[i, B:2 * B, rot(c + j, k + 2, 256)] = val[B:2 * B, j:j + 256]

    def fw_h(p):
        fm = fm_v[...]
        res = []
        for a in (2 * p, 2 * p + 1):
            for c in range(0, D, CW):
                hh = lax.dot_general(fm, hb[p % 2, c:c + CW, (a % 2) * B:(a % 2 + 1) * B], NT_DIMS,
                                     preferred_element_type=f32)
                res.append(hh)
                if a == 0:
                    sd = jnp.concatenate([skt[KS, :, c:c + CW]] * (B // 8), axis=0)
                    hh = jnp.concatenate([hh[0:B] + sd, hh[B:2 * B]], axis=0)
                put(hs[p], a % 2, c, hh, 1)
        return res

    def fw_k(p, zk):
        fm = fm_v[...]
        res = []
        for a in (2 * p, 2 * p + 1):
            for c in range(0, D, CW):
                hh = jnp.dot(fm, kvb[a % 4 + zk, :, c:c + CW], preferred_element_type=f32)
                res.append(hh)
                put(ks[p], a % 2, c, hh, 0)
        return res

    def term_tasks(groups, newp):
        def acc(a, g, first, r, c, z, GW):
            zr = zi = None
            for ap in g:
                d = a - ap
                xr = ks[ap // 2][ap % 2 + z, r:r + RG, c:c + GW]
                xi = ks[ap // 2][ap % 2 + z, B + r:B + r + RG, rot(c, 2, GW)]
                hr = hs[d // 2][d % 2 + z, r:r + RG, rot(c, 1, GW)]
                hi = hs[d // 2][d % 2 + z, B + r:B + r + RG, rot(c, 3, GW)]
                tr = xr * hr - xi * hi
                ti = xr * hi + xi * hr
                zr = tr if zr is None else zr + tr
                zi = ti if zi is None else zi + ti
            if not first:
                zr = zr + zp[a % NZ, r:r + RG, c:c + GW]
                zi = zi + zp[a % NZ, B + r:B + r + RG, c:c + GW]
            return zr, zi

        def part_task(a, g, first, r, c, z):
            zr, zi = acc(a, g, first, r, c, z, GW)
            zp[a % NZ, r:r + RG, c:c + GW] = zr
            zp[a % NZ, B + r:B + r + RG, c:c + GW] = zi

        def fin_task(fin, r, c, z):
            GW = GWF
            if fin[0][0] > 0:
                pr = wold[0, r:r + RG, c:c + GW]
                pi = wold[0, B + r:B + r + RG, c:c + GW]
            for (a, g, first, last) in fin:
                wr, wi = acc(a, g, first, r, c, z, GW)
                if a == 0:
                    zr, zi = wr, wi
                elif r < B // 2:
                    zr, zi = wr + pi, wi - pr
                else:
                    zr, zi = wr - pi, wi + pr
                zb[a % 2, r:r + RG, c:c + GW] = zr.astype(bf16)
                zb[a % 2, B + r:B + r + RG, c:c + GW] = zi.astype(bf16)
                pr, pi = wr, wi
            if fin[-1][0] < NB - 1:
                wold[0, r:r + RG, c:c + GW] = pr
                wold[0, B + r:B + r + RG, c:c + GW] = pi

        def srcs(gs):
            return (set(('k', ap // 2) for (a, g, _, _) in gs for ap in g)
                    | set(('h', (a - ap) // 2) for (a, g, _, _) in gs for ap in g))

        rc = [(r, c) for r in range(0, B, RG) for c in range(0, D, GW)]
        tasks = []
        for grp in groups:
            a, g, first, last = grp
            if not last:
                sr = srcs([grp])
                new = any(i == newp for (_, i) in sr)
                tasks += [(len(g), new, sr, ('zp', a % NZ),
                           functools.partial(part_task, a, g, first, r, c)) for (r, c) in rc]
        tasks.sort(key=lambda x: x[1])
        fin = [x for x in groups if x[3]]
        if fin:
            tasks += [(sum(len(x[1]) for x in fin) + 1, True, srcs(fin), ('zb', 0),
                       functools.partial(fin_task, fin, r, c)) for r in range(0, B, RG) for c in range(0, D, GWF)]
        return tasks

    def split_tasks(tasks, caps):
        total = sum(x[0] for x in tasks)
        out = [[] for _ in caps]
        cum = 0
        for x in tasks:
            pos = (cum + 0.5 * x[0]) / max(total, 1) * sum(caps)
            k = 0
            while k + 1 < len(caps) and pos > sum(caps[:k + 1]):
                k += 1
            out[k].append(x)
            cum += x[0]
        return out

    def run_tasks(tasks, val, z):
        for (kind, i) in sorted(set().union(*[x[2] for x in tasks])) if tasks else []:
            (ks if kind == 'k' else hs)[i][z, 2 * B:2 * B + 8, 0:128] = val
        for x in tasks:
            x[4](0)
        probes = {}
        for x in tasks:
            probes[x[3][0]] = x[3][1]
        return probes

    def probe(probes, z):
        vals = []
        if 'zp' in probes:
            vals.append(zp[probes['zp'] + z, 0:8, 0:128])
        if 'zb' in probes:
            vals.append(zb[z, 0:16, 0:128].astype(f32)[0:8])
        return vals

    def sync(vals):
        v = vals[0]
        for w in vals[1:]:
            v = v + w
        return _lsum(v)

    def inv(p, z):
        im = im_v[...]
        res = []
        for d in range(2):
            for c in range(0, D, CW):
                y = jnp.dot(im, zb[d + z, :, c:c + CW], preferred_element_type=f32)
                res.append(y)
                y_v[p, d * B:(d + 1) * B, c:c + CW] = y
        return res

    R = range(0, TM, LR)

    def corner(acc):
        return acc[acc.shape[0] - 8:, acc.shape[1] - 128:]

    def b16(v):
        return jnp.concatenate([v, v], axis=0).astype(bf16)

    def stat_part(x, i, r, n):
        w = x.shape[1]
        mu = _part(x) * (128.0 / w)
        dv = x - _wide(mu, w)
        ps[i, r:r + n] = mu
        ps[i + 1, r:r + n] = _part(dv * dv)

    def stat_mean(i, j, w, z):
        mu = ps[i + z]
        m = _lsum(mu) * (1.0 / 128)
        st[j] = m
        e = mu - m
        ps[i] = ps[i + 1 + z] + (w / 128.0) * (e * e)

    def stat_rstd(i, j, w, z):
        st[j + 1] = lax.rsqrt(_lsum(ps[i + z]) * (1.0 / w) + EPS)

    def norm(x, j, r, n):
        w = x.shape[1]
        return (x - _wide(st[j, r:r + n], w)) * _wide(st[j + 1, r:r + n], w)

    PG = 6

    def z_dot(xn, n):
        return jnp.dot(xn, win[:, n * TN:(n + 1) * TN], preferred_element_type=f32)

    def kick():
        return jnp.dot(fm_v[0:16, :], fm_v[0:128, :], preferred_element_type=f32)

    def lead(ref, i):
        return ref[i, 0:16, 0:128].astype(f32)[0:8]

    def tile_rows(t, r, n):
        if isinstance(t, int):
            return slice(t * TM // 2 + r, t * TM // 2 + r + n)
        return pl.ds(pl.multiple_of(t * (TM // 2) + r, 8), n)

    def block(items):
        z = [zs[j] for j in range(8)]
        c = dict(sg=None, acc=None, vals=[], xn={}, ng=0, rel=[])

        def release(ref):
            if not any(ref is x for x in c['rel']):
                c['rel'].append(ref)
                ref[z[0], TM:TM + 8, 0:128] = c['sg']

        def mxu(res):
            if c['sg'] is None:
                c['sg'] = res[0][0:8, 0:128]
            c['acc'] = res[-1]

        def get_xn(i):
            if i not in c['xn']:
                c['xn'][i] = pltpu.bitcast(xn_v[i, 0:TM // 2], bf16)
            return c['xn'][i]

        for it in items:
            kind = it[0]
            sg = c['sg']
            if kind == 'kick':
                mxu([kick()])
            elif kind == 'z1':
                for n in it[3]:
                    acc = z_dot(get_xn(it[2]), n)
                    z1_v[it[1], :, n * TN:(n + 1) * TN] = _gelu(acc).astype(bf16)
                    mxu([acc])
            elif kind == 'z2':
                for n in it[3]:
                    acc = z_dot(get_xn(it[2]), NCH + n)
                    it[1][0][it[1][1], 0:TM, n * TN:(n + 1) * TN] = _gelu(acc)
                    mxu([acc])
            elif kind == 'inv':
                mxu(inv(it[1], z[1] if it[2] else 0))
            elif kind == 'fwh':
                mxu(fw_h(it[1]))
            elif kind == 'fwk':
                mxu(fw_k(it[1], z[1] if it[2] else 0))
            elif kind == 'g':
                if c.get('wt') is not it[1]:
                    c['wt'], c['ws'] = it[1], wsp[it[1]]
                ws = c['ws']
                bbt = _wide(bb_v[it[1]], TN)
                for n in it[3]:
                    acc = jnp.dot(ws, _h(it[2][:, n * TN:(n + 1) * TN]), preferred_element_type=f32)
                    u = (z1_v[it[1], :, n * TN:(n + 1) * TN].astype(f32) * (acc + bbt)).astype(bf16)
                    u = pltpu.bitcast(u, u32)
                    if n < NCH - 1:
                        ua[0, 0:TM // 2, n * TN:(n + 1) * TN] = u
                    else:
                        ub[0, 0:TM // 2] = u
                    mxu([acc])
            elif kind == 'o':
                ua[z[1], TM // 2:TM // 2 + 8, 0:128] = pltpu.bitcast(sg, u32)
                ub[z[1], TM // 2:TM // 2 + 8, 0:128] = pltpu.bitcast(sg, u32)
                u = _h(jnp.concatenate([ua[0, 0:TM // 2], ub[0, 0:TM // 2]], axis=1))
                for n in range(D // TN):
                    acc = jnp.dot(u, wout[:, n * TN:(n + 1) * TN], preferred_element_type=f32)
                    x2 = (zp if it[2] is None else x_v)[it[1], 0:TM, n * TN:(n + 1) * TN] + acc
                    if it[2] is None:
                        z1_v[it[1], :, n * TN:(n + 1) * TN] = x2.astype(bf16)
                        if n == it[3]:
                            it[4].start()
                    else:
                        xa[it[2], 0:TM, n * TN:(n + 1) * TN] = x2
                    mxu([acc])
            elif kind == 'xn':
                release(it[1])
                for r in R:
                    if it[4]:
                        xn_v[1 - it[3], r // 2:(r + LR) // 2] = xn_v[it[3], r // 2:(r + LR) // 2]
                    xn_v[it[3], r // 2:(r + LR) // 2] = pltpu.bitcast(
                        norm(it[1][it[2], r:r + LR], 2, r, LR).astype(bf16), u32)
                xn_v[z[1], TM // 2:TM // 2 + 8, 0:128] = pltpu.bitcast(sg, u32)
                c['xn'] = {}
                if it[4]:
                    c['vals'].append(pltpu.bitcast(xn_v[it[3] + z[6], 0:8, 0:128], f32))
            elif kind == 'xmove':
                xn_v[0, 0:TM // 2] = xn_v[1, 0:TM // 2]
            elif kind == 'z2n':
                release(it[2][0])
                for r in R:
                    it[3][tile_rows(it[1], r // 2, LR // 2), :] = pltpu.bitcast(
                        norm(it[2][0][it[2][1], r:r + LR], it[4], r, LR).astype(bf16), u32)
                c['vals'].append(pltpu.bitcast(it[3][tile_rows(it[1] + z[6], 0, 8), 0:128], f32))
            elif kind == 'qstat':
                qb[z[0], TM:TM + 16, 0:128] = b16(sg)
                for r in R:
                    stat_part(qb[it[1] % 2, r:r + LR].astype(f32), 0, r, LR)
            elif kind == 'zstat':
                release(it[1][0])
                for r in range(0, TM, 8):
                    stat_part(it[1][0][it[1][1], r:r + 8], 2, r, 8)
            elif kind == 'x1':
                if it[2]:
                    qb[z[0], TM:TM + 16, 0:128] = b16(sg)
                for r in R:
                    x0 = qb[it[1] % 2, r:r + LR].astype(f32)
                    x1 = x0 + norm(x0, 0, r, LR) * y_v[it[1] + (0 if it[2] else z[1]), r:r + LR]
                    x_v[it[1], r:r + LR] = x1
                    stat_part(x1, 0, r, LR)
            elif kind == 'x2stat':
                release(xa)
                for r in R:
                    stat_part(xa[it[1], r:r + LR], 4, r, LR)
            elif kind == 'x3':
                release(xa)
                for r in R:
                    x0 = xa[it[2], r:r + LR]
                    x1 = x0 + norm(x0, 0, r, LR) * y_v[it[1], r:r + LR]
                    zp[it[1], r:r + LR] = x1
                    stat_part(x1, 0, r, LR)
            elif kind == 'kvprep':
                kb[z[0], B:B + 16, 0:128] = b16(sg)
                kvprep(it[1], 0)
                if not it[2]:
                    c['vals'].append(lead(kvb, (2 * it[1]) % 4 + z[6]))
            elif kind == 'terms':
                c['vals'] += probe(run_tasks(it[1], sg, z[0]), z[6])
            elif kind == 'mean' or kind == 'rstd':
                gate = corner(c['acc'])
                if len(it) > 2:
                    for v in c['vals']:
                        gate = gate + v
                    c['vals'] = []
                ps[PG + z[2], 8 * c['ng']:8 * c['ng'] + 8] = gate
                c['ng'] += 1
                for (i, j, w) in it[1]:
                    (stat_mean if kind == 'mean' else stat_rstd)(i, j, w, 0)
            elif kind == 'bb':
                bs16 = bspb[...].astype(f32)
                for i in range(S // 128):
                    bb_v[i // 2, (i % 2) * 128:(i % 2 + 1) * 128, :] = jnp.transpose(
                        jnp.broadcast_to(bs16[i:i + 1, :], (128, 128)))
        if c['vals']:
            ps[PG, 64:72] = sync([c['acc'][0:8, 0:128]] + c['vals'])

    def run(name, items):
        with jax.named_scope(name):
            pl.when(zs[15] == 0)(lambda: block(items))

    SQ, SX, SZ, S2, SL = (0, 0, D), (0, 2, D), (2, 4, FH), (4, 0, D), (2, 6, FH)
    Z0 = (zt[0], 0)
    ALL = list(range(NCH))

    def block_p0():
        kvprep(0, 0)

    def block_p1():
        fw_k(0, 0)
        fw_h(0)

    def block_p2():
        z = [zs[j] for j in range(4)]
        sg = fw_h(1)[0][0:8, 0:128]
        run_tasks(term_tasks([(0, [0], True, True), (1, [0, 1], True, True)], 0), sg, z[1])
        qb[0, TM:TM + 16, 0:128] = b16(sg)
        for r in R:
            stat_part(qb[z[1], r:r + LR].astype(f32), 0, r, LR)
        stat_mean(0, 0, D, z[2])
        inv(0, z[0])
        stat_rstd(0, 0, D, z[3])

    def block_p3():
        kvprep(1, 0)
        fw_k(1, zs[0])
        for r in R:
            x0 = qb[0, r:r + LR].astype(f32)
            x1 = x0 + norm(x0, 0, r, LR) * y_v[0, r:r + LR]
            x_v[0, r:r + LR] = x1
            xn_v[0, r // 2:(r + LR) // 2] = pltpu.bitcast(_ln(x1).astype(bf16), u32)

    for name, waits, fn, nxt in (
            ('P0', ((0, 0), (1, 0)), block_p0, [pair_copy(3, 0), pair_copy(2, 1)]),
            ('P1', ((2, 0),), block_p1, [pair_copy(0, 1), pair_copy(1, 1)]),
            ('P2', ((3, 0), (2, 1)), block_p2, [w_copy(0)]),
            ('P3', ((0, 1), (1, 1)), block_p3, [pair_copy(3, 1), w_copy(1)])):
        issue(*nxt)
        for (j, p) in waits:
            pair_copy(j, p).wait()
        with jax.named_scope(name):
            pl.when(zs[15] == 0)(fn)

    for t in range(NT):
        conv = t < NT - 1
        ta = term_tasks(plan[('A', t)], -1) if conv else []
        tb = term_tasks(plan[('B', t)], -1) if conv else []
        if t == 0:
            ch = split_tasks(ta, [3, 1.5, 2])
            issue(w_copy(2))
            w_copy(0).wait()
            run('A0a', [('kick',), ('terms', ch[0]), ('z2', Z0, 0, [0, 1, 2])])
            issue(pair_copy(0, 2), pair_copy(1, 2), pair_copy(2, 2))
            pair_copy(3, 1).wait()
            w_copy(1).wait()
            run('A0b', [('kick',), ('qstat', 1), ('terms', ch[1]), ('z2', Z0, 0, [3]), ('mean', [SQ]),
                        ('z2', Z0, 0, [4])])
            issue(w_copy(3))
            w_copy(2).wait()
            run('A0c', [('kick',), ('rstd', [SQ]), ('terms', ch[2]), ('z2', Z0, 0, [5, 6])])
            issue(w_copy(4))
            for j in range(3):
                pair_copy(j, 2).wait()
            run('B0a', [('inv', 1, 0), ('kvprep', 2, 1), ('fwh', 2), ('fwk', 2, 1)])
            issue(w_copy(5), pair_copy(3, 2))
            w_copy(3).wait()
            run('B0b', [('kick',), ('zstat', Z0), ('x1', 1, 1), ('z1', 0, 0, [0, 1]), ('mean', [SX, SZ]),
                        ('z1', 0, 0, [2])])
            issue(pair_copy(0, 3), pair_copy(1, 3))
            w_copy(4).wait()
            run('B0c', [('kick',), ('rstd', [SX, SZ]), ('terms', tb), ('bb',), ('z1', 0, 0, [3, 4, 5])])
            w_copy(5).wait()
            continue
        if t + 2 < NT:
            issue(pair_copy(2, t + 2), pair_copy(3, t + 2))
        if t + 3 < NT:
            issue(pair_copy(0, t + 3), pair_copy(1, t + 3))
        if t > 1:
            issue_big(2 * t - 3)
        if conv:
            pair_copy(3, t + 1).wait()
        if t + 2 < NT and t > 1:
            pair_copy(0, t + 2).wait()
            pair_copy(1, t + 2).wait()
        s0, s1 = t % 2, (t - 1) % 2
        za, zo = [(zc, u % 2) if u >= NT - 2 else (zt[u % 2], 0) for u in (t, t - 1)]
        items = [('z1', t - 1, s1, [NCH - 1 if conv else NCH - 2]), ('xn', x_v, t, s0, 0), ('z2n', t - 1, zo, z2a, 4)]
        if conv:
            items += [('qstat', t + 1)]
            if t + 2 < NT and t > 1:
                items += [('kvprep', t + 2, 0)]
            items += [('terms', ta), ('z2', za, s0, ALL[:4]), ('mean', [SQ]), ('z2', za, s0, ALL[4:5]),
                      ('rstd', [SQ]), ('z2', za, s0, ALL[5:])]
        else:
            items += [('z2', za, s0, ALL)]
        run('A%d' % t, items)
        if conv:
            issue_big(2 * t - 2)
        if t == 1:
            pair_copy(0, t + 2).wait()
            pair_copy(1, t + 2).wait()
        if t + 2 < NT:
            pair_copy(2, t + 2).wait()
        if conv:
            items = [('inv', t + 1, 0), ('zstat', za), ('x1', t + 1, 0)]
            if t == 1:
                items += [('kvprep', t + 2, 1)]
            items += [('terms', tb)]
            if t + 2 < NT:
                items += [('fwh', t + 2)]
            if t + 2 < NT and t > 1:
                items += [('fwk', t + 2, 0)]
            if t + 2 < NT:
                items += [('z1', t, s0, ALL[:2]), ('mean', [SZ]), ('z1', t, s0, ALL[2:3]), ('mean', [SX]),
                          ('z1', t, s0, ALL[3:4]), ('rstd', [SZ])]
                if t == 1:
                    items += [('fwk', t + 2, 1)]
                items += [('z1', t, s0, ALL[4:5]), ('rstd', [SX]), ('z1', t, s0, ALL[5:6])]
            else:
                items += [('z1', t, s0, ALL[:2]), ('mean', [SZ]), ('z1', t, s0, ALL[2:3]), ('mean', [SX]),
                          ('rstd', [SZ]), ('z1', t, s0, ALL[3:4]), ('rstd', [SX]), ('z1', t, s0, ALL[4:5])]
            run('B%d' % t, items)
        else:
            run('B7a', [('kick',), ('zstat', za), ('z1', t, s0, [0]), ('mean', [SZ]), ('z1', t, s0, [1]),
                        ('rstd', [SZ]), ('z1', t, s0, [2])])
            run('B7b', [('kick',), ('z2n', t, za, z2a, 4), ('z1', t - 1, s1, [NCH - 1])])

    for cp in big[-2:]:
        cp.wait()

    def stage_c(full, i, carry):
        p0 = lax.rem(i, 2)
        p1 = 1 - p0
        fx = [('x3', jnp.maximum(i - 2, 0), p0), ('x2stat', p1)]
        if not full:
            run('V1', [('g', i, z2a, ALL[:1]), ('xmove',)] + fx + [('g', i, z2a, ALL[1:3]), ('mean', [SX]),
                       ('g', i, z2a, ALL[3:4]), ('mean', [S2]), ('g', i, z2a, ALL[4:5]), ('rstd', [SX]),
                       ('g', i, z2a, ALL[5:6]), ('rstd', [S2]), ('g', i, z2a, ALL[6:]), ('o', i, p0)])
            return carry
        t4 = lax.rem(i + NT - 4, NT)
        run('V2', [('g', i, z2a, ALL[:1]), ('xn', zp, i - 3, 0, 1)] + fx
            + [('z2n', jnp.maximum(i - 5, 0), (zc, p1), z2b, 4), ('zstat', (zc, p0)),
               ('g', i, z2a, ALL[1:5]), ('mean', [SX], 1), ('g', i, z2a, ALL[5:6]), ('mean', [SZ]),
               ('g', i, z2a, ALL[6:]), ('mean', [S2]), ('z1', t4, 1, ALL[3:4]), ('rstd', [SX]),
               ('z1', t4, 1, ALL[4:5]), ('rstd', [SZ]), ('z1', t4, 1, ALL[5:6]), ('rstd', [S2]),
               ('z1', t4, 1, ALL[6:]), ('z1', i - 3, 0, ALL[:3]), ('z2', (zc, p1), 0, ALL), ('o', i, p0)])
        return carry

    def stage_d(t, carry):
        @pl.when(t >= 2)
        def _():
            for j in range(3):
                out_copy(jnp.maximum(t - 2, 0), j).wait()

        t0, t1 = 2 * t, 2 * t + 1
        run('D', [('g', t0, z2b, ALL), ('o', t0, None, D // TN - 1, out_copy(t, 0)),
                  ('g', t1, z2b, ALL), ('o', t1, None, OS - 1, out_copy(t, 1))])
        out_copy(t, 2).start()
        return carry

    lax.fori_loop(0, 3, functools.partial(stage_c, False), 0)
    lax.fori_loop(3, NT, functools.partial(stage_c, True), 0)
    zbuf = {3: (zc, 1), 4: (zc, 0), 5: (zt[0], 0), 6: (zt[1], 0), 7: (zc, 0)}
    for i in range(NT, NT + 3):
        p0, p1 = i % 2, (i + 1) % 2
        sz_old, sz_new = (SZ, SL) if p0 == 0 else (SL, SZ)
        items = [('z1', i - 4, p0, ALL[3:4]), ('xn', zp, i - 3, p1, 0), ('z2n', i - 5, zbuf[i - 5], z2b, sz_old[1]),
                 ('zstat', zbuf[i - 4])]
        stats = [sz_new]
        if i - 2 < NT:
            items += [('x3', i - 2, p0)]
            stats += [SX]
        if i - 1 < NT:
            items += [('x2stat', p1)]
            stats += [S2]
        items += [('z1', i - 4, p0, ALL[4:]), ('z1', i - 3, p1, ALL[:3])]
        gates = [('mean', [x]) for x in stats] + [('rstd', [x]) for x in stats]
        for n in ALL:
            items += gates[n:n + 1] + [('z2', zbuf[i - 3], p1, [n])]
        run('V3%d' % i, items)
    t = NT - 1
    run('T1', [('kick',), ('zstat', zbuf[t]), ('z2n', t - 1, zbuf[t - 1], z2b, SL[1]), ('z1', t, 1, [3]),
               ('mean', [SZ]), ('z1', t, 1, [4]), ('rstd', [SZ]), ('z1', t, 1, [5])])
    run('T2', [('kick',), ('z2n', t, zbuf[t], z2b, SZ[1]), ('z1', t, 1, [6])])
    lax.fori_loop(0, NT // 2, stage_d, 0)
    for t in range(NT // 2 - 2, NT // 2):
        for j in range(3):
            out_copy(t, j).wait()


@jax.jit
def pallas_interleave_layers__ssm_conv_h3__mixer_gmlp__prompt_kernel(
        A_q, A_k, A_v, A_shift_k, A_ssm_k, A_ssm_D, B_x, B_w_in, B_w_sp, B_b_sp, B_w_out):
    del B_x
    any_spec = pl.BlockSpec(memory_space=pl.ANY)
    scratch = [
        pltpu.VMEM((2, TM + 16, D), bf16),
        pltpu.VMEM((8, B + 16, D), bf16),
        pltpu.VMEM((8, B, D), bf16),
        pltpu.VMEM((2, D, TM), bf16),
        pltpu.VMEM((D, F), bf16),
        pltpu.VMEM((NT, TM, S), bf16),
        pltpu.VMEM((FH, D), bf16),
        pltpu.VMEM((KS, D), bf16),
        pltpu.VMEM((8, 128), bf16),
        pltpu.VMEM((16, 128), bf16),
        pltpu.VMEM((NT, TM + 8, D), f32),
        pltpu.VMEM((NT, TM, D), f32),
        pltpu.VMEM((NT, TM, FH), bf16),
        pltpu.VMEM((S // 2, FH), u32),
        pltpu.VMEM((S // 2, FH), u32),
        pltpu.VMEM((NT, TM, 128), f32),
        pltpu.VMEM((KS + 1, 8, D), f32),
        pltpu.VMEM((2 * B, B), bf16),
        pltpu.VMEM((B, 2 * B), bf16),
        pltpu.VMEM((4, B, D), bf16),
        [pltpu.VMEM((2, 2 * B + 8, D), f32)] * NT,
        [pltpu.VMEM((2, 2 * B + 8, D), f32)] * NT,
        pltpu.VMEM((1, TM, D), f32),
        pltpu.VMEM((NZ, 2 * B + 8, D), f32),
        pltpu.VMEM((2, 2 * B, D), bf16),
        pltpu.VMEM((2, TM // 2 + 8, D), u32),
        [pltpu.VMEM((1, TM + 8, FH), f32)] * 2,
        pltpu.VMEM((2, TM + 8, FH), f32),
        pltpu.VMEM((7, TM, 128), f32),
        pltpu.VMEM((8, TM, 128), f32),
        pltpu.VMEM((1, TM // 2 + 8, FH - TN), u32),
        pltpu.VMEM((1, TM // 2 + 8, TN), u32),
        pltpu.SMEM((16,), jnp.int32),
        pltpu.SemaphoreType.DMA((8,)),
        pltpu.SemaphoreType.DMA((3,)),
        pltpu.SemaphoreType.DMA((2,)),
        pltpu.SemaphoreType.DMA((6,)),
    ]
    out = pl.pallas_call(
        _kernel,
        out_shape=jax.ShapeDtypeStruct((NT, TM, D), bf16),
        in_specs=[any_spec] * 10,
        out_specs=any_spec,
        scratch_shapes=scratch,
        compiler_params=pltpu.CompilerParams(vmem_limit_bytes=127 * 1024 * 1024),
    )(A_q.reshape(NT, TM, D), A_k.reshape(NB, B, D), A_v.reshape(NB, B, D), A_shift_k.T, A_ssm_k,
      A_ssm_D.reshape(8, 128), B_w_in, B_w_sp.reshape(NT, TM, S), B_b_sp.reshape(16, 128), B_w_out)
    return out.reshape(1, S, D)
```
